```python
import jax
import jax.numpy as jnp

def _softmax(x, axis=-1):
    return jax.nn.softmax(x, axis=axis)
def _gelu(x):
    return jax.nn.gelu(x, approximate=True)
def _silu(x):
    return jax.nn.silu(x)
def _sigmoid(x):
    return jax.nn.sigmoid(x)
def _layernorm(x, axis=-1, eps=1e-5):
    m = jnp.mean(x, axis=axis, keepdims=True)
    v = jnp.var(x, axis=axis, keepdims=True)
    return (x - m) / jnp.sqrt(v + eps)
def _scatter_add(tgt, idx, src, axis=0):
    return tgt.at[idx].add(src)
def _segment_sum(src, seg, n):
    return jax.ops.segment_sum(src, seg, n)
class _Rng:
    def __init__(self, key):
        self._k = key
    def _next(self):
        self._k, sub = jax.random.split(self._k)
        return sub
    def normal(self, shape):
        return jax.random.normal(self._next(), shape, dtype=jnp.bfloat16)
    def randint(self, lo, hi, shape):
        return jax.random.randint(self._next(), shape, lo, hi, dtype=jnp.int32)
    def uniform(self, shape, lo=0.0, hi=1.0):
        return jax.random.uniform(self._next(), shape, jnp.bfloat16, lo, hi)
    def permutation(self, n):
        return jax.random.permutation(self._next(), n)


kernel_name = 'gated_mix__linear_kernel_hedgehog__moe_arch_mod__prompt'

def setup_inputs():
    _rng = _Rng(jax.random.key(int.from_bytes(__import__("os").urandom(4), "little")))
    _w = (lambda a: (lambda t: t.astype(jnp.bfloat16) if jnp.issubdtype(t.dtype, jnp.floating) else t)(jnp.asarray(a)))
    def _A_setup():
        B, S, D, H = 1, 2048, 1024, 32
        Dh = D // H
        return {
            "x": _w((lambda *s: _rng.normal(s) * 0.05)(B, S, D)),
            "wqkv": _w((lambda *s: _rng.normal(s) * 0.05)(D, 3 * D)),
            "w_phi": _w((lambda *s: _rng.normal(s) * 0.05)(H, Dh, Dh) * (Dh ** -0.5)),
            "wo": _w((lambda *s: _rng.normal(s) * 0.05)(D, D)),
        }
    _A_in = _A_setup()

    def _B_setup():
        B, S, D, F, C = 1, 2048, 1024, 3584, 1
        return {
            "x": _w((lambda *s: _rng.normal(s) * 0.05)(B, S, D)),
            "w_r": _w((lambda *s: _rng.normal(s) * 0.05)(D)),
            "w_gate": _w((lambda *s: _rng.normal(s) * 0.05)(D, F)),
            "w_up": _w((lambda *s: _rng.normal(s) * 0.05)(D, F)),
            "w_down": _w((lambda *s: _rng.normal(s) * 0.05)(F, D)),
        }
    _B_in = _B_setup()

    return {
        "A_x": _A_in["x"],
        "A_wqkv": _A_in["wqkv"],
        "A_w_phi": _A_in["w_phi"],
        "A_wo": _A_in["wo"],
        "B_x": _B_in["x"],
        "B_w_r": _B_in["w_r"],
        "B_w_gate": _B_in["w_gate"],
        "B_w_up": _B_in["w_up"],
        "B_w_down": _B_in["w_down"],
        "gate_w": _w((lambda *s: _rng.normal(s) * 0.05)(1024)),
    }

def reference(A_x, A_wqkv, A_w_phi, A_wo, B_x, B_w_r, B_w_gate, B_w_up, B_w_down, gate_w):
    def _A_ref(x, wqkv, w_phi, wo):
        B, S, D = x.shape
        H = 32; Dh = D // H
        qkv = (lambda x, *d: x.transpose(*d))((x @ wqkv).reshape(B, S, 3, H, Dh), 2, 0, 3, 1, 4)
        q, k, v = qkv[0], qkv[1], qkv[2]
        pq = jnp.einsum("bhsd,hdf->bhsf", q, w_phi)
        pk = jnp.einsum("bhsd,hdf->bhsf", k, w_phi)
        phi_q = jnp.concatenate([_softmax(pq, axis=-1), _softmax(-pq, axis=-1)], axis=-1)
        phi_k = jnp.concatenate([_softmax(pk, axis=-1), _softmax(-pk, axis=-1)], axis=-1)
        kv = jnp.einsum("bhsf,bhsd->bhfd", phi_k, v)
        z  = jnp.einsum("bhsf->bhf", phi_k)
        num = jnp.einsum("bhqf,bhfd->bhqd", phi_q, kv)
        den = jnp.einsum("bhqf,bhf->bhq", phi_q, z)[..., None] + 1e-6
        o = num / den
        return (lambda x, *d: x.transpose(*d))(o, 0, 2, 1, 3).reshape(B, S, D) @ wo

    def _B_ref(x, w_r, w_gate, w_up, w_down):
        B, S, D = x.shape
        C = 1
        r = x @ w_r
        idx = jnp.argsort(-r, axis=-1)[:, :C]
        idx_e = jnp.repeat(idx.reshape(B, C, 1), D, axis=2)
        x_sel = jnp.take_along_axis(x, idx_e, axis=1)
        g = _silu(x_sel @ w_gate)
        u = x_sel @ w_up
        y = (g * u) @ w_down
        r_sel = _sigmoid(jnp.take_along_axis(r, idx, axis=1))
        y = y * r_sel.reshape(B, C, 1)
        b_off = (jnp.arange(B) * S).reshape(B, 1)
        flat_idx = (idx + b_off).reshape(B * C)
        zero = (x * 0.0).reshape(B * S, D)
        upd = _scatter_add(zero, flat_idx, y.reshape(B * C, D), axis=0)
        return x + upd.reshape(B, S, D)

    x = A_x
    g = _sigmoid((x * gate_w).sum(-1, keepdims=True))
    a = _A_ref(x, A_wqkv, A_w_phi, A_wo)
    b = _B_ref(x, B_w_r, B_w_gate, B_w_up, B_w_down)
    return g * a + (1 - g) * b
```

```python
import functools
import jax
import jax.numpy as jnp
from jax import lax
import jax.experimental.pallas as pl
import jax.experimental.pallas.tpu as pltpu

F32 = jnp.float32
BF16 = jnp.bfloat16
I32 = jnp.int32
LOG2E = 1.4426950408889634
NT = (((1,), (1,)), ((), ()))


def _ld(v):
    return pltpu.bitcast(v, BF16)


def _st(v):
    return pltpu.bitcast(v.astype(BF16), I32)


def _red(v, op):
    r = v[:, 0]
    for k in range(1, v.shape[1]):
        r = op(r, v[:, k])
    r = op(r, pltpu.roll(r, 4, 1))
    r = op(r, pltpu.roll(r, 2, 1))
    return r


def _rcp(s):
    r = pl.reciprocal(s, approx=True)
    return r * (2.0 - s * r)


def _phi(p):
    n = p.shape[0] // 64
    t = p.shape[1]
    p4 = p.reshape(n, 8, 8, t)
    mx = _red(p4, jnp.maximum)[:, None]
    mn = _red(p4, jnp.minimum)[:, None]
    ep = jnp.exp2(p4 - mx)
    en = jnp.exp2(mn - p4)
    ep = ep * _rcp(_red(ep, jnp.add))[:, None]
    en = en * _rcp(_red(en, jnp.add))[:, None]
    return jnp.concatenate([ep, en], axis=1).reshape(n * 128, t)


def _make_kernel(S, D, F, H, T, FC, WC, F0):
    NTILE = S // T
    NCH = F // FC
    G = D // 128
    L = T // 128
    NW = D // WC
    NO = D // 256

    def kernel(ax_h, wqkv_h, wphi_h, wo_h, wr_h, wg_h, wu_h, wd_h, gw_h, out_h,
               x_v, w_v, wt_v, wphi_v, bd_v, wo_v, wr_v, gw_v, wg_v, wu_v, wd_v,
               pq_v, gate_v, kv_v, kvb_v, z_v, xb_v, o_v, out_v,
               sem_x, sem_q, sem_w, sem_s, sem_f, sem_o):
        def cp_x(i):
            return pltpu.make_async_copy(ax_h.at[pl.ds(i * T, T)], x_v.at[i].bitcast(BF16), sem_x.at[i])

        def cp_q(c):
            return pltpu.make_async_copy(wqkv_h.at[:, pl.ds(c * WC, WC)],
                                         w_v.at[0, c].bitcast(BF16), sem_q.at[c])

        def cp_w(j):
            return [pltpu.make_async_copy(wqkv_h.at[:, pl.ds(j * D + c * WC, WC)],
                                          w_v.at[j, c].bitcast(BF16), sem_w.at[(j - 1) * NW + c]) for c in range(NW)]

        cp_wo = pltpu.make_async_copy(wo_h, wo_v.bitcast(BF16), sem_s.at[3])
        cp_phi = pltpu.make_async_copy(wphi_h, wphi_v, sem_s.at[0])
        cp_wr = pltpu.make_async_copy(wr_h, wr_v, sem_s.at[1])
        cp_gw = pltpu.make_async_copy(gw_h, gw_v, sem_s.at[2])

        def cp_f(c):
            return (
                pltpu.make_async_copy(wg_h.at[:, pl.ds(c * FC, FC)], wg_v.at[c].bitcast(BF16), sem_f.at[c]),
                pltpu.make_async_copy(wu_h.at[:, pl.ds(c * FC, FC)], wu_v.at[c].bitcast(BF16), sem_f.at[NCH + c]),
                pltpu.make_async_copy(wd_h.at[pl.ds(c * FC, FC)], wd_v.at[c].bitcast(BF16), sem_f.at[2 * NCH + c]),
            )

        def cp_o(i, n):
            return pltpu.make_async_copy(out_v.at[i, n].bitcast(BF16),
                                         out_h.at[pl.ds(i * T, T), pl.ds(n * 256, 256)], sem_o.at[i * NO + n])

        cp_phi.start()
        cp_q(0).start()
        cp_x(0).start()
        cp_wr.start()
        cp_gw.start()
        for c in range(1, NW):
            cp_q(c).start()

        kv_v[...] = jnp.zeros_like(kv_v)
        z_v[...] = jnp.zeros_like(z_v)

        r128 = lax.broadcasted_iota(I32, (128, 128), 0)
        c128 = lax.broadcasted_iota(I32, (128, 128), 1)
        diag = ((r128 // 64) * 2 + (r128 % 2)) == (c128 // 32)
        er = lax.broadcasted_iota(I32, (128, 32), 0)
        ec = lax.broadcasted_iota(I32, (128, 32), 1)
        eye = jnp.where(((er % 64) // 2) == ec, 1.0, 0.0).astype(BF16)
        cp_phi.wait()
        for g in range(G):
            wp = wphi_v[pl.ds(4 * g, 4)].reshape(128, 32)
            bd = lax.dot_general(eye, wp, NT, preferred_element_type=F32)
            bd_v[g] = _st(jnp.where(diag, bd, 0.0))

        def w_cols(j, g):
            c, o = divmod(g * 128, WC)
            return _ld(w_v[j, c, :, o:o + 128])

        def fold(j, g):
            wt = lax.dot_general(_ld(bd_v[g]), w_cols(j, g), NT, preferred_element_type=F32)
            wt_v[j, g] = _st(wt * LOG2E)

        def proj(j, i, g):
            return lax.dot_general(_ld(wt_v[j, g]), _ld(x_v[i]), NT, preferred_element_type=F32)

        best = jnp.full((1, 1), -jnp.inf, F32)
        bidx = jnp.zeros((1, 1), I32)
        pend = None
        RC = 32
        for i in range(NTILE):
            cp_x(i).wait()
            if i == 0:
                cp_wr.wait()
                cp_gw.wait()
                gw = gw_v[...].astype(F32).reshape(1, D)
                wr = wr_v[...].astype(F32).reshape(1, D)
            if i + 1 < NTILE:
                cp_x(i + 1).start()
            if i == 1:
                for d in cp_w(1):
                    d.start()
            if i == 2:
                for d in cp_w(2):
                    d.start()
            if i == 4:
                for d in cp_f(0):
                    d.start()
            if i == 6:
                for d in cp_f(1):
                    d.start()
            if i == NTILE - 2:
                for d in cp_w(2):
                    d.wait()
            for g in range(G):
                if i == 0:
                    if (g * 128) % WC == 0:
                        cp_q(g * 128 // WC).wait()
                    fold(0, g)
                p = proj(0, i, g)
                if pend is not None:
                    pi, pg, pp = pend
                    pq_v[pi, pg] = _st(_phi(pp))
                pend = (i, g, p)
                r0 = g * RC
                xs = _ld(x_v[i, r0 // 2:(r0 + RC) // 2, :]).astype(F32)
                gs = jnp.sum(xs * gw, axis=1, keepdims=True)
                gate_v[i, r0:r0 + RC, :] = jnp.broadcast_to(jax.nn.sigmoid(gs), (RC, 128))
                r = jnp.sum(xs * wr, axis=1, keepdims=True).astype(BF16).astype(F32)
                r = jnp.where(r != r, -jnp.inf, r)
                m = jnp.max(r, axis=0, keepdims=True)
                tok = i * T + r0 + lax.broadcasted_iota(I32, (RC, 1), 0)
                am = jnp.min(jnp.where(r == m, tok, S), axis=0, keepdims=True)
                better = m > best
                bidx = jnp.where(better, am, bidx)
                best = jnp.where(better, m, best)
                if i >= NTILE - 2 and g % 2 == 0:
                    gg = (i - (NTILE - 2)) * 4 + g // 2
                    wt_v[2, gg] = pltpu.bitcast(w_cols(2, gg).T, I32)

        for d in cp_w(1):
            d.wait()
        for d in cp_f(2):
            d.start()
        fold(1, 0)
        pi, pg, pp = pend
        pq_v[pi, pg] = _st(_phi(pp))
        idx = jnp.max(bidx)
        for g in range(1, G):
            fold(1, g)
        it = idx // T
        base = pl.multiple_of(((idx % T) // 16) * 8, 8)
        blk = _ld(x_v[it, pl.ds(base, 8), :]).astype(F32)
        sel = lax.broadcasted_iota(I32, (16, D), 0) == (idx % 16)
        xs = jnp.sum(jnp.where(sel, blk, 0.0), axis=0, keepdims=True)
        for g in range(G):
            xb_v[g * 128:(g + 1) * 128, :] = jnp.broadcast_to(xs[:, g * 128:(g + 1) * 128], (128, 128)).T
        r_sel = jnp.sum(xs * wr, axis=1, keepdims=True)
        r_gate = jax.nn.sigmoid(r_sel.astype(BF16).astype(F32))

        FL = FC // 128

        def matvec(w_ref, c, k0, k1, lanes, xb):
            acc = jnp.sum((_ld(w_ref[c, k0 // 2:k1 // 2, :]).astype(F32) * jnp.concatenate([xb] * lanes, axis=1))
                          .reshape((k1 - k0) // 8, 8, lanes * 128), axis=0)
            return acc

        def kv_step(vt, ph, g):
            zs = ph[:, 0:128]
            for l in range(1, L):
                zs = zs + ph[:, l * 128:(l + 1) * 128]
            z_v[g] += zs
            phb = ph.astype(BF16)
            for q in range(2):
                kv_v[2 * g + q] += lax.dot_general(
                    vt[q * 64:(q + 1) * 64], phb[q * 128:(q + 1) * 128], NT, preferred_element_type=F32)

        yacc = jnp.zeros((8, D), F32)
        pend = None
        for i in range(NTILE):
            c = i - F0
            do_f = 0 <= c < NCH
            if do_f:
                for d in cp_f(c):
                    d.wait()
            if i + 3 < NCH:
                for d in cp_f(i + 3):
                    d.start()
            if i == NCH - 3:
                cp_wo.start()
            for g in range(G):
                p = proj(1, i, g)
                if pend is not None:
                    kv_step(*pend)
                if do_f:
                    if g < 2:
                        ga = matvec(wg_v, c, g * 512, (g + 1) * 512, FL, xb_v[g * 512:(g + 1) * 512, :])
                        gacc = ga if g == 0 else gacc + ga
                    elif g < 4:
                        ua = matvec(wu_v, c, (g - 2) * 512, (g - 1) * 512, FL, xb_v[(g - 2) * 512:(g - 1) * 512, :])
                        uacc = ua if g == 2 else uacc + ua
                    else:
                        if g == 4:
                            gsum = jnp.sum(gacc, axis=0, keepdims=True)
                            hh = gsum * jax.nn.sigmoid(gsum) * jnp.sum(uacc, axis=0, keepdims=True)
                        for l in range((g - 4) * FL // 4, (g - 3) * FL // 4):
                            hb = jnp.broadcast_to(hh[:, l * 128:(l + 1) * 128], (128, 128)).T
                            yacc = yacc + matvec(wd_v, c, l * 128, (l + 1) * 128, G, hb)
                vt = proj(2, i, g).astype(BF16)
                pend = (vt, _phi(p), g)

        cp_wo.wait()
        kv_step(*pend)
        y = jnp.sum(yacc, axis=0, keepdims=True) * r_gate
        kr = lax.broadcasted_iota(I32, (64, 128), 0)
        kc = lax.broadcasted_iota(I32, (64, 128), 1)
        kmask = (kr // 32) == (kc % 2)
        for j in range(H // 2):
            kvb_v[j] = _st(jnp.where(kmask, kv_v[j], 0.0))
        for g in range(G):
            z_v[g] = jnp.broadcast_to(jnp.sum(z_v[g], axis=1, keepdims=True), (256, 128))

        def attn(i, g):
            phq = _ld(pq_v[i, g])
            zb = jnp.concatenate([z_v[g]] * L, axis=1)
            den = _red((phq.astype(F32) * zb).reshape(2, 16, 8, T), jnp.add) + 1e-6
            rden = 1.0 / den
            os_ = []
            for q in range(2):
                num = jnp.dot(_ld(kvb_v[2 * g + q]), phq[q * 128:(q + 1) * 128], preferred_element_type=F32)
                os_.append(num[0:32] * rden[q, 0:1])
                os_.append(num[32:64] * rden[q, 1:2])
            o = jnp.concatenate(os_, axis=0).astype(BF16)
            o_v[i % 2, :, g * 128:(g + 1) * 128] = pltpu.bitcast(o.T, I32)

        def mix(i, n, a):
            g = jnp.concatenate([gate_v[i]] * 2, axis=1)
            xt = _ld(x_v[i, :, n * 256:(n + 1) * 256]).astype(F32)
            tok = i * T + lax.broadcasted_iota(I32, (T, 256), 0)
            upd = xt * 0.0 + jnp.where(tok == idx, y[:, n * 256:(n + 1) * 256], 0.0)
            b = xt + upd
            out_v[i, n] = _st(g * a + (1.0 - g) * b)
            cp_o(i, n).start()

        for g in range(G):
            attn(0, g)
        pend = None
        for i in range(NTILE):
            for n in range(NO):
                a = jnp.dot(_ld(o_v[i % 2]), _ld(wo_v[:, n * 256:(n + 1) * 256]), preferred_element_type=F32)
                if pend is not None:
                    mix(*pend)
                pend = (i, n, a)
                if i + 1 < NTILE:
                    for g in range(n * G // NO, (n + 1) * G // NO):
                        attn(i + 1, g)
        mix(*pend)
        for i in range(NTILE):
            for n in range(NO):
                cp_o(i, n).wait()

    return kernel


def make(T=256, FC=512, WC=256, F0=1):
    @jax.jit
    def run(A_x, A_wqkv, A_w_phi, A_wo, B_x, B_w_r, B_w_gate, B_w_up, B_w_down, gate_w):
        B, S, D = A_x.shape
        F = B_w_gate.shape[1]
        H = A_w_phi.shape[0]
        NTILE = S // T
        NCH = F // FC
        G = D // 128
        NW = D // WC
        any_spec = pl.BlockSpec(memory_space=pl.ANY)
        V = pltpu.VMEM
        scratch = [
            V((NTILE, T // 2, D), I32),
            V((3, NW, D // 2, WC), I32),
            V((3, G, 64, D), I32),
            V((H, 32, 32), BF16),
            V((G, 64, 128), I32),
            V((D // 2, D), I32),
            V((D,), BF16),
            V((D,), BF16),
            V((NCH, D // 2, FC), I32),
            V((NCH, D // 2, FC), I32),
            V((NCH, FC // 2, D), I32),
            V((NTILE, G, 128, T), I32),
            V((NTILE, T, 128), F32),
            V((H // 2, 64, 128), F32),
            V((H // 2, 32, 128), I32),
            V((G, 256, 128), F32),
            V((D, 128), F32),
            V((2, T // 2, D), I32),
            V((NTILE, D // 256, T // 2, 256), I32),
            pltpu.SemaphoreType.DMA((NTILE,)),
            pltpu.SemaphoreType.DMA((NW,)),
            pltpu.SemaphoreType.DMA((2 * NW,)),
            pltpu.SemaphoreType.DMA((4,)),
            pltpu.SemaphoreType.DMA((3 * NCH,)),
            pltpu.SemaphoreType.DMA((NTILE * (D // 256),)),
        ]
        out = pl.pallas_call(
            _make_kernel(S, D, F, H, T, FC, WC, F0),
            out_shape=jax.ShapeDtypeStruct((S, D), A_x.dtype),
            in_specs=[any_spec] * 9,
            out_specs=any_spec,
            scratch_shapes=scratch,
            compiler_params=pltpu.CompilerParams(vmem_limit_bytes=100 * 2**20),
        )(A_x.reshape(S, D), A_wqkv, A_w_phi, A_wo, B_w_r, B_w_gate, B_w_up, B_w_down, gate_w)
        return out.reshape(B, S, D)
    return run


_run = make()


@jax.jit
def pallas_gated_mix__linear_kernel_hedgehog__moe_arch_mod__prompt_kernel(
    A_x, A_wqkv, A_w_phi, A_wo, B_x, B_w_r, B_w_gate, B_w_up, B_w_down, gate_w
):
    return _run(A_x, A_wqkv, A_w_phi, A_wo, B_x, B_w_r, B_w_gate, B_w_up, B_w_down, gate_w)
```

```python
import contextlib

import jax
import jax.numpy as jnp
from jax import lax
import jax.experimental.pallas as pl
import jax.experimental.pallas.tpu as pltpu

F32 = jnp.float32
BF16 = jnp.bfloat16
I32 = jnp.int32
LOG2E = 1.4426950408889634
NT = (((1,), (1,)), ((), ()))
NN = (((1,), (0,)), ((), ()))


def _ld(v):
    return pltpu.bitcast(v, BF16)


def _pack(a, b):
    return pltpu.bitcast(pltpu.pack_elementwise([a, b], packed_dtype=BF16), I32)


def _unpack(w, k):
    return pltpu.unpack_elementwise(w, index=k, packed_dtype=BF16, unpacked_dtype=F32)


def _tree(vs, op):
    while len(vs) > 1:
        vs = [op(vs[k], vs[k + 1]) if k + 1 < len(vs) else vs[k] for k in range(0, len(vs), 2)]
    return vs[0]


def _left(a11, a12, a21, a22):
    return [a11 + a22, a21 + a22, a11, a22, a11 + a12, a21 - a11, a12 - a22]


def _right(b11, b12, b21, b22):
    return [b11 + b22, b11, b12 - b22, b21 - b11, b22, b11 + b12, b21 + b22]


def _combine(mul, jobs):
    count = [0]

    def step(m):
        t = mul(m)
        for n, fn in jobs:
            if n == count[0]:
                fn()
        count[0] += 1
        return t

    m1 = step(0)
    c11 = m1 + step(6)
    c22 = m1 + step(5)
    m4 = step(3)
    c11 = c11 + m4
    m5 = step(4)
    c11 = c11 - m5
    m2 = step(1)
    c21 = m4 + m2
    c22 = c22 - m2
    m3 = step(2)
    return (c11, m5 + m3), (c21, c22 + m3)


def _red(v, op):
    r = _tree([v[k] for k in range(v.shape[0])], op)
    r = op(r, pltpu.roll(r, 4, 0))
    return op(r, pltpu.roll(r, 2, 0))


def _rcp(s):
    r = pl.reciprocal(s, approx=True)
    return r * (2.0 - s * r)


def _phi(p):
    p = p.reshape(8, 8, 128)
    ep = jnp.exp2(p - _red(p, jnp.maximum))
    en = jnp.exp2(_red(p, jnp.minimum) - p)
    ep = ep * _rcp(_red(ep, jnp.add))
    en = en * _rcp(_red(en, jnp.add))
    return ep.reshape(64, 128), en.reshape(64, 128)


def _make_kernel(S, D, F, H, P):
    scope = jax.named_scope if P["PROF"] else (lambda n: contextlib.nullcontext())
    T = 256
    NTILE = S // T
    G = D // 128
    U = G // 2
    K2 = D // 2
    NF = F // 128
    F0, CLK = P["F0"], P["CLK"]
    NA = (NTILE - F0) * U
    assert (NF - NA) * 6 + 3 <= (NTILE - 1) * U
    SUMS = (0, 2, 3, 5, 6)

    def kernel(ax_h, wqkv_h, wphi_h, wo_h, wr_h, wg_h, wu_h, wd_h, gw_h, out_h,
               x_v, xs_v, w_v, wa_v, wphi_v, wo_v, wr_v, gw_v, wg_v, wu_v, wd_v,
               pq_v, gate_v, kv_v, z_v, xb_v, out_v, sem):
        def cp_x(lo, hi, s):
            return pltpu.make_async_copy(ax_h.at[pl.ds(lo * T, (hi - lo) * T)],
                                         x_v.at[pl.ds(lo * T // 2, (hi - lo) * T // 2)].bitcast(BF16), sem.at[s])

        def cp_q(lo, hi, s):
            return pltpu.make_async_copy(wqkv_h.at[:, pl.ds(lo * 256, (hi - lo) * 256)],
                                         w_v.at[0, :, pl.ds(lo * 256, (hi - lo) * 256)].bitcast(BF16), sem.at[s])

        cp_small = [pltpu.make_async_copy(wr_h, wr_v, sem.at[7]), pltpu.make_async_copy(gw_h, gw_v, sem.at[7]),
                    pltpu.make_async_copy(wphi_h, wphi_v, sem.at[7])]
        half = NTILE // 2
        cp_x0, cp_x1, cp_x2, cp_x3 = cp_x(0, 1, 0), cp_x(1, 2, 5), cp_x(2, half, 1), cp_x(half, NTILE, 10)
        cp_q0, cp_q1, cp_q2 = cp_q(0, 1, 3), cp_q(1, 3, 4), cp_q(3, 4, 5)
        cp_kv = [pltpu.make_async_copy(wqkv_h.at[:, pl.ds(j * D, D)], w_v.at[j].bitcast(BF16), sem.at[2])
                 for j in (1, 2)]

        def cp_ffn(lo, n, s):
            return [
                pltpu.make_async_copy(wg_h.at[:, pl.ds(lo, n)], wg_v.at[:, pl.ds(lo, n)].bitcast(BF16), sem.at[s]),
                pltpu.make_async_copy(wu_h.at[:, pl.ds(lo, n)], wu_v.at[:, pl.ds(lo, n)].bitcast(BF16), sem.at[s]),
                pltpu.make_async_copy(wd_h.at[pl.ds(lo, n)], wd_v.at[pl.ds(lo // 2, n // 2)].bitcast(BF16), sem.at[s]),
            ]

        cuts = list(range(0, NA, 2 * U)) + [NA, NF]
        cp_f = [cp_ffn(lo * 128, (hi - lo) * 128, 11 + n) for n, (lo, hi) in enumerate(zip(cuts, cuts[1:]))]
        cp_f[0].append(pltpu.make_async_copy(wo_h, wo_v.bitcast(BF16), sem.at[11]))

        def start(ds):
            for d in ds:
                d.start()

        def wait(ds, name):
            with scope(name):
                for d in ds:
                    d.wait()

        start(cp_small + [cp_q0, cp_x0])

        kv_v[...] = jnp.zeros_like(kv_v)
        z_v[...] = jnp.zeros_like(z_v)

        r128 = lax.broadcasted_iota(I32, (128, 128), 0)
        c128 = lax.broadcasted_iota(I32, (128, 128), 1)
        diag = (2 * ((r128 % 64) // 32) + r128 // 64) == (c128 // 32)
        er = lax.broadcasted_iota(I32, (128, 32), 0)
        ec = lax.broadcasted_iota(I32, (128, 32), 1)
        eye = jnp.where((er % 32) == ec, 1.0, 0.0).astype(BF16)
        wait(cp_small, "w_small")
        start([cp_q1])
        bd = []
        for g in range(G):
            wp = wphi_v[pl.ds(4 * g, 4)].reshape(128, 32)
            t = lax.dot_general(eye, wp, NT, preferred_element_type=F32)
            bd.append(pltpu.bitcast(jnp.where(diag, t, 0.0).astype(BF16), I32))
        gw = gw_v[...].astype(F32).reshape(1, D)
        wr = wr_v[...].astype(F32).reshape(1, D)

        never = lax.broadcasted_iota(I32, (8, 128), 0) > (pltpu.bitcast(gw[:, 0:128], I32) & 0xFFFF) + 8
        clock = []

        def after(w, dep, every=False):
            if dep is None:
                return w
            dep = pltpu.bitcast(dep, w.dtype)
            if every:
                return jnp.concatenate([jnp.concatenate(
                    [jnp.where(never, dep, w[r:r + 8, c:c + 128]) for c in range(0, w.shape[1], 128)], axis=1)
                    for r in range(0, w.shape[0], 8)], axis=0)
            w0 = jnp.where(never, dep, w[0:8, 0:128])
            if w.shape[1] > 128:
                w0 = jnp.concatenate([w0, w[0:8, 128:]], axis=1)
            return jnp.concatenate([w0, w[8:]], axis=0) if w.shape[0] > 8 else w0

        def now(back=1):
            return clock[-back] if len(clock) >= back else None

        due = {}
        tick = []

        def before(v, ahead):
            parts = [v[r:r + 8, c:c + 128] for r in range(0, v.shape[0], 8) for c in range(0, v.shape[1], 128)]
            due.setdefault(len(clock) + ahead, []).append(_tree(parts, jnp.maximum))

        def mm(w, rhs, dims):
            deps = due.pop(len(clock), []) + tick + ([now(CLK)] if len(clock) >= CLK else [])
            if deps:
                tick[:] = [_tree(deps, jnp.maximum)]
                w = after(w, tick[0])
            t = lax.dot_general(_ld(w), rhs, dims, preferred_element_type=F32)
            clock.append(t[0:8, 0:128])
            return t

        def fold(j, s):
            a, b = [mm(bd[g], _ld(w_v[j, :, g * 128:(g + 1) * 128]), NT) * LOG2E for g in (2 * s, 2 * s + 1)]
            for m, t in enumerate(_left(a[:, :K2], a[:, K2:], b[:, :K2], b[:, K2:])):
                wa_v[j, s, m] = _pack(t[0:64], t[64:128])

        def prep_w(j, ref, s):
            def job(c):
                def run():
                    blocks = [pltpu.bitcast(_ld(after(ref[(k * U + c) * 64:(k * U + c + 1) * 64, g * 128:(g + 1) * 128],
                                                      now())).T, I32)
                              for g in (2 * s, 2 * s + 1) for k in range(2)]
                    lo, hi = [_left(*[_unpack(w, e) for w in blocks]) for e in range(2)]
                    for m in range(7):
                        wa_v[j, s, m, :, c * 128:(c + 1) * 128] = (
                            blocks[0] if m == 2 else blocks[3] if m == 3 else _pack(lo[m], hi[m]))
                return run
            return [job(c) for c in range(U)]

        def xblk(i, t, k, c=None):
            cols = slice(k * K2, (k + 1) * K2) if c is None else slice(k * K2 + c * 128, k * K2 + (c + 1) * 128)
            return x_v[(2 * i + t) * 64:(2 * i + t + 1) * 64, cols]

        route = [jnp.full((1, 1), -jnp.inf, F32), jnp.zeros((1, 1), I32)]

        def prep_x(i):
            acc = {}

            def job(c):
                def run():
                    words = [after(xblk(i, 0, 0, c), now(P["XL"]), True), xblk(i, 1, 0, c),
                             xblk(i, 0, 1, c), after(xblk(i, 1, 1, c), now(P["XL"]), True)]
                    vals = [[_unpack(w, e) for w in words] for e in range(2)]
                    lo, hi = [_right(*v) for v in vals]
                    for m in range(7):
                        t = words[0] if m == 1 else words[3] if m == 4 else _pack(lo[m], hi[m])
                        xs_v[i, m, c * 64:(c + 1) * 64, :] = pltpu.bitcast(_ld(t).T, I32)
                    w1, w2 = wr[:, c * 128:(c + 1) * 128], wr[:, K2 + c * 128:K2 + (c + 1) * 128]
                    for t in range(2):
                        for e in range(2):
                            part = vals[e][t] * w1 + vals[e][2 + t] * w2
                            acc[t, e] = part if c == 0 else acc[t, e] + part
                    if c < U - 1:
                        return
                    for t in range(2):
                        rs, toks = [], []
                        for e in range(2):
                            r = jnp.sum(acc[t, e], axis=1, keepdims=True).astype(BF16).astype(F32)
                            rs.append(jnp.where(r != r, -jnp.inf, r))
                            toks.append(i * T + t * 128 + e + 2 * lax.broadcasted_iota(I32, (64, 1), 0))
                        top = jnp.max(jnp.maximum(*rs), axis=0, keepdims=True)
                        arg = jnp.min(jnp.minimum(*[jnp.where(r == top, k, S) for r, k in zip(rs, toks)]),
                                      axis=0, keepdims=True)
                        better = top > route[0]
                        route[1] = jnp.where(better, arg, route[1])
                        route[0] = jnp.where(better, top, route[0])
                return run
            return [job(c) for c in range(U)]

        def gates(i):
            def job(t, r0):
                def run():
                    lo = (i * T + t * 128 + r0) // 2
                    xs = _ld(after(x_v[lo:lo + 32, :], now())).astype(F32)
                    gs = jnp.sum(xs * gw, axis=1, keepdims=True)
                    gate_v[i, t, r0:r0 + 64, :] = jnp.broadcast_to(jax.nn.sigmoid(gs), (64, 128))
                return run
            return [job(t, r0) for t in range(2) for r0 in (0, 64)]

        def x_op(i, m):
            return xs_v[i, m]

        def proj(j, i, s, jobs):
            ops = [x_op(i, m) for m in range(7)]
            return _combine(lambda m: mm(wa_v[j, s, m], _ld(ops[m]), NN), jobs)

        held = []

        def phi_q(i, s, ps):
            def job(e, q):
                def run():
                    for t in range(2):
                        held.append(((i, 2 * s + e, slice(q * 64, (q + 1) * 64), slice(t * 128, (t + 1) * 128)),
                                     _pack(*_phi(after(ps[e][t][q * 64:(q + 1) * 64], now(P["QL"]))))))
                    if i < NTILE - 1:
                        store_held()
                return run
            return [job(e, q) for e in range(2) for q in range(2)]

        def store_held():
            while held:
                where, val = held.pop(0)
                pq_v[where] = val

        def at(slots, jobs):
            return list(zip(slots, jobs))

        wait([cp_q0], "w_q0")
        fold(0, 0)
        wait([cp_x0], "w_x0")
        start([cp_q2, cp_x1])
        for fn in prep_x(0):
            fn()
        pend = []

        def sync(done, name, begin):
            def run():
                wait(done, name)
                start(begin)
            return [(P["HS"], run)]

        for i in range(NTILE - 1):
            px = prep_x(i + 1)
            for s in range(U):
                jobs = []
                if i == 0:
                    if s == 1:
                        wait([cp_q1], "w_q1")
                        start([cp_x2])
                        fold(0, 1)
                        fold(0, 2)
                    if s == 2:
                        wait([cp_q2, cp_x1], "w_q2")
                        start([cp_x3])
                        fold(0, 3)
                    if s >= 2:
                        jobs += at(P["HX2"], px[2 * (s - 2):2 * (s - 1)])
                else:
                    if (i, s) == (1, 0):
                        jobs += sync([cp_x2], "w_x2", cp_kv)
                    if (i, s) == (half - 1, 0):
                        jobs += sync([cp_x3], "w_x3", [])
                    if (i, s) == (NTILE - 2, 0):
                        jobs += sync(cp_kv, "w_kv", cp_f[0])
                    jobs += at(P["HX"], px[s:s + 1])
                if i == NTILE - 2:
                    jobs += at(P["HW"], prep_w(2, w_v.at[2], s))
                    jobs += at(P["HK"], [lambda s=s: fold(1, s)])
                pend = phi_q(i, s, proj(0, i, s, jobs + at(P["HA"], pend)))

        idx = jnp.max(route[1])
        blk = _ld(x_v[pl.ds(pl.multiple_of((idx // 16) * 8, 8), 8), :]).astype(F32)
        sel = lax.broadcasted_iota(I32, (16, D), 0) == (idx % 16)
        xs = jnp.sum(jnp.where(sel, blk, 0.0), axis=0, keepdims=True)
        r_sel = jnp.sum(xs * wr, axis=1, keepdims=True)
        r_gate = jax.nn.sigmoid(r_sel.astype(BF16).astype(F32))

        def spread_token():
            for g in range(G):
                xb_v[g * 128:(g + 1) * 128, :] = after(
                    jnp.broadcast_to(xs[:, g * 128:(g + 1) * 128], (128, 128)), now()).T

        ffn = {"y": [jnp.zeros((8, K2), F32)] * 2}

        def ffn_jobs(f):
            def up(k):
                def run():
                    xb = after(xb_v[k * 256:(k + 1) * 256, :], now(P["FL"]))
                    for name, w_ref in (("g", wg_v), ("u", wu_v)):
                        w = _ld(w_ref[k * 128:(k + 1) * 128, f * 128:(f + 1) * 128]).astype(F32)
                        t = jnp.sum((w * xb).reshape(32, 8, 128), axis=0)
                        ffn[name] = t if k == 0 else ffn[name] + t
                    if k == 3:
                        g, u = [jnp.sum(ffn[name], axis=0, keepdims=True) for name in "gu"]
                        ffn["h", f] = jnp.broadcast_to(g * jax.nn.sigmoid(g) * u, (128, 128)).T
                return run

            def down(n):
                def run():
                    w = _ld(wd_v[(f - 1) * 64:f * 64, n * K2:(n + 1) * K2]).astype(F32)
                    hb = jnp.concatenate([after(ffn["h", f - 1], now(P["FL"]))] * U, axis=1)
                    ffn["y"][n] = ffn["y"][n] + jnp.sum((w * hb).reshape(16, 8, K2), axis=0)
                return run

            return ([down(n) for n in range(2)] if 0 < f else []) + ([up(k) for k in range(4)] if f < NF else [])

        kr = lax.broadcasted_iota(I32, (64, 128), 0)
        kc = lax.broadcasted_iota(I32, (64, 128), 1)
        kmask = (kr // 32) == ((kc // 2) % 2)
        kvb = [None] * (H // 2)

        def kv_step(i, s, ps, vs):
            def job(e, q):
                def run():
                    tie = now(P["KVL"])
                    g = 2 * s + e
                    j = 2 * g + q
                    rows = slice(q * 64, (q + 1) * 64)
                    phis = [_phi(after(ps[e][t][rows], tie)) for t in range(2)]
                    zs = [z_v[g, sign, rows] + (phis[0][sign] + phis[1][sign]) for sign in range(2)]
                    phb = jnp.concatenate([_pack(*ph) for ph in phis], axis=1)
                    kv_v[j] += mm(vs[2 * e + q], _ld(phb), NT)
                    if i == NTILE - 1:
                        zs = [jnp.broadcast_to(jnp.sum(z, axis=1, keepdims=True), (64, 128)) for z in zs]
                        t = jnp.concatenate([kv_v[j, pl.ds(0, 32, stride=2), :], kv_v[j, pl.ds(1, 32, stride=2), :]],
                                            axis=0)
                        kvb[j] = pltpu.bitcast(jnp.where(kmask, t, 0.0).astype(BF16), I32)
                    for sign in range(2):
                        z_v[g, sign, rows] = zs[sign]
                return run
            return [job(e, q) for e in range(2) for q in range(2)]

        def tile(i):
            return idx // T if i == NTILE - 1 else i + (idx // T <= i).astype(I32)

        o_pairs, o_parts = {}, {}

        def attn(i, g):
            def pair(h, q):
                def run():
                    rows = slice(q * 64, (q + 1) * 64)
                    w = pq_v[tile(i), h, rows]
                    dn = (_unpack(w, 0) * jnp.concatenate([after(z_v[h, 0, rows], now(P["AL"]))] * 2, axis=1)
                          + _unpack(w, 1) * jnp.concatenate([z_v[h, 1, rows]] * 2, axis=1))
                    rden = 1.0 / (_red(dn.reshape(8, 8, T), jnp.add) + 1e-6)
                    num = mm(kvb[2 * h + q], _ld(w), NN)
                    o_pairs[i, h, q] = [num[0:32] * rden[0:1], num[32:64] * rden[1:2]]
                return run

            def join():
                a, b = [jnp.concatenate(o_pairs.pop((i, h, 0)) + o_pairs.pop((i, h, 1)), axis=0) for h in (g, g + U)]
                o_parts[i, g] = _right(a[:, :128], a[:, 128:], b[:, :128], b[:, 128:])

            return [pair(h, q) for h in (g, g + U) for q in range(2)] + [join]

        def o_ops(i):
            parts = [o_parts.pop((i, g)) for g in range(U)]
            return [jnp.concatenate([p[m] for p in parts], axis=0).astype(BF16) for m in range(7)]

        first = [attn(0, g) for g in range(U)]
        HB = P["HB"]
        for i in range(NTILE):
            gj = gates(i)
            for s in range(U):
                fj = ffn_jobs((i - F0) * U + s) if i >= F0 else []
                if (i, s) == (0, 0):
                    fj = [spread_token]
                n, odd = divmod(i - F0, 2)
                if s == U - 1 and n >= -1 and odd:
                    start(cp_f[n + 2] if n + 2 < len(cp_f) else [])
                vt = proj(2, i, s, (sync(cp_f[n], "w_f", []) if s == 0 and n >= 0 and not odd else [])
                          + at(HB[1], pend[:HB[0]]) + at(P["HF"][0], fj[:3]) + at(P["HG"], gj[s:s + 1]))
                vts = [jnp.concatenate([_pack(b[q * 64:q * 64 + 32], b[q * 64 + 32:q * 64 + 64]) for b in vt[e]], axis=1)
                       for e in range(2) for q in range(2)]
                jobs = at(HB[2], pend[HB[0]:]) + at(P["HF"][1], fj[3:])
                if F0 <= i < F0 + U:
                    jobs += at(P["HO"], prep_w(3, wo_v, i - F0)[s:s + 1])
                if i == NTILE - 1 and s >= 2:
                    jobs += at(P["H0"], [first[g][n] for g in (2 * s - 4, 2 * s - 3) for n in range(2)])
                pend = kv_step(i, s, proj(1, i, s, jobs), vts)

        late = [[], [(0, 2), (0, 3), (0, 4), (1, 2), (1, 3), (1, 4)], [(2, 2), (2, 3), (2, 4)], [(3, 2), (3, 3), (3, 4)]]
        for s in range(U):
            jobs = at(P["HA"], pend) + at(P["H1"][s], [first[g][n] for g, n in late[s]])
            pend = phi_q(NTILE - 1, s, proj(0, NTILE - 1, s, jobs))

        def cp_o(i, lo, n):
            return pltpu.make_async_copy(out_v.at[pl.ds(i * T, T), pl.ds(lo, n)],
                                         out_h.at[pl.ds(pl.multiple_of(tile(i) * T, T), T), pl.ds(lo, n)], sem.at[6])

        outs = []

        def mix(i, c, blocks):
            def job(n, t):
                def run():
                    r0, c0 = i * T + t * 128, (2 * c + n) * 128
                    g = gate_v[tile(i), t]
                    xt = _ld(x_v[pl.ds(pl.multiple_of(tile(i) * 128 + t * 64, 64), 64), c0:c0 + 128]).astype(F32)
                    upd = xt * 0.0
                    if i == NTILE - 1:
                        tok = t * 128 + lax.broadcasted_iota(I32, (128, 128), 0)
                        upd = upd + jnp.where(tok == idx % T, ffn["out"][:, c0:c0 + 128], 0.0)
                    a = after(blocks[n][t], now(P["ML"])).T
                    res = g * a + (1.0 - g) * (xt + upd)
                    out_v[r0:r0 + 128, c0:c0 + 128] = res.astype(BF16)
                    before(res, P["DM"])
                    if (n, t) != (1, 1):
                        return
                    if i == NTILE - 1:
                        new = [cp_o(i, c * 256, 256)]
                    else:
                        new = [cp_o(i, 0, D)] if c == U - 1 else []
                    start(new)
                    outs.extend(new)
                return run
            return [job(n, t) for n in range(2) for t in range(2)]

        def finish_ffn():
            ffn["out"] = jnp.sum(jnp.concatenate(ffn["y"], axis=1), axis=0, keepdims=True) * r_gate

        rest = [fn for f in range(NA, NF + 1) for fn in ffn_jobs(f)] + [finish_ffn]
        for i in range(NTILE):
            ops = o_ops(i)
            aj = [fn for g in range(U) for fn in attn(i + 1, g)] if i + 1 < NTILE else []
            for c in range(U):
                jobs = at(P["HA"], pend) + [(n - 7 * c, fn) for n, fn in zip(P["HT"], aj) if n // 7 == c]
                if (i, c) == (0, 0):
                    jobs = sync(cp_f[-1], "w_f", []) + jobs
                if (i, c) == (1, 0):
                    store_held()
                if rest:
                    jobs += at(P["HC"], [rest.pop(0)])
                pend = mix(i, c, _combine(lambda m: mm(wa_v[3, c, m], ops[m], NN), jobs))
        for fn in pend:
            fn()
        wait(outs, "w_out")

    return kernel


DEFAULTS = dict(
    F0=2, DM=5, QL=1, XL=1, ML=1, AL=1, FL=1, HS=1, H0=(0, 1, 3, 6), H1=((), (0, 1, 2, 3, 5, 6), (1, 3, 5), (1, 3, 5)), HC=(6,), CLK=3, KVL=4, PROF=False, FLAGS=None,
    HA=(0, 2, 4, 6), HX=(1,), HX2=(3, 6), HW=(2, 3, 4, 6), HK=(2,),
    HB=(2, (3, 6), (2, 5)), HF=((0, 2, 5), (1, 4, 6)), HG=(4,), HO=(0,),
    A0=[(0, 0), (0, 1), (1, 0), (1, 1), (2, 0), (2, 1), (3, 0), (3, 1), (0, 2), (0, 3), (0, 4), (1, 2), (1, 3), (1, 4),
        (2, 2), (2, 3), (2, 4), (3, 2), (3, 3), (3, 4)],
    HT=(0, 1, 2, 3, 5, 5, 6, 7, 8, 10, 10, 11, 12, 13, 15, 15, 16, 17, 18, 21),
)


def make(**kw):
    P = dict(DEFAULTS, **kw)

    @jax.jit
    def run(A_x, A_wqkv, A_w_phi, A_wo, B_x, B_w_r, B_w_gate, B_w_up, B_w_down, gate_w):
        B, S, D = A_x.shape
        F = B_w_gate.shape[1]
        H = A_w_phi.shape[0]
        NTILE = S // 256
        G = D // 128
        any_spec = pl.BlockSpec(memory_space=pl.ANY)
        V = pltpu.VMEM
        scratch = [
            V((S // 2, D), I32),
            V((NTILE, 7, D // 4, 128), I32),
            V((3, D // 2, D), I32),
            V((4, G // 2, 7, 64, D // 2), I32),
            V((H, 32, 32), BF16),
            V((D // 2, D), I32),
            V((D,), BF16),
            V((D,), BF16),
            V((D // 2, F), I32),
            V((D // 2, F), I32),
            V((F // 2, D), I32),
            V((NTILE, G, 128, 256), I32),
            V((NTILE, 2, 128, 128), F32),
            V((H // 2, 64, 128), F32),
            V((G, 2, 128, 128), F32),
            V((D, 128), F32),
            V((S, D), BF16),
            pltpu.SemaphoreType.DMA((15,)),
        ]
        out = pl.pallas_call(
            _make_kernel(S, D, F, H, P),
            out_shape=jax.ShapeDtypeStruct((S, D), A_x.dtype),
            in_specs=[any_spec] * 9,
            out_specs=any_spec,
            scratch_shapes=scratch,
            compiler_params=pltpu.CompilerParams(vmem_limit_bytes=110 * 2**20, flags=P["FLAGS"]),
        )(A_x.reshape(S, D), A_wqkv, A_w_phi, A_wo, B_w_r, B_w_gate, B_w_up, B_w_down, gate_w)
        return out.reshape(B, S, D)
    return run


_run = make()


@jax.jit
def pallas_gated_mix__linear_kernel_hedgehog__moe_arch_mod__prompt_kernel(
    A_x, A_wqkv, A_w_phi, A_wo, B_x, B_w_r, B_w_gate, B_w_up, B_w_down, gate_w
):
    return _run(A_x, A_wqkv, A_w_phi, A_wo, B_x, B_w_r, B_w_gate, B_w_up, B_w_down, gate_w)
```

```python
import contextlib

import jax
import jax.numpy as jnp
from jax import lax
import jax.experimental.pallas as pl
import jax.experimental.pallas.tpu as pltpu

F32 = jnp.float32
BF16 = jnp.bfloat16
I32 = jnp.int32
LOG2E = 1.4426950408889634
NT = (((1,), (1,)), ((), ()))
NN = (((1,), (0,)), ((), ()))


def _ld(v):
    return pltpu.bitcast(v, BF16)


def _pack(a, b):
    return pltpu.bitcast(pltpu.pack_elementwise([a, b], packed_dtype=BF16), I32)


def _unpack(w, k):
    return pltpu.unpack_elementwise(w, index=k, packed_dtype=BF16, unpacked_dtype=F32)


def _tree(vs, op):
    while len(vs) > 1:
        vs = [op(vs[k], vs[k + 1]) if k + 1 < len(vs) else vs[k] for k in range(0, len(vs), 2)]
    return vs[0]


def _left(a11, a12, a21, a22):
    return [a11 + a22, a21 + a22, a11, a22, a11 + a12, a21 - a11, a12 - a22]


def _right(b11, b12, b21, b22):
    return [b11 + b22, b11, b12 - b22, b21 - b11, b22, b11 + b12, b21 + b22]


def _combine(mul, jobs):
    count = [0]

    def step(m):
        t = mul(m)
        for n, fn in jobs:
            if n == count[0]:
                fn()
        count[0] += 1
        return t

    m1 = step(0)
    c11 = m1 + step(6)
    c22 = m1 + step(5)
    m4 = step(3)
    c11 = c11 + m4
    m5 = step(4)
    c11 = c11 - m5
    m2 = step(1)
    c21 = m4 + m2
    c22 = c22 - m2
    m3 = step(2)
    return (c11, m5 + m3), (c21, c22 + m3)


def _red(v, op):
    r = _tree([v[k] for k in range(v.shape[0])], op)
    r = op(r, pltpu.roll(r, 4, 0))
    return op(r, pltpu.roll(r, 2, 0))


def _rcp(s):
    r = pl.reciprocal(s, approx=True)
    return r * (2.0 - s * r)


def _phi(p, tie):
    p = p.reshape(8, 8, 128)
    ep = jnp.exp2(p - tie(_red(p, jnp.maximum), 0))
    en = jnp.exp2(tie(_red(p, jnp.minimum), 1) - p)
    ep = ep * _rcp(_red(ep, jnp.add))
    en = en * _rcp(_red(en, jnp.add))
    return ep.reshape(64, 128), en.reshape(64, 128)


def _make_kernel(S, D, F, H, P):
    scope = jax.named_scope if P["PROF"] else (lambda n: contextlib.nullcontext())
    T = 256
    NTILE = S // T
    G = D // 128
    U = G // 2
    K2 = D // 2
    NF = F // 128
    F0 = P["F0"]
    NA = P["NA"]
    SUMS = (0, 2, 3, 5, 6)

    def kernel(ax_h, wqkv_h, wphi_h, wo_h, wr_h, wg_h, wu_h, wd_h, gw_h, out_h,
               x_v, xs_v, w_v, wa_v, wphi_v, wo_v, wr_v, gw_v, wg_v, wu_v, wd_v,
               pq_v, gate_v, kv_v, z_v, xb_v, out_v, sem):
        def cp_x(lo, hi, s):
            return pltpu.make_async_copy(ax_h.at[pl.ds(lo * T, (hi - lo) * T)],
                                         x_v.at[pl.ds(lo * T // 2, (hi - lo) * T // 2)].bitcast(BF16), sem.at[s])

        def cp_q(lo, hi, s):
            return pltpu.make_async_copy(wqkv_h.at[:, pl.ds(lo * 256, (hi - lo) * 256)],
                                         w_v.at[0, :, pl.ds(lo * 256, (hi - lo) * 256)].bitcast(BF16), sem.at[s])

        cp_small = [pltpu.make_async_copy(wr_h, wr_v, sem.at[0]), pltpu.make_async_copy(gw_h, gw_v, sem.at[0]),
                    pltpu.make_async_copy(wphi_h.at[0:8], wphi_v.at[0:8], sem.at[0])]
        cp_s = [[cp_q(s, s + 1, 8 + s)] for s in range(U)]
        cp_s[1].append(pltpu.make_async_copy(wphi_h.at[8:H], wphi_v.at[8:H], sem.at[9]))
        cp_1 = [cp_x(0, 1, 1)]
        cp_2 = [cp_x(1, 2, 2)]

        def cp_rows(src, dst, n, s):
            return pltpu.make_async_copy(src.at[pl.ds(n * 256, 256)], dst.at[pl.ds(n * 128, 128)].bitcast(BF16), sem.at[s])

        def cp_slab(f, s):
            cols = pl.ds(f * 128, 128)
            return [pltpu.make_async_copy(wg_h.at[:, cols], wg_v.at[:, cols].bitcast(BF16), sem.at[s]),
                    pltpu.make_async_copy(wu_h.at[:, cols], wu_v.at[:, cols].bitcast(BF16), sem.at[s]),
                    pltpu.make_async_copy(wd_h.at[cols], wd_v.at[pl.ds(f * 64, 64)].bitcast(BF16), sem.at[s])]

        batch = {
            "x23": [[cp_x(i, i + 1, 3)] for i in (2, 3)],
            "x456": [[cp_x(i, i + 1, 4)] for i in (4, 5, 6)],
            "kv": [[cp_x(7, 8, 5)]] + [[cp_rows(wqkv_h.at[:, pl.ds(j * D, D)], w_v.at[j], n, 5)]
                                       for j in (2, 1) for n in range(U)],
            "f0": [cp_slab(f, 7) for f in range(NA)],
            "f1": [[cp_rows(wo_h, wo_v, n, 12)] + cp_slab(NA + n, 12) for n in range(U)]
                  + [cp_slab(f, 12) for f in range(NA + U, 2 * NA)],
            "f2": [cp_slab(f, 13) for f in range(2 * NA, NF)],
        }
        queue = [ds for name in ("x23", "x456", "kv", "f0", "f1", "f2") for ds in batch[name]]

        def issue(n):
            for ds in queue[:n]:
                start(ds)
            del queue[:n]

        flying = []
        arrived = set()

        def start(ds):
            for d in ds:
                d.start()
                flying.append(d)

        def wait(ds, name):
            with scope(name):
                for d in ds:
                    assert any(d is e for e in flying)
                    flying[:] = [e for e in flying if e is not d]
                    d.wait()

        start(cp_small + cp_s[0] + cp_1)

        kv_v[...] = jnp.zeros_like(kv_v)
        z_v[...] = jnp.zeros_like(z_v)

        r128 = lax.broadcasted_iota(I32, (128, 128), 0)
        c128 = lax.broadcasted_iota(I32, (128, 128), 1)
        diag = (2 * ((r128 % 64) // 32) + r128 // 64) == (c128 // 32)
        er = lax.broadcasted_iota(I32, (128, 32), 0)
        ec = lax.broadcasted_iota(I32, (128, 32), 1)
        eye = jnp.where((er % 32) == ec, 1.0, 0.0).astype(BF16)
        wait(cp_small, "w_small")
        bd = {}

        def prep_phi(groups):
            for g in groups:
                wp = wphi_v[pl.ds(4 * g, 4)].reshape(128, 32)
                t = lax.dot_general(eye, wp, NT, preferred_element_type=F32)
                bd[g] = pltpu.bitcast(jnp.where(diag, t, 0.0).astype(BF16), I32)

        prep_phi(range(2))
        gw = gw_v[...].astype(F32).reshape(1, D)
        wr = wr_v[...].astype(F32).reshape(1, D)

        never = lax.broadcasted_iota(I32, (8, 128), 0) > (pltpu.bitcast(gw[:, 0:128], I32) & 0xFFFF) + 8
        clock = []

        def after(w, dep, every=False):
            if dep is None:
                return w
            dep = pltpu.bitcast(dep, w.dtype)
            if every:
                return jnp.concatenate([jnp.concatenate(
                    [jnp.where(never, dep, w[r:r + 8, c:c + 128]) for c in range(0, w.shape[1], 128)], axis=1)
                    for r in range(0, w.shape[0], 8)], axis=0)
            w0 = jnp.where(never, dep, w[0:8, 0:128])
            if w.shape[1] > 128:
                w0 = jnp.concatenate([w0, w[0:8, 128:]], axis=1)
            return jnp.concatenate([w0, w[8:]], axis=0) if w.shape[0] > 8 else w0

        def now(back=1, row=0):
            if not back or len(clock) < back:
                return None
            t = clock[-back]
            row = row * 8 % t.shape[0]
            return t[row:row + 8, 0:128]

        due = {}

        def before(v, ahead):
            if ahead is None:
                return
            v = pltpu.bitcast(v, I32)
            parts = [v[r:r + 8, c:c + 128] for r in range(0, v.shape[0], 8) for c in range(0, v.shape[1], 128)]
            due.setdefault(len(clock) + ahead, []).append(_tree(parts, jnp.bitwise_or))

        def mm(w, rhs, dims):
            deps = due.pop(len(clock), [])
            if deps:
                w = after(w, _tree(deps, jnp.bitwise_or))
            t = lax.dot_general(_ld(w), rhs, dims, preferred_element_type=F32)
            clock.append(t)
            return t

        def fold(j, s):
            assert j == 0 or "kv" in arrived
            a, b = [mm(bd[g], _ld(w_v[j, :, g * 128:(g + 1) * 128]), NT) * LOG2E for g in (2 * s, 2 * s + 1)]
            for m, t in enumerate(_left(a[:, :K2], a[:, K2:], b[:, :K2], b[:, K2:])):
                w = _pack(t[0:64], t[64:128])
                wa_v[j, s, m] = w
                before(w, P["DK"] if j == 1 else None)

        def prep_w(j, ref, s):
            def job(c):
                def run():
                    assert ("kv" if j == 2 else "f1") in arrived
                    blocks = [pltpu.bitcast(_ld(after(ref[(k * U + c) * 64:(k * U + c + 1) * 64, g * 128:(g + 1) * 128],
                                                      now(P["WL"]))).T, I32)
                              for g in (2 * s, 2 * s + 1) for k in range(2)]
                    lo, hi = [_left(*[_unpack(w, e) for w in blocks]) for e in range(2)]
                    for m in range(7):
                        w = blocks[0] if m == 2 else blocks[3] if m == 3 else _pack(lo[m], hi[m])
                        wa_v[j, s, m, :, c * 128:(c + 1) * 128] = w
                        before(w, P["DW"] if m in SUMS else None)
                return run
            return [job(c) for c in range(U)]

        def xblk(i, t, k, c=None):
            cols = slice(k * K2, (k + 1) * K2) if c is None else slice(k * K2 + c * 128, k * K2 + (c + 1) * 128)
            return x_v[(2 * i + t) * 64:(2 * i + t + 1) * 64, cols]

        route = [jnp.full((1, 1), -jnp.inf, F32), jnp.zeros((1, 1), I32)]

        def prep_x(i):
            acc = {}

            def job(c):
                def run():
                    assert i < 2 or ("x23" if i < 4 else "x456" if i < 7 else "kv") in arrived
                    words = [after(xblk(i, 0, 0, c), now(P["XL"]), True), xblk(i, 1, 0, c),
                             xblk(i, 0, 1, c), after(xblk(i, 1, 1, c), now(P["XL"]), True)]
                    vals = [[_unpack(w, e) for w in words] for e in range(2)]
                    lo, hi = [_right(*v) for v in vals]
                    for m in range(7):
                        t = words[0] if m == 1 else words[3] if m == 4 else _pack(lo[m], hi[m])
                        w = pltpu.bitcast(_ld(t).T, I32)
                        xs_v[i, m, c * 64:(c + 1) * 64, :] = w
                        before(w[0:8], P["DX"] if i > 0 else None)
                    w1, w2 = wr[:, c * 128:(c + 1) * 128], wr[:, K2 + c * 128:K2 + (c + 1) * 128]
                    for t in range(2):
                        for e in range(2):
                            part = vals[e][t] * w1 + vals[e][2 + t] * w2
                            acc[t, e] = part if c == 0 else acc[t, e] + part
                    if c < U - 1:
                        return
                    for t in range(2):
                        rs, toks = [], []
                        for e in range(2):
                            r = jnp.sum(acc[t, e], axis=1, keepdims=True).astype(BF16).astype(F32)
                            rs.append(jnp.where(r != r, -jnp.inf, r))
                            toks.append(i * T + t * 128 + e + 2 * lax.broadcasted_iota(I32, (64, 1), 0))
                        top = jnp.max(jnp.maximum(*rs), axis=0, keepdims=True)
                        arg = jnp.min(jnp.minimum(*[jnp.where(r == top, k, S) for r, k in zip(rs, toks)]),
                                      axis=0, keepdims=True)
                        better = top > route[0]
                        route[1] = jnp.where(better, arg, route[1])
                        route[0] = jnp.where(better, top, route[0])
                return run
            return [job(c) for c in range(U)]

        def gates(i):
            def job(t, r0):
                def run():
                    lo = (i * T + t * 128 + r0) // 2
                    xs = _ld(after(x_v[lo:lo + 32, :], now(P["GL"]))).astype(F32)
                    gs = jnp.sum(xs * gw, axis=1, keepdims=True)
                    gate = jnp.broadcast_to(jax.nn.sigmoid(gs), (64, 128))
                    gate_v[i, t, r0:r0 + 64, :] = gate
                    before(gate, P["DG"])
                return run
            return [job(t, r0) for t in range(2) for r0 in (0, 64)]

        def x_op(i, m):
            return xs_v[i, m]

        def proj(j, i, s, jobs):
            ops = [x_op(i, m) for m in range(7)]
            return _combine(lambda m: mm(wa_v[j, s, m], _ld(ops[m]), NN), jobs)

        held = []

        def phi_q(i, s, ps):
            def job(e, q):
                def run():
                    for t in range(2):
                        held.append(((i, 2 * s + e, slice(q * 64, (q + 1) * 64), slice(t * 128, (t + 1) * 128)),
                                     _pack(*_phi(ps[e][t][q * 64:(q + 1) * 64],
                                                 lambda v, k: after(v, now(P["QL"], P["QR"][t][k]))))))
                        before(held[-1][1], P["DQ"])
                    if i < NTILE - 1:
                        store_held()
                return run
            return [job(e, q) for e in range(2) for q in range(2)]

        def store_held():
            while held:
                where, val = held.pop(0)
                pq_v[where] = val

        def at(slots, jobs):
            return list(zip(slots, jobs))

        wait(cp_s[0], "w_q0")
        start(cp_s[1])
        fold(0, 0)
        wait(cp_1, "w_x0")
        start(cp_s[2])
        for fn in prep_x(0):
            fn()
        pend = []

        def sync(name):
            def run():
                wait([d for ds in batch[name] for d in ds], "w_" + name)
                arrived.add(name)
            return [(P["HS"], run)]

        for i in range(NTILE - 1):
            px = prep_x(i + 1)
            for s in range(U):
                jobs = []
                if i == 0 and s > 0:
                    wait(cp_s[s] + (cp_2 if s == U - 1 else []), "w_q%d" % s)
                    start([cp_s[3], cp_2, []][s - 1])
                    if s == 1:
                        prep_phi(range(2, G))
                    fold(0, s)
                issue(P["IA"][i][s])
                for name, where in (("x23", (1, 2)), ("x456", (3, 0)), ("kv", (NTILE - 2, 0))):
                    if (i, s) == where:
                        jobs += sync(name)
                if i == 0:
                    jobs += at(P["HX4"], px) if s == U - 1 else []
                elif i == 1:
                    jobs += at(P["HX2"], px[2 * (s - 2):2 * (s - 1)]) if s >= 2 else []
                else:
                    jobs += at(P["HX6" if i == NTILE - 2 else "HX"], px[s:s + 1])
                if i == NTILE - 2:
                    jobs += at(P["HW"], prep_w(2, w_v.at[2], s))
                    jobs += at(P["HK"], [lambda s=s: fold(1, s)])
                pend = phi_q(i, s, proj(0, i, s, jobs + at(P["HA6" if i == NTILE - 2 else "HA"], pend)))

        idx = jnp.max(route[1])
        blk = _ld(x_v[pl.ds(pl.multiple_of((idx // 16) * 8, 8), 8), :]).astype(F32)
        sel = lax.broadcasted_iota(I32, (16, D), 0) == (idx % 16)
        xs = jnp.sum(jnp.where(sel, blk, 0.0), axis=0, keepdims=True)
        r_sel = jnp.sum(xs * wr, axis=1, keepdims=True)
        r_gate = jax.nn.sigmoid(r_sel.astype(BF16).astype(F32))

        def spread_token():
            for g in range(G):
                xb_v[g * 128:(g + 1) * 128, :] = after(
                    jnp.broadcast_to(xs[:, g * 128:(g + 1) * 128], (128, 128)), now()).T

        ffn = {"y": [jnp.zeros((8, K2), F32)] * 2}

        def ffn_jobs(f):
            def up(k):
                def run():
                    assert "f%d" % (f // NA) in arrived
                    xb = after(xb_v[k * 256:(k + 1) * 256, :], now(P["FL"]))
                    for name, w_ref in (("g", wg_v), ("u", wu_v)):
                        w = _ld(w_ref[k * 128:(k + 1) * 128, f * 128:(f + 1) * 128]).astype(F32)
                        t = jnp.sum((w * xb).reshape(32, 8, 128), axis=0)
                        ffn[name] = t if k == 0 else ffn[name] + t
                        before(ffn[name], P["DF"])
                    if k == 3:
                        g, u = [jnp.sum(ffn[name], axis=0, keepdims=True) for name in "gu"]
                        ffn["h", f] = jnp.broadcast_to(g * jax.nn.sigmoid(g) * u, (128, 128)).T
                return run

            def down(n):
                def run():
                    assert "f%d" % ((f - 1) // NA) in arrived
                    w = _ld(wd_v[(f - 1) * 64:f * 64, n * K2:(n + 1) * K2]).astype(F32)
                    hb = jnp.concatenate([after(ffn["h", f - 1], now(P["FL"]))] * U, axis=1)
                    ffn["y"][n] = ffn["y"][n] + jnp.sum((w * hb).reshape(16, 8, K2), axis=0)
                    before(ffn["y"][n], P["DF"])
                return run

            return ([down(n) for n in range(2)] if 0 < f else []) + ([up(k) for k in range(4)] if f < NF else [])

        kr = lax.broadcasted_iota(I32, (64, 128), 0)
        kc = lax.broadcasted_iota(I32, (64, 128), 1)
        kmask = (kr // 32) == ((kc // 2) % 2)
        kvb = [None] * (H // 2)

        def kv_step(i, s, ps, vs):
            def job(e, q):
                def run():
                    g = 2 * s + e
                    j = 2 * g + q
                    rows = slice(q * 64, (q + 1) * 64)
                    phis = [_phi(ps[e][t][rows], lambda v, k: after(v, now(P["KVL"], P["KR"][t][k]))) for t in range(2)]
                    zs = [z_v[g, sign, rows] + (phis[0][sign] + phis[1][sign]) for sign in range(2)]
                    phb = jnp.concatenate([_pack(*ph) for ph in phis], axis=1)
                    kv_v[j] += mm(vs[2 * e + q], _ld(phb), NT)
                    if i == NTILE - 1:
                        zs = [jnp.broadcast_to(jnp.sum(z, axis=1, keepdims=True), (64, 128)) for z in zs]
                        t = jnp.concatenate([kv_v[j, pl.ds(0, 32, stride=2), :], kv_v[j, pl.ds(1, 32, stride=2), :]],
                                            axis=0)
                        kvb[j] = pltpu.bitcast(jnp.where(kmask, t, 0.0).astype(BF16), I32)
                    for sign in range(2):
                        z_v[g, sign, rows] = zs[sign]
                return run
            return [job(e, q) for e in range(2) for q in range(2)]

        def tile(i):
            return idx // T if i == NTILE - 1 else i + (idx // T <= i).astype(I32)

        o_pairs, o_parts = {}, {}

        def attn(i, g):
            def pair(h, q):
                def run():
                    rows = slice(q * 64, (q + 1) * 64)
                    w = pq_v[tile(i), h, rows]
                    dn = (_unpack(w, 0) * jnp.concatenate([after(z_v[h, 0, rows], now(P["AL"]))] * 2, axis=1)
                          + _unpack(w, 1) * jnp.concatenate([z_v[h, 1, rows]] * 2, axis=1))
                    rden = 1.0 / (_red(dn.reshape(8, 8, T), jnp.add) + 1e-6)
                    num = mm(kvb[2 * h + q], _ld(w), NN)
                    o_pairs[i, h, q] = [num[0:32] * rden[0:1], num[32:64] * rden[1:2]]
                return run

            def join():
                a, b = [jnp.concatenate(o_pairs.pop((i, h, 0)) + o_pairs.pop((i, h, 1)), axis=0) for h in (g, g + U)]
                o_parts[i, g] = _right(a[:, :128], a[:, 128:], b[:, :128], b[:, 128:])
                for m in SUMS:
                    before(o_parts[i, g][m][0:8], P["DA"])

            return [pair(h, q) for h in (g, g + U) for q in range(2)] + [join]

        def o_ops(i):
            parts = [o_parts.pop((i, g)) for g in range(U)]
            return [jnp.concatenate([p[m] for p in parts], axis=0).astype(BF16) for m in range(7)]

        first = [attn(0, g) for g in range(U)]
        def finish_ffn():
            ffn["out"] = jnp.sum(jnp.concatenate(ffn["y"], axis=1), axis=0, keepdims=True) * r_gate

        rest = [(f, fn) for f in range(NF + 1) for fn in ffn_jobs(f)] + [(0, finish_ffn)]
        ready = [0]

        def take(n):
            got, rest[:] = rest[:n], rest[n:]
            assert all(min(f, NF - 1) < ready[0] for f, _ in got)
            return [fn for _, fn in got]

        HB = P["HB"]
        for i in range(NTILE):
            gj = gates(i)
            ready[0] = 2 * NA if i >= P["F1"] else NA if i >= F0 else 0
            for s in range(U):
                fj = take(P["QB"][i][s])
                if (i, s) == (0, 0):
                    fj = [spread_token]
                issue(2 if i == 0 and s % 2 == 0 else 1)
                vt = proj(2, i, s, (sync("f0") if (i, s) == (F0, 0) else sync("f1") if (i, s) == (P["F1"], 0) else [])
                          + at(HB[1], pend[:HB[0]]) + at(P["HF0"][6 - max(len(fj), 3):], fj[:-3]) + at(P["HG"], gj[s:s + 1]))
                vts = [jnp.concatenate([_pack(b[q * 64:q * 64 + 32], b[q * 64 + 32:q * 64 + 64]) for b in vt[e]], axis=1)
                       for e in range(2) for q in range(2)]
                jobs = at(HB[2], pend[HB[0]:]) + at(P["HF1"], fj[-3:])
                if P["F1"] <= i < P["F1"] + 2:
                    jobs += at(P["HO"], prep_w(3, wo_v, (i - P["F1"]) * 2 + s // 2)[2 * (s % 2):2 * (s % 2) + 2])
                if i == NTILE - 1 and s >= 2:
                    jobs += at(P["H0"], [first[g][n] for g in (2 * s - 4, 2 * s - 3) for n in range(2)])
                pend = kv_step(i, s, proj(1, i, s, jobs), vts)

        late = [[], [(0, 2), (0, 3), (0, 4), (1, 2), (1, 3), (1, 4)], [(2, 2), (2, 3), (2, 4)], [(3, 2), (3, 3), (3, 4)]]
        for s in range(U):
            jobs = at(P["HA7"], pend) + at(P["H1"][s], [first[g][n] for g, n in late[s]])
            pend = phi_q(NTILE - 1, s, proj(0, NTILE - 1, s, jobs))

        def cp_o(i, lo, n):
            return pltpu.make_async_copy(out_v.at[pl.ds(i * T, T), pl.ds(lo, n)],
                                         out_h.at[pl.ds(pl.multiple_of(tile(i) * T, T), T), pl.ds(lo, n)], sem.at[6])

        outs = []

        def mix(i, c, blocks):
            def job(n, t):
                def run():
                    r0, c0 = i * T + t * 128, (2 * c + n) * 128
                    g = gate_v[tile(i), t]
                    xt = _ld(x_v[pl.ds(pl.multiple_of(tile(i) * 128 + t * 64, 64), 64), c0:c0 + 128]).astype(F32)
                    upd = xt * 0.0
                    if i == NTILE - 1:
                        tok = t * 128 + lax.broadcasted_iota(I32, (128, 128), 0)
                        upd = upd + jnp.where(tok == idx % T, ffn["out"][:, c0:c0 + 128], 0.0)
                    a = after(blocks[n][t], now(P["ML"])).T
                    res = g * a + (1.0 - g) * (xt + upd)
                    out_v[r0:r0 + 128, c0:c0 + 128] = res.astype(BF16)
                    before(res, P["DM"])
                    if (n, t) != (1, 1):
                        return
                    if i == NTILE - 1:
                        new = [cp_o(i, c * 256, 256)]
                    else:
                        new = [cp_o(i, 0, D)] if c == U - 1 else []
                    start(new)
                    outs.extend(new)
                return run
            return [job(n, t) for n in range(2) for t in range(2)]

        for i in range(NTILE):
            ops = o_ops(i)
            assert i < NTILE - 1 or not rest
            aj = [fn for g in range(U) for fn in attn(i + 1, g)] if i + 1 < NTILE else []
            for c in range(U):
                jobs = at(P["HM"], pend) + [(n - 7 * c, fn) for n, fn in zip(P["HT"], aj) if n // 7 == c]
                if (i, c) == (1, 0):
                    store_held()
                if (i, c) == P["W7"]:
                    jobs = sync("f2") + jobs
                    ready[0] = NF
                fj = take(P["QC"][c])
                jobs += at(P["HC"], fj)
                pend = mix(i, c, _combine(lambda m: mm(wa_v[3, c, m], ops[m], NN), jobs))
        for fn in pend:
            fn()
        wait(outs, "w_out")
        assert not flying

    return kernel


DEFAULTS = dict(
    F0=2, F1=5, W7=(0, 0), NA=12, HS=1, PROF=False, FLAGS=None,
    IA=((0, 0, 0, 2), (0, 0, 1, 1), (1, 1, 1, 1), (1, 1, 1, 1), (1, 1, 1, 0), (1, 0, 1, 0), (1, 0, 1, 0)),
    QB=((0,) * 4, (0,) * 4, (4, 6, 6, 6)) + ((6,) * 4,) * 5, QC=(1, 1, 1, 1),
    HA=(0, 2, 4, 6), QL=2, DQ=7, XL=3, DX=7, HX=(2,), HX2=(3, 6), HX4=(1, 1, 4, 5), QR=((0, 4), (8, 12)),
    HA6=(0, 2, 4, 6), HX6=(1,), HW=(1, 2, 4, 6), HK=(2,), DK=None, DW=5, WL=1,
    HB=(2, (3, 6), (2, 5)), KVL=4, KR=((0, 4), (8, 12)), HG=(5,), DG=5, GL=1,
    HF0=(0, 2, 5), HF1=(1, 4, 6), DF=6, FL=1, HO=(0, 5), H0=(0, 1, 3, 6),
    H1=((), (0, 1, 2, 3, 5, 6), (1, 3, 5), (1, 3, 5)), HA7=(0, 2, 4, 6),
    HM=(0, 2, 4, 6), HT=(0, 2, 3, 3, 5, 5, 6, 7, 8, 10, 11, 11, 12, 13, 15, 15, 16, 17, 18, 21),
    HC=(6,), DM=4, ML=3, AL=1, DA=None,
)


def make(**kw):
    P = dict(DEFAULTS, **kw)

    @jax.jit
    def run(A_x, A_wqkv, A_w_phi, A_wo, B_x, B_w_r, B_w_gate, B_w_up, B_w_down, gate_w):
        B, S, D = A_x.shape
        F = B_w_gate.shape[1]
        H = A_w_phi.shape[0]
        NTILE = S // 256
        G = D // 128
        any_spec = pl.BlockSpec(memory_space=pl.ANY)
        V = pltpu.VMEM
        scratch = [
            V((S // 2, D), I32),
            V((NTILE, 7, D // 4, 128), I32),
            V((3, D // 2, D), I32),
            V((4, G // 2, 7, 64, D // 2), I32),
            V((H, 32, 32), BF16),
            V((D // 2, D), I32),
            V((D,), BF16),
            V((D,), BF16),
            V((D // 2, F), I32),
            V((D // 2, F), I32),
            V((F // 2, D), I32),
            V((NTILE, G, 128, 256), I32),
            V((NTILE, 2, 128, 128), F32),
            V((H // 2, 64, 128), F32),
            V((G, 2, 128, 128), F32),
            V((D, 128), F32),
            V((S, D), BF16),
            pltpu.SemaphoreType.DMA((14,)),
        ]
        out = pl.pallas_call(
            _make_kernel(S, D, F, H, P),
            out_shape=jax.ShapeDtypeStruct((S, D), A_x.dtype),
            in_specs=[any_spec] * 9,
            out_specs=any_spec,
            scratch_shapes=scratch,
            compiler_params=pltpu.CompilerParams(vmem_limit_bytes=110 * 2**20, flags=P["FLAGS"]),
        )(A_x.reshape(S, D), A_wqkv, A_w_phi, A_wo, B_w_r, B_w_gate, B_w_up, B_w_down, gate_w)
        return out.reshape(B, S, D)
    return run


_run = make()


@jax.jit
def pallas_gated_mix__linear_kernel_hedgehog__moe_arch_mod__prompt_kernel(
    A_x, A_wqkv, A_w_phi, A_wo, B_x, B_w_r, B_w_gate, B_w_up, B_w_down, gate_w
):
    return _run(A_x, A_wqkv, A_w_phi, A_wo, B_x, B_w_r, B_w_gate, B_w_up, B_w_down, gate_w)
```

```python
import contextlib

import jax
import jax.numpy as jnp
from jax import lax
import jax.experimental.pallas as pl
import jax.experimental.pallas.tpu as pltpu

F32 = jnp.float32
BF16 = jnp.bfloat16
I32 = jnp.int32
LOG2E = 1.4426950408889634
NT = (((1,), (1,)), ((), ()))
NN = (((1,), (0,)), ((), ()))


def _ld(v):
    return pltpu.bitcast(v, BF16)


def _pack(a, b):
    return pltpu.bitcast(pltpu.pack_elementwise([a, b], packed_dtype=BF16), I32)


def _unpack(w, k):
    return pltpu.unpack_elementwise(w, index=k, packed_dtype=BF16, unpacked_dtype=F32)


def _tree(vs, op):
    while len(vs) > 1:
        vs = [op(vs[k], vs[k + 1]) if k + 1 < len(vs) else vs[k] for k in range(0, len(vs), 2)]
    return vs[0]


def _left(a11, a12, a21, a22):
    return [a11 + a22, a21 + a22, a11, a22, a11 + a12, a21 - a11, a12 - a22]


def _right(b11, b12, b21, b22):
    return [b11 + b22, b11, b12 - b22, b21 - b11, b22, b11 + b12, b21 + b22]


def _combine(mul, jobs, early=lambda c11, c21: None):
    count = [0]

    def step(m):
        t = mul(m)
        for n, fn in jobs:
            if n == count[0]:
                fn()
        count[0] += 1
        return t

    m1 = step(0)
    c11 = m1 + step(6)
    c22 = m1 + step(5)
    m4 = step(3)
    c11 = c11 + m4
    m5 = step(4)
    c11 = c11 - m5
    m2 = step(1)
    c21 = m4 + m2
    early(c11, c21)
    c22 = c22 - m2
    m3 = step(2)
    return (c11, m5 + m3), (c21, c22 + m3)


def _red(v, op):
    r = _tree([v[k] for k in range(v.shape[0])], op)
    r = op(r, pltpu.roll(r, 4, 0))
    return op(r, pltpu.roll(r, 2, 0))


def _rcp(s):
    r = pl.reciprocal(s, approx=True)
    return r * (2.0 - s * r)


def _phi(p, tie):
    p = p.reshape(8, 8, 128)
    ep = jnp.exp2(p - tie(_red(p, jnp.maximum), 0))
    en = jnp.exp2(tie(_red(p, jnp.minimum), 1) - p)
    ep = ep * _rcp(_red(ep, jnp.add))
    en = en * _rcp(_red(en, jnp.add))
    return ep.reshape(64, 128), en.reshape(64, 128)


def _make_kernel(S, D, F, H, P):
    scope = jax.named_scope if P["PROF"] else (lambda n: contextlib.nullcontext())
    T = 256
    NTILE = S // T
    G = D // 128
    U = G // 2
    K2 = D // 2
    NF = F // 128
    F0 = P["F0"]
    NA = P["NA"]
    SUMS = (0, 2, 3, 5, 6)

    def kernel(ax_h, wqkv_h, wphi_h, wo_h, wr_h, wg_h, wu_h, wd_h, gw_h, out_h,
               x_v, xs_v, w_v, wa_v, wphi_v, wo_v, wr_v, gw_v, wg_v, wu_v, wd_v,
               pq_v, gate_v, kv_v, z_v, xb_v, out_v, sem):
        def cp_x(lo, hi, s):
            return pltpu.make_async_copy(ax_h.at[pl.ds(lo * T, (hi - lo) * T)],
                                         x_v.at[pl.ds(lo * T // 2, (hi - lo) * T // 2)].bitcast(BF16), sem.at[s])

        def cp_q(lo, hi, s):
            return pltpu.make_async_copy(wqkv_h.at[:, pl.ds(lo * 256, (hi - lo) * 256)],
                                         w_v.at[0, :, pl.ds(lo * 256, (hi - lo) * 256)].bitcast(BF16), sem.at[s])

        cp_small = [pltpu.make_async_copy(wr_h, wr_v, sem.at[0]), pltpu.make_async_copy(gw_h, gw_v, sem.at[0]),
                    pltpu.make_async_copy(wphi_h.at[0:8], wphi_v.at[0:8], sem.at[0])]
        def cp_rows(src, dst, n, s):
            return pltpu.make_async_copy(src.at[pl.ds(n * 256, 256)], dst.at[pl.ds(n * 128, 128)].bitcast(BF16), sem.at[s])

        def cp_slab(f, s):
            cols = pl.ds(f * 128, 128)
            return [pltpu.make_async_copy(wg_h.at[:, cols], wg_v.at[:, cols].bitcast(BF16), sem.at[s]),
                    pltpu.make_async_copy(wu_h.at[:, cols], wu_v.at[:, cols].bitcast(BF16), sem.at[s]),
                    pltpu.make_async_copy(wd_h.at[cols], wd_v.at[pl.ds(f * 64, 64)].bitcast(BF16), sem.at[s])]

        batch = {
            "q0": [[cp_q(0, 1, 8)]],
            "x0": [[cp_x(0, 1, 1)]],
            "q1": [[cp_q(1, 2, 9), pltpu.make_async_copy(wphi_h.at[8:H], wphi_v.at[8:H], sem.at[9])]],
            "x1": [[cp_x(1, 2, 2)]],
            "q2": [[cp_q(2, 4, 10)]],
            "x": [[cp_x(2, 5, 3)]],
            "kv": [[cp_x(i, i + 1, 4)] for i in (5, 6, 7)]
                  + [[cp_rows(wqkv_h.at[:, pl.ds(j * D, D)], w_v.at[j], n, 4)] for j in (2, 1) for n in range(U)],
            "f0": [cp_slab(f, 5) for f in range(NA)],
            "f1": [[cp_rows(wo_h, wo_v, n, 7)] + cp_slab(NA + n, 7) for n in range(U)]
                  + [cp_slab(f, 7) for f in range(NA + U, 2 * NA)],
            "f2": [cp_slab(f, 12) for f in range(2 * NA, NF)],
        }
        queue = [ds for name in batch for ds in batch[name]]

        def issue(n):
            for ds in queue[:n]:
                start(ds)
            del queue[:n]

        flying = []
        arrived = set()

        def start(ds):
            for d in ds:
                d.start()
                flying.append(d)

        def wait(ds, name):
            with scope(name):
                for d in ds:
                    assert any(d is e for e in flying)
                    flying[:] = [e for e in flying if e is not d]
                    d.wait()

        start(cp_small)
        issue(2)

        kv_v[...] = jnp.zeros_like(kv_v)
        z_v[...] = jnp.zeros_like(z_v)

        r128 = lax.broadcasted_iota(I32, (128, 128), 0)
        c128 = lax.broadcasted_iota(I32, (128, 128), 1)
        diag = (2 * ((r128 % 64) // 32) + r128 // 64) == (c128 // 32)
        er = lax.broadcasted_iota(I32, (128, 32), 0)
        ec = lax.broadcasted_iota(I32, (128, 32), 1)
        eye = jnp.where((er % 32) == ec, 1.0, 0.0).astype(BF16)
        wait(cp_small, "w_small")
        bd = {}

        def prep_phi(groups):
            for g in groups:
                wp = wphi_v[pl.ds(4 * g, 4)].reshape(128, 32)
                t = lax.dot_general(eye, wp, NT, preferred_element_type=F32)
                bd[g] = pltpu.bitcast(jnp.where(diag, t, 0.0).astype(BF16), I32)

        prep_phi(range(2))
        gw = gw_v[...].astype(F32).reshape(1, D)
        wr = wr_v[...].astype(F32).reshape(1, D)

        never = lax.broadcasted_iota(I32, (8, 128), 0) > (pltpu.bitcast(gw[:, 0:128], I32) & 0xFFFF) + 8
        clock = []

        def after(w, dep, every=False):
            if dep is None:
                return w
            dep = pltpu.bitcast(dep, w.dtype)
            if every:
                return jnp.concatenate([jnp.concatenate(
                    [jnp.where(never, dep, w[r:r + 8, c:c + 128]) for c in range(0, w.shape[1], 128)], axis=1)
                    for r in range(0, w.shape[0], 8)], axis=0)
            w0 = jnp.where(never, dep, w[0:8, 0:128])
            if w.shape[1] > 128:
                w0 = jnp.concatenate([w0, w[0:8, 128:]], axis=1)
            return jnp.concatenate([w0, w[8:]], axis=0) if w.shape[0] > 8 else w0

        def now(back=1, row=0):
            if not back or len(clock) < back:
                return None
            t = clock[-back]
            row = row * 8 % t.shape[0]
            return t[row:row + 8, 0:128]

        due = {}

        def before(v, ahead):
            if ahead is None:
                return
            v = pltpu.bitcast(v, I32)
            parts = [v[r:r + 8, c:c + 128] for r in range(0, v.shape[0], 8) for c in range(0, v.shape[1], 128)]
            due.setdefault(len(clock) + ahead, []).append(_tree(parts, jnp.bitwise_or))

        def mm(w, rhs, dims):
            deps = due.pop(len(clock), [])
            if deps:
                w = after(w, _tree(deps, jnp.bitwise_or))
            t = lax.dot_general(_ld(w), rhs, dims, preferred_element_type=F32)
            clock.append(t)
            return t

        def fold(j, s):
            assert j == 0 or "kv" in arrived
            a, b = [mm(bd[g], _ld(w_v[j, :, g * 128:(g + 1) * 128]), NT) * LOG2E for g in (2 * s, 2 * s + 1)]
            for m, t in enumerate(_left(a[:, :K2], a[:, K2:], b[:, :K2], b[:, K2:])):
                w = _pack(t[0:64], t[64:128])
                wa_v[j, s, m] = w
                before(w, P["DK"] if j == 1 else None)

        def prep_w(j, ref, s):
            def job(c):
                def run():
                    assert ("kv" if j == 2 else "f1") in arrived
                    blocks = [pltpu.bitcast(_ld(after(ref[(k * U + c) * 64:(k * U + c + 1) * 64, g * 128:(g + 1) * 128],
                                                      now(P["WL"]))).T, I32)
                              for g in (2 * s, 2 * s + 1) for k in range(2)]
                    lo, hi = [_left(*[_unpack(w, e) for w in blocks]) for e in range(2)]
                    for m in range(7):
                        w = blocks[0] if m == 2 else blocks[3] if m == 3 else _pack(lo[m], hi[m])
                        wa_v[j, s, m, :, c * 128:(c + 1) * 128] = w
                        before(w, P["DW"] if m in SUMS else None)
                return run
            return [job(c) for c in range(U)]

        def xblk(i, t, k, c=None):
            cols = slice(k * K2, (k + 1) * K2) if c is None else slice(k * K2 + c * 128, k * K2 + (c + 1) * 128)
            return x_v[(2 * i + t) * 64:(2 * i + t + 1) * 64, cols]

        route = [jnp.full((1, 1), -jnp.inf, F32), jnp.zeros((1, 1), I32)]

        def prep_x(i):
            acc = {}

            def job(c):
                def run():
                    assert ("x%d" % i if i < 2 else "x" if i < 5 else "kv") in arrived
                    words = [after(xblk(i, 0, 0, c), now(P["XL"]), True), xblk(i, 1, 0, c),
                             xblk(i, 0, 1, c), after(xblk(i, 1, 1, c), now(P["XL"]), True)]
                    vals = [[_unpack(w, e) for w in words] for e in range(2)]
                    lo, hi = [_right(*v) for v in vals]
                    for m in range(7):
                        t = words[0] if m == 1 else words[3] if m == 4 else _pack(lo[m], hi[m])
                        w = pltpu.bitcast(_ld(t).T, I32)
                        xs_v[i, m, c * 64:(c + 1) * 64, :] = w
                        before(w[0:8], P["DX"] if i > 0 else None)
                    w1, w2 = wr[:, c * 128:(c + 1) * 128], wr[:, K2 + c * 128:K2 + (c + 1) * 128]
                    for t in range(2):
                        for e in range(2):
                            part = vals[e][t] * w1 + vals[e][2 + t] * w2
                            acc[t, e] = part if c == 0 else acc[t, e] + part
                    if c < U - 1:
                        return
                    for t in range(2):
                        rs, toks = [], []
                        for e in range(2):
                            r = jnp.sum(acc[t, e], axis=1, keepdims=True).astype(BF16).astype(F32)
                            rs.append(jnp.where(r != r, -jnp.inf, r))
                            toks.append(i * T + t * 128 + e + 2 * lax.broadcasted_iota(I32, (64, 1), 0))
                        top = jnp.max(jnp.maximum(*rs), axis=0, keepdims=True)
                        arg = jnp.min(jnp.minimum(*[jnp.where(r == top, k, S) for r, k in zip(rs, toks)]),
                                      axis=0, keepdims=True)
                        better = top > route[0]
                        route[1] = jnp.where(better, arg, route[1])
                        route[0] = jnp.where(better, top, route[0])
                return run
            return [job(c) for c in range(U)]

        def gates(i):
            def job(t, r0):
                def run():
                    lo = (i * T + t * 128 + r0) // 2
                    xs = _ld(after(x_v[lo:lo + 32, :], now(P["GL"]))).astype(F32)
                    gs = jnp.sum(xs * gw, axis=1, keepdims=True)
                    gate = jnp.broadcast_to(jax.nn.sigmoid(gs), (64, 128))
                    gate_v[i, t, r0:r0 + 64, :] = gate
                    before(gate, P["DG"])
                return run
            return [job(t, r0) for t in range(2) for r0 in (0, 64)]

        def x_op(i, m):
            return xs_v[i, m]

        def proj(j, i, s, jobs):
            ops = [x_op(i, m) for m in range(7)]
            return _combine(lambda m: mm(wa_v[j, s, m], _ld(ops[m]), NN), jobs)

        held = []

        def phi_q(i, s, ps):
            def job(e, q):
                def run():
                    for t in range(2):
                        held.append(((i, 2 * s + e, slice(q * 64, (q + 1) * 64), slice(t * 128, (t + 1) * 128)),
                                     _pack(*_phi(ps[e][t][q * 64:(q + 1) * 64],
                                                 lambda v, k: after(v, now(P["QL"], P["QR"][t][k]))))))
                        before(held[-1][1], P["DQ"])
                    if i < NTILE - 1:
                        store_held()
                return run
            return [job(e, q) for e in range(2) for q in range(2)]

        def store_held():
            while held:
                where, val = held.pop(0)
                pq_v[where] = val

        def at(slots, jobs):
            return list(zip(slots, jobs))

        def arrive(name):
            wait([d for ds in batch[name] for d in ds], "w_" + name)
            arrived.add(name)

        def sync(name, then=0, slot=None):
            def run():
                arrive(name)
                issue(then)
            return [(P["HS"] if slot is None else slot, run)]

        arrive("q0")
        issue(1)
        fold(0, 0)
        arrive("x0")
        issue(1)
        for fn in prep_x(0):
            fn()
        pend = []
        pv = [fn for s in range(U) for fn in prep_w(2, w_v.at[2], s)]
        px = [prep_x(i) for i in range(NTILE)]
        order = [(0, 0), (0, 1), (1, 0), (1, 1), (0, 2), (1, 2), (0, 3), (1, 3)]
        order += [(i, s) for i in range(2, NTILE - 1) for s in range(U)]
        for n, (i, s) in enumerate(order):
            jobs = []
            if n == 1:
                arrive("q1")
                issue(1)
                prep_phi(range(2, G))
                fold(0, 1)
                jobs += sync("x1", 1, P["HS1"]) + at(P["HX1"], px[1])
            if n == 4:
                arrive("q2")
                issue(1)
                fold(0, 2)
                jobs += at(P["HK0"], [lambda: fold(0, 3)])
            if n > 4:
                issue(P["IA"][n - 5])
            if n == 7:
                jobs += sync("x") + at(P["HX4"], px[2])
            if n >= 8:
                if (i, s) == (4, 2):
                    jobs += sync("kv")
                if i == 4:
                    jobs += at(P["HX2"], px[5][2 * (s - 2):2 * (s - 1)]) if s >= 2 else []
                else:
                    jobs += at(P["HX6" if i > 4 else "HX"], px[i + 1][s:s + 1])
                k = P["QW"].get(i, (0,) * U)[s]
                jobs += at(P["HW"][:k], pv[:k])
                del pv[:k]
                if (i, s) in P["SK"]:
                    jobs += at(P["HK"], [lambda i=i, s=s: fold(1, P["SK"].index((i, s)))])
            pend = phi_q(i, s, proj(0, i, s, jobs + at(P["HA6" if i > 4 else "HA"], pend)))

        assert not pv
        idx = jnp.clip(jnp.max(route[1]), 0, S - 1)
        blk = _ld(x_v[pl.ds(pl.multiple_of((idx // 16) * 8, 8), 8), :]).astype(F32)
        sel = lax.broadcasted_iota(I32, (16, D), 0) == (idx % 16)
        xs = jnp.sum(jnp.where(sel, blk, 0.0), axis=0, keepdims=True)
        r_sel = jnp.sum(xs * wr, axis=1, keepdims=True)
        r_gate = jax.nn.sigmoid(r_sel.astype(BF16).astype(F32))

        def spread_token():
            for g in range(G):
                xb_v[g * 128:(g + 1) * 128, :] = after(
                    jnp.broadcast_to(xs[:, g * 128:(g + 1) * 128], (128, 128)), now()).T

        ffn = {"y": [jnp.zeros((8, K2), F32)] * 2}

        def ffn_jobs(f):
            def up(k):
                def run():
                    assert "f%d" % (f // NA) in arrived
                    xb = after(xb_v[k * 256:(k + 1) * 256, :], now(P["FL"]))
                    for name, w_ref in (("g", wg_v), ("u", wu_v)):
                        w = _ld(w_ref[k * 128:(k + 1) * 128, f * 128:(f + 1) * 128]).astype(F32)
                        t = jnp.sum((w * xb).reshape(32, 8, 128), axis=0)
                        ffn[name] = t if k == 0 else ffn[name] + t
                        before(ffn[name], P["DF"])
                    if k == 3:
                        g, u = [jnp.sum(ffn[name], axis=0, keepdims=True) for name in "gu"]
                        ffn["h", f] = jnp.broadcast_to(g * jax.nn.sigmoid(g) * u, (128, 128)).T
                return run

            def down(n):
                def run():
                    assert "f%d" % ((f - 1) // NA) in arrived
                    w = _ld(wd_v[(f - 1) * 64:f * 64, n * K2:(n + 1) * K2]).astype(F32)
                    hb = jnp.concatenate([after(ffn["h", f - 1], now(P["FL"]))] * U, axis=1)
                    ffn["y"][n] = ffn["y"][n] + jnp.sum((w * hb).reshape(16, 8, K2), axis=0)
                    before(ffn["y"][n], P["DF"])
                return run

            return ([down(n) for n in range(2)] if 0 < f else []) + ([up(k) for k in range(4)] if f < NF else [])

        kr = lax.broadcasted_iota(I32, (64, 128), 0)
        kc = lax.broadcasted_iota(I32, (64, 128), 1)
        kmask = (kr // 32) == ((kc // 2) % 2)
        kvb = [None] * (H // 2)

        def kv_step(i, s, ps, vs):
            def job(e, q):
                def run():
                    g = 2 * s + e
                    j = 2 * g + q
                    rows = slice(q * 64, (q + 1) * 64)
                    phis = [_phi(ps[e][t][rows], lambda v, k: after(v, now(P["KVL"], P["KR"][t][k]))) for t in range(2)]
                    zs = [z_v[g, sign, rows] + (phis[0][sign] + phis[1][sign]) for sign in range(2)]
                    phb = jnp.concatenate([_pack(*ph) for ph in phis], axis=1)
                    kv_v[j] += mm(vs[2 * e + q], _ld(phb), NT)
                    if i == NTILE - 1:
                        zs = [jnp.broadcast_to(jnp.sum(z, axis=1, keepdims=True), (64, 128)) for z in zs]
                        t = jnp.concatenate([kv_v[j, pl.ds(0, 32, stride=2), :], kv_v[j, pl.ds(1, 32, stride=2), :]],
                                            axis=0)
                        kvb[j] = pltpu.bitcast(jnp.where(kmask, t, 0.0).astype(BF16), I32)
                    for sign in range(2):
                        z_v[g, sign, rows] = zs[sign]
                return run
            return [job(e, q) for e in range(2) for q in range(2)]

        def tile(i):
            return idx // T if i == NTILE - 1 else i + (idx // T <= i).astype(I32)

        o_pairs, o_parts = {}, {}

        def attn(i, g):
            def pair(h, q):
                def run():
                    rows = slice(q * 64, (q + 1) * 64)
                    w = pq_v[tile(i), h, rows]
                    dn = (_unpack(w, 0) * jnp.concatenate([after(z_v[h, 0, rows], now(P["AL"], P["AR"][q]))] * 2, axis=1)
                          + _unpack(w, 1) * jnp.concatenate([z_v[h, 1, rows]] * 2, axis=1))
                    rden = 1.0 / (_red(dn.reshape(8, 8, T), jnp.add) + 1e-6)
                    num = mm(kvb[2 * h + q], _ld(w), NN)
                    o_pairs[i, h, q] = [num[0:32] * rden[0:1], num[32:64] * rden[1:2]]
                return run

            def join():
                a, b = [jnp.concatenate(o_pairs.pop((i, h, 0)) + o_pairs.pop((i, h, 1)), axis=0) for h in (g, g + U)]
                o_parts[i, g] = _right(a[:, :128], a[:, 128:], b[:, :128], b[:, 128:])
                for m in SUMS:
                    before(o_parts[i, g][m][0:8], P["DA"])

            return [pair(h, q) for h in (g, g + U) for q in range(2)] + [join]

        def o_ops(i):
            parts = [o_parts.pop((i, g)) for g in range(U)]
            return [jnp.concatenate([p[m] for p in parts], axis=0).astype(BF16) for m in range(7)]

        first = [attn(0, g) for g in range(U)]
        def finish_ffn():
            ffn["out"] = jnp.sum(jnp.concatenate(ffn["y"], axis=1), axis=0, keepdims=True) * r_gate

        rest = [(f, fn) for f in range(NF + 1) for fn in ffn_jobs(f)] + [(0, finish_ffn)]
        ready = [0]

        def take(n):
            got, rest[:] = rest[:n], rest[n:]
            assert all(min(f, NF - 1) < ready[0] for f, _ in got)
            return [fn for _, fn in got]

        HB = P["HB"]
        for i in range(NTILE):
            gj = gates(i)
            ready[0] = 2 * NA if i >= P["F1"] else NA if i >= F0 else 0
            for s in range(U):
                fj = take(P["QB"][i][s])
                if (i, s) == (0, 0):
                    fj = [spread_token]
                issue(P["IB"][i][s])
                vt = proj(2, i, s, (sync("f0") if (i, s) == (F0, 0) else sync("f1") if (i, s) == (P["F1"], 0) else [])
                          + at(HB[1], pend[:HB[0]]) + at(sorted(P["HF0"][len(fj) // 2 * -1:]), fj[:len(fj) // 2]) + at(P["HG"], gj[s:s + 1]))
                vts = [jnp.concatenate([_pack(b[q * 64:q * 64 + 32], b[q * 64 + 32:q * 64 + 64]) for b in vt[e]], axis=1)
                       for e in range(2) for q in range(2)]
                jobs = at(HB[2], pend[HB[0]:]) + at(sorted(P["HF1"][:(len(fj) + 1) // 2]), fj[len(fj) // 2:])
                if P["F1"] <= i < P["F1"] + 2:
                    jobs += at(P["HO"], prep_w(3, wo_v, (i - P["F1"]) * 2 + s // 2)[2 * (s % 2):2 * (s % 2) + 2])
                if i == NTILE - 1 and s >= 2:
                    jobs += at(P["H0"], [first[g][n] for g in (2 * s - 4, 2 * s - 3) for n in range(2)])
                pend = kv_step(i, s, proj(1, i, s, jobs), vts)

        late = [[], [(0, 2), (0, 3), (0, 4), (1, 2), (1, 3), (1, 4)], [(2, 2), (2, 3), (2, 4)], [(3, 2), (3, 3), (3, 4)]]
        for s in range(U):
            jobs = at(P["HA7"], pend) + at(P["H1"][s], [first[g][n] for g, n in late[s]])
            pend = phi_q(NTILE - 1, s, proj(0, NTILE - 1, s, jobs))

        def cp_o(i, r0, nr, c0, nc):
            rows = pl.ds(pl.multiple_of(tile(i) * T + r0, 128), nr)
            return pltpu.make_async_copy(out_v.at[pl.ds(i * T + r0, nr), pl.ds(c0, nc)],
                                         out_h.at[rows, pl.ds(c0, nc)], sem.at[6])

        outs = []

        def mix(i, c, blocks):
            def job(n, t):
                def run():
                    r0, c0 = i * T + t * 128, (2 * c + n) * 128
                    g = gate_v[tile(i), t]
                    xt = _ld(x_v[pl.ds(pl.multiple_of(tile(i) * 128 + t * 64, 64), 64), c0:c0 + 128]).astype(F32)
                    upd = xt * 0.0
                    if i == NTILE - 1:
                        tok = t * 128 + lax.broadcasted_iota(I32, (128, 128), 0)
                        upd = upd + jnp.where(tok == idx % T, ffn["out"][:, c0:c0 + 128], 0.0)
                    a = after(blocks[n][t], now(P["ML"], P["MR"][2 * t + n])).T
                    res = g * a + (1.0 - g) * (xt + upd)
                    out_v[r0:r0 + 128, c0:c0 + 128] = res.astype(BF16)
                    before(res, P["DM"])
                    if i == NTILE - 1:
                        new = [cp_o(i, t * 128, 128, c * 256, 256)] if n == 1 else []
                    else:
                        new = [cp_o(i, 0, T, 0, D)] if (c, n, t) == (U - 1, 1, 1) else []
                    start(new)
                    outs.extend(new)
                return run
            return [job(n, t) for t in range(2) for n in range(2)]

        for i in range(NTILE):
            ops = o_ops(i)
            assert i < NTILE - 1 or not rest
            aj = [fn for g in range(U) for fn in attn(i + 1, g)] if i + 1 < NTILE else []
            for c in range(U):
                jobs = at(P["HM"], pend) + [(n - 7 * c, fn) for n, fn in zip(P["HT"], aj) if n // 7 == c]
                if (i, c) == (1, 0):
                    store_held()
                if (i, c) == P["W7"]:
                    jobs = sync("f2") + jobs
                    ready[0] = NF
                fj = take(P["QC"][c])
                jobs += at(P["HC"][-len(fj):], fj)
                if (i, c) == (NTILE - 1, U - 1):
                    def early(c11, c21):
                        for fn in mix(i, c, ((c11, None), (c21, None)))[:2]:
                            fn()
                    pend = mix(i, c, _combine(lambda m: mm(wa_v[3, c, m], ops[m], NN), jobs, early))[2:]
                else:
                    pend = mix(i, c, _combine(lambda m: mm(wa_v[3, c, m], ops[m], NN), jobs))
        for fn in pend:
            fn()
        wait(outs, "w_out")
        assert not flying

    return kernel


DEFAULTS = dict(
    F0=2, F1=5, NA=12, W7=(0, 0), HS=1, PROF=False, FLAGS=None,
    HS1=2, HX1=(2, 3, 4, 5), HK0=(2,),
    IA=(0, 1, 1) + (1, 1, 1, 1) + (1, 1, 1, 1) + (1, 0, 1, 0) + (1, 0, 1, 0) + (1, 0, 1, 0),
    IB=((1, 1, 2, 1),) + ((1, 1, 1, 1),) * 7,
    QB=((0,) * 4, (0,) * 4, (4, 6, 6, 6)) + ((6,) * 4,) * 5, QC=(1, 1, 1, 1),
    QW={5: (2, 2, 2, 2), 6: (2, 2, 2, 2)}, SK=((5, 1), (5, 3), (6, 1), (6, 3)),
    HA=(0, 2, 4, 6), QL=2, DQ=7, XL=3, DX=7, HX=(2,), HX2=(3, 6), HX4=(1, 2, 4, 5), QR=((0, 4), (8, 12)),
    HA6=(0, 2, 4, 6), HX6=(1,), HW=(1, 5), HK=(2,), DK=None, DW=5, WL=1,
    HB=(2, (3, 6), (2, 5)), KVL=4, KR=((0, 4), (8, 12)), HG=(5,), DG=5, GL=1,
    HF0=(0, 2, 5), HF1=(1, 4, 6), DF=6, FL=1, HO=(0, 5), H0=(0, 1, 3, 6),
    H1=((), (0, 1, 2, 3, 5, 6), (1, 3, 5), (1, 3, 5)), HA7=(0, 2, 4, 6),
    HM=(0, 2, 4, 6), HT=(0, 2, 3, 3, 5, 5, 6, 7, 8, 10, 11, 11, 12, 13, 15, 15, 16, 17, 18, 21),
    HC=(6,), DM=4, ML=3, AL=1, DA=None, MR=(0, 0, 0, 0), AR=(0, 0),
)


def make(**kw):
    P = dict(DEFAULTS, **kw)

    @jax.jit
    def run(A_x, A_wqkv, A_w_phi, A_wo, B_x, B_w_r, B_w_gate, B_w_up, B_w_down, gate_w):
        B, S, D = A_x.shape
        F = B_w_gate.shape[1]
        H = A_w_phi.shape[0]
        NTILE = S // 256
        G = D // 128
        any_spec = pl.BlockSpec(memory_space=pl.ANY)
        V = pltpu.VMEM
        scratch = [
            V((S // 2, D), I32),
            V((NTILE, 7, D // 4, 128), I32),
            V((3, D // 2, D), I32),
            V((4, G // 2, 7, 64, D // 2), I32),
            V((H, 32, 32), BF16),
            V((D // 2, D), I32),
            V((D,), BF16),
            V((D,), BF16),
            V((D // 2, F), I32),
            V((D // 2, F), I32),
            V((F // 2, D), I32),
            V((NTILE, G, 128, 256), I32),
            V((NTILE, 2, 128, 128), F32),
            V((H // 2, 64, 128), F32),
            V((G, 2, 128, 128), F32),
            V((D, 128), F32),
            V((S, D), BF16),
            pltpu.SemaphoreType.DMA((13,)),
        ]
        out = pl.pallas_call(
            _make_kernel(S, D, F, H, P),
            out_shape=jax.ShapeDtypeStruct((S, D), A_x.dtype),
            in_specs=[any_spec] * 9,
            out_specs=any_spec,
            scratch_shapes=scratch,
            compiler_params=pltpu.CompilerParams(vmem_limit_bytes=110 * 2**20, flags=P["FLAGS"]),
        )(A_x.reshape(S, D), A_wqkv, A_w_phi, A_wo, B_w_r, B_w_gate, B_w_up, B_w_down, gate_w)
        return out.reshape(B, S, D)
    return run


_run = make()


@jax.jit
def pallas_gated_mix__linear_kernel_hedgehog__moe_arch_mod__prompt_kernel(
    A_x, A_wqkv, A_w_phi, A_wo, B_x, B_w_r, B_w_gate, B_w_up, B_w_down, gate_w
):
    return _run(A_x, A_wqkv, A_w_phi, A_wo, B_x, B_w_r, B_w_gate, B_w_up, B_w_down, gate_w)
```

```python
import contextlib

import jax
import jax.numpy as jnp
from jax import lax
import jax.experimental.pallas as pl
import jax.experimental.pallas.tpu as pltpu

F32 = jnp.float32
BF16 = jnp.bfloat16
I32 = jnp.int32
LOG2E = 1.4426950408889634
NT = (((1,), (1,)), ((), ()))
NN = (((1,), (0,)), ((), ()))


def _ld(v):
    return pltpu.bitcast(v, BF16)


def _pack(a, b):
    return pltpu.bitcast(pltpu.pack_elementwise([a, b], packed_dtype=BF16), I32)


def _unpack(w, k):
    return pltpu.unpack_elementwise(w, index=k, packed_dtype=BF16, unpacked_dtype=F32)


def _tree(vs, op):
    while len(vs) > 1:
        vs = [op(vs[k], vs[k + 1]) if k + 1 < len(vs) else vs[k] for k in range(0, len(vs), 2)]
    return vs[0]


def _left(a11, a12, a21, a22):
    return [a11 + a22, a21 + a22, a11, a22, a11 + a12, a21 - a11, a12 - a22]


def _right(b11, b12, b21, b22):
    return [b11 + b22, b11, b12 - b22, b21 - b11, b22, b11 + b12, b21 + b22]


_USES = (((0, 1), (3, 1)), ((2, 1), (3, -1)), ((1, 1), (3, 1)), ((0, 1), (2, 1)),
         ((0, -1), (1, 1)), ((3, 1),), ((0, 1),))


def _combine(mul, jobs, order=(0, 6, 5, 3, 4, 1, 2), early=None):
    c = [None] * 4
    for n, m in enumerate(order):
        if early and n == 6:
            early(c[0], c[2])
        t = mul(m)
        for k, sign in _USES[m]:
            if c[k] is None:
                c[k] = t if sign > 0 else -t
            else:
                c[k] = c[k] + t if sign > 0 else c[k] - t
        for at, fn in jobs:
            if at == n:
                fn()
    return (c[0], c[1]), (c[2], c[3])


def _red(v, op):
    r = _tree([v[k] for k in range(v.shape[0])], op)
    r = op(r, pltpu.roll(r, 4, 0))
    return op(r, pltpu.roll(r, 2, 0))


def _rcp(s):
    r = pl.reciprocal(s, approx=True)
    return r * (2.0 - s * r)


def _phi(p, tie):
    p = p.reshape(8, 8, 128)
    ep = jnp.exp2(p - tie(_red(p, jnp.maximum), 0))
    en = jnp.exp2(tie(_red(p, jnp.minimum), 1) - p)
    ep = ep * _rcp(_red(ep, jnp.add))
    en = en * _rcp(_red(en, jnp.add))
    return ep.reshape(64, 128), en.reshape(64, 128)


def _make_kernel(S, D, F, H, P):
    scope = jax.named_scope if P["PROF"] else (lambda n: contextlib.nullcontext())
    T = 256
    NTILE = S // T
    G = D // 128
    U = G // 2
    K2 = D // 2
    NF = F // 128
    F0 = P["F0"]
    NA = P["NA"]
    SUMS = (0, 2, 3, 5, 6)

    def kernel(ax_h, wqkv_h, wphi_h, wo_h, wr_h, wg_h, wu_h, wd_h, gw_h, out_h,
               x_v, xs_v, w_v, wa_v, wphi_v, wo_v, wr_v, gw_v, wg_v, wu_v, wd_v,
               pq_v, gate_v, kv_v, z_v, xb_v, out_v, sem):
        def cp_x(lo, hi, s, n=1):
            step = (hi - lo) * T // n
            return [pltpu.make_async_copy(ax_h.at[pl.ds(r, step)], x_v.at[pl.ds(r // 2, step // 2)].bitcast(BF16), sem.at[s])
                    for r in range(lo * T, hi * T, step)]

        def cp_q(u, s, n=1):
            cols = pl.ds(u * 256, 256)
            return [pltpu.make_async_copy(wqkv_h.at[pl.ds(r, D // n), cols],
                                          w_v.at[0, pl.ds(r // 2, D // n // 2), cols].bitcast(BF16), sem.at[s])
                    for r in range(0, D, D // n)]

        cp_small = [pltpu.make_async_copy(wr_h, wr_v, sem.at[0]), pltpu.make_async_copy(gw_h, gw_v, sem.at[0]),
                    pltpu.make_async_copy(wphi_h.at[0:8], wphi_v.at[0:8], sem.at[0])]
        def cp_rows(src, dst, n, s):
            return pltpu.make_async_copy(src.at[pl.ds(n * 256, 256)], dst.at[pl.ds(n * 128, 128)].bitcast(BF16), sem.at[s])

        def cp_slab(f, s):
            cols = pl.ds(f * 128, 128)
            return [pltpu.make_async_copy(wg_h.at[:, cols], wg_v.at[:, cols].bitcast(BF16), sem.at[s]),
                    pltpu.make_async_copy(wu_h.at[:, cols], wu_v.at[:, cols].bitcast(BF16), sem.at[s]),
                    pltpu.make_async_copy(wd_h.at[cols], wd_v.at[pl.ds(f * 64, 64)].bitcast(BF16), sem.at[s])]

        batch = {
            "q0": [cp_q(0, 8, P["NS"])],
            "x0": [cp_x(0, 1, 1, P["NS"])],
            "q1": [cp_q(1, 9, P["NS"]) + [pltpu.make_async_copy(wphi_h.at[8:H], wphi_v.at[8:H], sem.at[9])]],
            "x1": [cp_x(1, 2, 2, P["NS"])],
            "q2": [cp_q(2, 10, P["NS"])],
            "q3": [cp_q(3, 10, P["NS"])],
            "x": [cp_x(2, 5, 3, 3)],
            "kv": [cp_x(i, i + 1, 4) for i in (5, 6, 7)]
                  + [[cp_rows(wqkv_h.at[:, pl.ds(j * D, D)], w_v.at[j], n, 4)] for j in (2, 1) for n in range(U)],
            "f0": [cp_slab(f, 5) for f in range(NA)],
            "f1": [[cp_rows(wo_h, wo_v, n, 7)] + cp_slab(NA + n, 7) for n in range(U)]
                  + [cp_slab(f, 7) for f in range(NA + U, 2 * NA)],
            "f2": [cp_slab(f, 12) for f in range(2 * NA, NF)],
        }
        queue = [ds for name in batch for ds in batch[name]]

        def issue(n):
            for ds in queue[:n]:
                start(ds)
            del queue[:n]

        flying = []
        arrived = set()

        def start(ds):
            for d in ds:
                d.start()
                flying.append(d)

        def wait(ds, name):
            with scope(name):
                for d in ds:
                    assert any(d is e for e in flying)
                    flying[:] = [e for e in flying if e is not d]
                    d.wait()

        start(cp_small)
        issue(2)

        kv_v[...] = jnp.zeros_like(kv_v)
        z_v[...] = jnp.zeros_like(z_v)

        r128 = lax.broadcasted_iota(I32, (128, 128), 0)
        c128 = lax.broadcasted_iota(I32, (128, 128), 1)
        diag = (2 * ((r128 % 64) // 32) + r128 // 64) == (c128 // 32)
        er = lax.broadcasted_iota(I32, (128, 32), 0)
        ec = lax.broadcasted_iota(I32, (128, 32), 1)
        eye = jnp.where((er % 32) == ec, 1.0, 0.0).astype(BF16)
        wait(cp_small, "w_small")
        bd = {}

        def prep_phi(groups):
            for g in groups:
                wp = wphi_v[pl.ds(4 * g, 4)].reshape(128, 32)
                t = lax.dot_general(eye, wp, NT, preferred_element_type=F32)
                bd[g] = pltpu.bitcast(jnp.where(diag, t, 0.0).astype(BF16), I32)

        prep_phi(range(2))
        gw = gw_v[...].astype(F32).reshape(1, D)
        wr = wr_v[...].astype(F32).reshape(1, D)

        never = lax.broadcasted_iota(I32, (8, 128), 0) > (pltpu.bitcast(gw[:, 0:128], I32) & 0xFFFF) + 8
        clock = []

        def after(w, dep, every=False):
            if dep is None:
                return w
            dep = pltpu.bitcast(dep, w.dtype)
            if every:
                return jnp.concatenate([jnp.concatenate(
                    [jnp.where(never, dep, w[r:r + 8, c:c + 128]) for c in range(0, w.shape[1], 128)], axis=1)
                    for r in range(0, w.shape[0], 8)], axis=0)
            w0 = jnp.where(never, dep, w[0:8, 0:128])
            if w.shape[1] > 128:
                w0 = jnp.concatenate([w0, w[0:8, 128:]], axis=1)
            return jnp.concatenate([w0, w[8:]], axis=0) if w.shape[0] > 8 else w0

        def now(back=1, row=0):
            if not back or len(clock) < back:
                return None
            t = clock[-back]
            row = row * 8 % t.shape[0]
            return t[row:row + 8, 0:128]

        due = {}

        def before(v, ahead):
            if ahead is None:
                return
            v = pltpu.bitcast(v, I32)
            parts = [v[r:r + 8, c:c + 128] for r in range(0, v.shape[0], 8) for c in range(0, v.shape[1], 128)]
            due.setdefault(len(clock) + ahead, []).append(_tree(parts, jnp.bitwise_or))

        def mm(w, rhs, dims):
            deps = due.pop(len(clock), [])
            if deps:
                w = after(w, _tree(deps, jnp.bitwise_or))
            t = lax.dot_general(_ld(w), rhs, dims, preferred_element_type=F32)
            clock.append(t)
            return t

        def fold(j, s, n):
            def job(lo, hi):
                def run():
                    assert "q%d" % s in arrived if j == 0 else "kv" in arrived
                    blocks = [mm(bd[g], _ld(w_v[j, (k * K2 + lo) // 2:(k * K2 + hi) // 2, g * 128:(g + 1) * 128]), NT)
                              * LOG2E for g in (2 * s, 2 * s + 1) for k in range(2)]
                    for m, t in enumerate(_left(*blocks)):
                        w = _pack(t[0:64], t[64:128])
                        wa_v[j, s, m, :, lo:hi] = w
                        before(w, P["DK"] if j == 1 else None)
                return run
            return [job(c * K2 // n, (c + 1) * K2 // n) for c in range(n)]

        def run_all(jobs):
            for fn in jobs:
                fn()

        def prep_w(j, ref, s):
            def job(c):
                def run():
                    assert ("kv" if j == 2 else "f1") in arrived
                    blocks = [pltpu.bitcast(_ld(after(ref[(k * U + c) * 64:(k * U + c + 1) * 64, g * 128:(g + 1) * 128],
                                                      now(P["WL"]))).T, I32)
                              for g in (2 * s, 2 * s + 1) for k in range(2)]
                    lo, hi = [_left(*[_unpack(w, e) for w in blocks]) for e in range(2)]
                    for m in range(7):
                        w = blocks[0] if m == 2 else blocks[3] if m == 3 else _pack(lo[m], hi[m])
                        wa_v[j, s, m, :, c * 128:(c + 1) * 128] = w
                        before(w, None if m in (2, 3) else P["DW"])
                return run
            return [job(c) for c in range(U)]

        def xblk(i, t, k, c=None):
            cols = slice(k * K2, (k + 1) * K2) if c is None else slice(k * K2 + c * 128, k * K2 + (c + 1) * 128)
            return x_v[(2 * i + t) * 64:(2 * i + t + 1) * 64, cols]

        route = [jnp.full((8, 1), -jnp.inf, F32), jnp.zeros((8, 1), I32)]

        first_x = [[] for _ in range(7)]

        def prep_x(i):
            acc = {}

            def job(c):
                def run():
                    assert ("x%d" % i if i < 2 else "x" if i < 5 else "kv") in arrived
                    words = [after(xblk(i, 0, 0, c), now(P["XL"]), True), xblk(i, 1, 0, c),
                             xblk(i, 0, 1, c), after(xblk(i, 1, 1, c), now(P["XL"]), True)]
                    vals = [[_unpack(w, e) for w in words] for e in range(2)]
                    lo, hi = [_right(*v) for v in vals]
                    for m in range(7):
                        t = words[0] if m == 1 else words[3] if m == 4 else _pack(lo[m], hi[m])
                        if i == 0:
                            first_x[m].append(t)
                            continue
                        w = pltpu.bitcast(_ld(t).T, I32)
                        xs_v[i, m, c * 64:(c + 1) * 64, :] = w
                        before(w[0:8], P["DX"] if i > 0 else None)
                    w1, w2 = wr[:, c * 128:(c + 1) * 128], wr[:, K2 + c * 128:K2 + (c + 1) * 128]
                    for t in range(2):
                        for e in range(2):
                            part = vals[e][t] * w1 + vals[e][2 + t] * w2
                            acc[t, e] = part if c == 0 else acc[t, e] + part
                    if c < U - 1:
                        return
                    tok = i * T + 2 * lax.broadcasted_iota(I32, (8, 1), 0)
                    found = [tuple(route)]
                    for t in range(2):
                        rs = [jnp.sum(acc[t, e], axis=1, keepdims=True).astype(BF16).astype(F32) for e in range(2)]
                        rs = [jnp.where(r != r, -jnp.inf, r) for r in rs]
                        found += [(rs[e][8 * k:8 * k + 8], tok + (t * 128 + 16 * k + e))
                                  for k in range(8) for e in range(2)]
                    route[:] = _tree(found, lambda a, b: (jnp.maximum(a[0], b[0]), jnp.where(b[0] > a[0], b[1], a[1])))
                    before(jnp.broadcast_to(route[1], (8, 128)), P["DR"] if i > 0 else None)
                return run
            return [job(c) for c in range(U)]

        def gates(i):
            def job(t, r0):
                def run():
                    lo = (i * T + t * 128 + r0) // 2
                    xs = _ld(after(x_v[lo:lo + 32, :], now(P["GL"]))).astype(F32)
                    gs = jnp.sum(xs * gw, axis=1, keepdims=True)
                    gate = jnp.broadcast_to(jax.nn.sigmoid(gs), (64, 128))
                    gate_v[i, t, r0:r0 + 64, :] = gate
                    before(gate, P["DG"])
                return run
            return [job(t, r0) for t in range(2) for r0 in (0, 64)]

        def x_op(i, m):
            return xs_v[i, m]

        def proj(j, i, s, jobs):
            if i == 0:
                ops = [xblk(0, 0, 0) if m == 1 else xblk(0, 1, 1) if m == 4 else jnp.concatenate(first_x[m], axis=1)
                       for m in range(7)]
                order = (1, 4, 0, 6, 5, 3, 2) if (j, s) == (0, 0) else (0, 6, 5, 3, 4, 1, 2)
                return _combine(lambda m: mm(wa_v[j, s, m], _ld(ops[m]), NT), jobs, order)
            ops = [x_op(i, m) for m in range(7)]
            return _combine(lambda m: mm(wa_v[j, s, m], _ld(ops[m]), NN), jobs)

        held = []

        def phi_q(i, s, ps):
            def job(e, q):
                def run():
                    for t in range(2):
                        held.append(((i, 2 * s + e, slice(q * 64, (q + 1) * 64), slice(t * 128, (t + 1) * 128)),
                                     _pack(*_phi(ps[e][t][q * 64:(q + 1) * 64],
                                                 lambda v, k: after(v, now(P["QL"], P["QR"][t][k]))))))
                        before(held[-1][1], P["DQ"])
                    if i < NTILE - 1:
                        store_held()
                return run
            return [job(e, q) for e in range(2) for q in range(2)]

        def store_held():
            while held:
                where, val = held.pop(0)
                pq_v[where] = val

        def at(slots, jobs):
            return list(zip(slots, jobs))

        def arrive(name):
            wait([d for ds in batch[name] for d in ds], "w_" + name)
            arrived.add(name)

        def sync(name, then=0, slot=None):
            def run():
                arrive(name)
                issue(then)
            return [(P["HS"] if slot is None else slot, run)]

        arrive("q0")
        issue(1)
        run_all(fold(0, 0, U))
        arrive("x0")
        issue(1)
        run_all(prep_x(0))
        pend = []
        pv = [fn for s in range(U) for fn in prep_w(2, w_v.at[2], s)]
        pk = [fn for s in range(U) for fn in fold(1, s, P["NK"])]
        px = [prep_x(i) for i in range(NTILE)]
        order = [(0, 0), (0, 1), (1, 0), (1, 1), (0, 2), (1, 2), (0, 3), (1, 3)]
        order += [(i, s) for i in range(2, NTILE - 1) for s in range(U)]
        for n, (i, s) in enumerate(order):
            jobs = []
            if n == 1:
                arrive("q1")
                issue(1)
                prep_phi(range(2, G))
                run_all(fold(0, 1, U))
                jobs += sync("x1", 2, P["HS1"]) + at(P["HX1"], px[1])
            if n == 4:
                arrive("q2")
                arrive("q3")
                issue(1)
                run_all(fold(0, 2, U))
                jobs += at(P["HK0"], fold(0, 3, U))
            if n > 4:
                issue(P["IA"][n - 5])
            if n == 7:
                jobs += sync("x") + at(P["HX4"], px[2])
            if n >= 8:
                if (i, s) == (4, 2):
                    jobs += sync("kv")
                if i == 4:
                    jobs += at(P["HX2"], px[5][2 * (s - 2):2 * (s - 1)]) if s >= 2 else []
                else:
                    jobs += at(P["HX6" if i > 4 else "HX"], px[i + 1][s:s + 1])
                k = P["QW"].get(i, (0,) * U)[s]
                jobs += at(sorted(P["HW"][:k]), pv[:k])
                del pv[:k]
                k = P["QK"].get(i, (0,) * U)[s]
                jobs += at(sorted(P["HK"][:k]), pk[:k])
                del pk[:k]
            pend = phi_q(i, s, proj(0, i, s, jobs + at(P["HA6" if i > 4 else "HA"], pend)))

        assert not pv and not pk
        top = jnp.max(route[0], axis=0, keepdims=True)
        idx = jnp.clip(jnp.min(jnp.where(route[0] == top, route[1], S)), 0, S - 1)
        blk = _ld(x_v[pl.ds(pl.multiple_of((idx // 16) * 8, 8), 8), :]).astype(F32)
        sel = lax.broadcasted_iota(I32, (16, D), 0) == (idx % 16)
        xs = jnp.sum(jnp.where(sel, blk, 0.0), axis=0, keepdims=True)
        r_sel = jnp.sum(xs * wr, axis=1, keepdims=True)
        r_gate = jax.nn.sigmoid(r_sel.astype(BF16).astype(F32))

        def spread_token():
            for g in range(G):
                xb_v[g * 128:(g + 1) * 128, :] = after(
                    jnp.broadcast_to(xs[:, g * 128:(g + 1) * 128], (128, 128)), now()).T

        ffn = {"y": [jnp.zeros((8, K2), F32)] * 2}

        def ffn_jobs(f):
            def up(k):
                def run():
                    assert "f%d" % (f // NA) in arrived
                    xb = after(xb_v[k * 256:(k + 1) * 256, :], now(P["FL"]))
                    for name, w_ref in (("g", wg_v), ("u", wu_v)):
                        w = _ld(w_ref[k * 128:(k + 1) * 128, f * 128:(f + 1) * 128]).astype(F32)
                        t = jnp.sum((w * xb).reshape(32, 8, 128), axis=0)
                        ffn[name] = t if k == 0 else ffn[name] + t
                        before(ffn[name], P["DF"])
                    if k == 3:
                        g, u = [jnp.sum(ffn[name], axis=0, keepdims=True) for name in "gu"]
                        ffn["h", f] = jnp.broadcast_to(g * jax.nn.sigmoid(g) * u, (128, 128)).T
                return run

            def down(n):
                def run():
                    assert "f%d" % ((f - 1) // NA) in arrived
                    w = _ld(wd_v[(f - 1) * 64:f * 64, n * K2:(n + 1) * K2]).astype(F32)
                    hb = jnp.concatenate([after(ffn["h", f - 1], now(P["FL"]))] * U, axis=1)
                    ffn["y"][n] = ffn["y"][n] + jnp.sum((w * hb).reshape(16, 8, K2), axis=0)
                    before(ffn["y"][n], P["DF"])
                return run

            return ([down(n) for n in range(2)] if 0 < f else []) + ([up(k) for k in range(4)] if f < NF else [])

        kr = lax.broadcasted_iota(I32, (64, 128), 0)
        kc = lax.broadcasted_iota(I32, (64, 128), 1)
        kmask = (kr // 32) == ((kc // 2) % 2)
        kvb = [None] * (H // 2)

        def kv_step(i, s, ps, vs):
            def job(e, q):
                def run():
                    g = 2 * s + e
                    j = 2 * g + q
                    rows = slice(q * 64, (q + 1) * 64)
                    phis = [_phi(ps[e][t][rows], lambda v, k: after(v, now(P["KVL"], P["KR"][t][k]))) for t in range(2)]
                    zs = [z_v[g, sign, rows] + (phis[0][sign] + phis[1][sign]) for sign in range(2)]
                    phb = jnp.concatenate([_pack(*ph) for ph in phis], axis=1)
                    kv_v[j] += mm(vs[2 * e + q], _ld(phb), NT)
                    if i == NTILE - 1:
                        zs = [jnp.broadcast_to(jnp.sum(z, axis=1, keepdims=True), (64, 128)) for z in zs]
                        t = jnp.concatenate([kv_v[j, pl.ds(0, 32, stride=2), :], kv_v[j, pl.ds(1, 32, stride=2), :]],
                                            axis=0)
                        kvb[j] = pltpu.bitcast(jnp.where(kmask, t, 0.0).astype(BF16), I32)
                    for sign in range(2):
                        z_v[g, sign, rows] = zs[sign]
                return run
            return [job(e, q) for e in range(2) for q in range(2)]

        def tile(i):
            return idx // T if i == NTILE - 1 else i + (idx // T <= i).astype(I32)

        o_pairs, o_parts = {}, {}

        def attn(i, g):
            def pair(h, q):
                def run():
                    rows = slice(q * 64, (q + 1) * 64)
                    w = pq_v[tile(i), h, rows]
                    dn = (_unpack(w, 0) * jnp.concatenate([after(z_v[h, 0, rows], now(P["AL"], P["AR"][q]))] * 2, axis=1)
                          + _unpack(w, 1) * jnp.concatenate([z_v[h, 1, rows]] * 2, axis=1))
                    rden = 1.0 / (_red(dn.reshape(8, 8, T), jnp.add) + 1e-6)
                    num = mm(kvb[2 * h + q], _ld(w), NN)
                    o_pairs[i, h, q] = [num[0:32] * rden[0:1], num[32:64] * rden[1:2]]
                return run

            def join():
                a, b = [jnp.concatenate(o_pairs.pop((i, h, 0)) + o_pairs.pop((i, h, 1)), axis=0) for h in (g, g + U)]
                o_parts[i, g] = _right(a[:, :128], a[:, 128:], b[:, :128], b[:, 128:])
                for m in SUMS:
                    before(o_parts[i, g][m][0:8], P["DA"])

            return [pair(h, q) for h in (g, g + U) for q in range(2)] + [join]

        def o_ops(i):
            parts = [o_parts.pop((i, g)) for g in range(U)]
            return [jnp.concatenate([p[m] for p in parts], axis=0).astype(BF16) for m in range(7)]

        first = [attn(0, g) for g in range(U)]
        def finish_ffn():
            ffn["out"] = jnp.sum(jnp.concatenate(ffn["y"], axis=1), axis=0, keepdims=True) * r_gate

        rest = [(f, fn) for f in range(NF + 1) for fn in ffn_jobs(f)] + [(0, finish_ffn)]
        ready = [0]

        def take(n):
            got, rest[:] = rest[:n], rest[n:]
            assert all(min(f, NF - 1) < ready[0] for f, _ in got)
            return [fn for _, fn in got]

        HB = P["HB"]
        for i in range(NTILE):
            gj = gates(i)
            ready[0] = 2 * NA if i >= P["F1"] else NA if i >= F0 else 0
            for s in range(U):
                fj = take(P["QB"][i][s])
                if (i, s) == (0, 0):
                    fj = [spread_token]
                issue(P["IB"][i][s])
                vt = proj(2, i, s, (sync("f0") if (i, s) == (F0, 0) else sync("f1") if (i, s) == (P["F1"], 0) else [])
                          + at(HB[1], pend[:HB[0]]) + at(sorted(P["HF0"][len(fj) // 2 * -1:]), fj[:len(fj) // 2]) + at(P["HG"], gj[s:s + 1]))
                vts = [jnp.concatenate([_pack(b[q * 64:q * 64 + 32], b[q * 64 + 32:q * 64 + 64]) for b in vt[e]], axis=1)
                       for e in range(2) for q in range(2)]
                jobs = at(HB[2], pend[HB[0]:]) + at(sorted(P["HF1"][:(len(fj) + 1) // 2]), fj[len(fj) // 2:])
                if P["F1"] <= i < P["F1"] + 2:
                    jobs += at(P["HO"], prep_w(3, wo_v, (i - P["F1"]) * 2 + s // 2)[2 * (s % 2):2 * (s % 2) + 2])
                if i == NTILE - 1 and s >= 2:
                    jobs += at(P["H0"], [first[g][n] for g in (2 * s - 4, 2 * s - 3) for n in range(2)])
                pend = kv_step(i, s, proj(1, i, s, jobs), vts)

        late = [[], [(0, 2), (0, 3), (0, 4), (1, 2), (1, 3), (1, 4)], [(2, 2), (2, 3), (2, 4)], [(3, 2), (3, 3), (3, 4)]]
        for s in range(U):
            jobs = at(P["HA7"], pend) + at(P["H1"][s], [first[g][n] for g, n in late[s]])
            pend = phi_q(NTILE - 1, s, proj(0, NTILE - 1, s, jobs))

        def cp_o(i, r0, nr, c0, nc):
            rows = pl.ds(pl.multiple_of(tile(i) * T + r0, 128), nr)
            return pltpu.make_async_copy(out_v.at[pl.ds(i * T + r0, nr), pl.ds(c0, nc)],
                                         out_h.at[rows, pl.ds(c0, nc)], sem.at[6])

        outs = []

        def mix(i, c, blocks):
            def job(n, t):
                def run():
                    r0, c0 = i * T + t * 128, (2 * c + n) * 128
                    g = gate_v[tile(i), t]
                    xt = _ld(x_v[pl.ds(pl.multiple_of(tile(i) * 128 + t * 64, 64), 64), c0:c0 + 128]).astype(F32)
                    upd = xt * 0.0
                    if i == NTILE - 1:
                        tok = t * 128 + lax.broadcasted_iota(I32, (128, 128), 0)
                        upd = upd + jnp.where(tok == idx % T, ffn["out"][:, c0:c0 + 128], 0.0)
                    a = after(blocks[n][t], now(P["ML"], P["MR"][2 * t + n])).T
                    res = g * a + (1.0 - g) * (xt + upd)
                    out_v[r0:r0 + 128, c0:c0 + 128] = res.astype(BF16)
                    before(res, P["DM"])
                    if i == NTILE - 1:
                        new = [cp_o(i, t * 128, 128, c * 256, 256)] if n == 1 else []
                    else:
                        new = [cp_o(i, 0, T, 0, D)] if (c, n, t) == (U - 1, 1, 1) else []
                    start(new)
                    outs.extend(new)
                return run
            return [job(n, t) for t in range(2) for n in range(2)]

        for i in range(NTILE):
            ops = o_ops(i)
            assert i < NTILE - 1 or not rest
            aj = [fn for g in range(U) for fn in attn(i + 1, g)] if i + 1 < NTILE else []
            for c in range(U):
                jobs = at(P["HM"], pend) + [(n - 7 * c, fn) for n, fn in zip(P["HT"], aj) if n // 7 == c]
                if (i, c) == (1, 0):
                    store_held()
                if (i, c) == P["W7"]:
                    jobs = sync("f2") + jobs
                    ready[0] = NF
                fj = take(P["QC"][c])
                jobs += at(P["HC"][-len(fj):], fj)
                if (i, c) == (NTILE - 1, U - 1):
                    def early(c11, c21):
                        for fn in mix(i, c, ((c11, None), (c21, None)))[:2]:
                            fn()
                    pend = mix(i, c, _combine(lambda m: mm(wa_v[3, c, m], ops[m], NN), jobs, early=early))[2:]
                else:
                    pend = mix(i, c, _combine(lambda m: mm(wa_v[3, c, m], ops[m], NN), jobs))
        for fn in pend:
            fn()
        wait(outs, "w_out")
        assert not flying

    return kernel


DEFAULTS = dict(
    F0=2,
    F1=5,
    NA=12,
    W7=(0, 0),
    HS=1,
    PROF=False,
    FLAGS=None,
    NS=1,
    HS1=2,
    HX1=(2, 3, 4, 5),
    HK0=(0, 2, 4, 6),
    IA=(0, 1, 1, 1, 1, 1, 1, 1, 1, 1, 1, 1, 0, 1, 0, 1, 0, 1, 0, 1, 0, 1, 0),
    IB=((1, 1, 2, 1), (1, 1, 1, 1), (1, 1, 1, 1), (1, 1, 1, 1), (1, 1, 1, 1), (1, 1, 1, 1), (1, 1, 1, 1), (1, 1, 1, 1)),
    QB=((0, 0, 0, 0), (0, 0, 0, 0), (4, 6, 6, 6), (6, 6, 6, 6), (6, 6, 6, 6), (6, 6, 6, 6), (6, 6, 6, 6), (6, 6, 6, 6)),
    QC=(1, 1, 1, 1),
    QW={5: (2, 2, 2, 2), 6: (2, 2, 2, 2)},
    NK=2,
    QK={5: (1, 1, 1, 1), 6: (1, 1, 1, 1)},
    HA=(0, 2, 4, 6),
    QL=2,
    DQ=None,
    XL=3,
    DX=4,
    DR=None,
    HX=(4,),
    HX4=(1, 2, 4, 5),
    QR=((0, 4), (8, 12)),
    HA6=(0, 2, 4, 6),
    HX6=(1,),
    HX2=(3, 6),
    HW=(1, 5, 3),
    DK=None,
    DW=5,
    WL=3,
    HB=(2, (3, 6), (2, 5)),
    KVL=4,
    KR=((0, 4), (8, 12)),
    HG=(6,),
    DG=5,
    GL=2,
    HF0=(0, 2, 5),
    HF1=(1, 4, 6),
    DF=8,
    FL=1,
    HO=(2, 6),
    H0=(0, 3, 6, 6),
    H1=((), (0, 1, 2, 3, 5, 6), (1, 1, 5), (1, 1, 3)),
    HA7=(0, 0, 4, 5),
    HM=(0, 2, 4, 6),
    HT=(0, 2, 3, 3, 5, 5, 6, 7, 8, 10, 11, 11, 12, 13, 15, 15, 16, 17, 18, 21),
    HC=(6,),
    DM=4,
    ML=4,
    AL=2,
    DA=None,
    MR=(8, 0, 0, 0),
    AR=(0, 0),
    HK=(0, 4),
)


def make(**kw):
    P = dict(DEFAULTS, **kw)

    @jax.jit
    def run(A_x, A_wqkv, A_w_phi, A_wo, B_x, B_w_r, B_w_gate, B_w_up, B_w_down, gate_w):
        B, S, D = A_x.shape
        F = B_w_gate.shape[1]
        H = A_w_phi.shape[0]
        NTILE = S // 256
        G = D // 128
        any_spec = pl.BlockSpec(memory_space=pl.ANY)
        V = pltpu.VMEM
        scratch = [
            V((S // 2, D), I32),
            V((NTILE, 7, D // 4, 128), I32),
            V((3, D // 2, D), I32),
            V((4, G // 2, 7, 64, D // 2), I32),
            V((H, 32, 32), BF16),
            V((D // 2, D), I32),
            V((D,), BF16),
            V((D,), BF16),
            V((D // 2, F), I32),
            V((D // 2, F), I32),
            V((F // 2, D), I32),
            V((NTILE, G, 128, 256), I32),
            V((NTILE, 2, 128, 128), F32),
            V((H // 2, 64, 128), F32),
            V((G, 2, 128, 128), F32),
            V((D, 128), F32),
            V((S, D), BF16),
            pltpu.SemaphoreType.DMA((13,)),
        ]
        out = pl.pallas_call(
            _make_kernel(S, D, F, H, P),
            out_shape=jax.ShapeDtypeStruct((S, D), A_x.dtype),
            in_specs=[any_spec] * 9,
            out_specs=any_spec,
            scratch_shapes=scratch,
            compiler_params=pltpu.CompilerParams(vmem_limit_bytes=110 * 2**20, flags=P["FLAGS"]),
        )(A_x.reshape(S, D), A_wqkv, A_w_phi, A_wo, B_w_r, B_w_gate, B_w_up, B_w_down, gate_w)
        return out.reshape(B, S, D)
    return run


_run = make()


@jax.jit
def pallas_gated_mix__linear_kernel_hedgehog__moe_arch_mod__prompt_kernel(
    A_x, A_wqkv, A_w_phi, A_wo, B_x, B_w_r, B_w_gate, B_w_up, B_w_down, gate_w
):
    return _run(A_x, A_wqkv, A_w_phi, A_wo, B_x, B_w_r, B_w_gate, B_w_up, B_w_down, gate_w)
```

```python
import contextlib

import jax
import jax.numpy as jnp
from jax import lax
import jax.experimental.pallas as pl
import jax.experimental.pallas.tpu as pltpu

F32 = jnp.float32
BF16 = jnp.bfloat16
I32 = jnp.int32
LOG2E = 1.4426950408889634
NT = (((1,), (1,)), ((), ()))
NN = (((1,), (0,)), ((), ()))


def _ld(v):
    return pltpu.bitcast(v, BF16)


def _pack(a, b):
    return pltpu.bitcast(pltpu.pack_elementwise([a, b], packed_dtype=BF16), I32)


def _unpack(w, k):
    return pltpu.unpack_elementwise(w, index=k, packed_dtype=BF16, unpacked_dtype=F32)


def _tree(vs, op):
    while len(vs) > 1:
        vs = [op(vs[k], vs[k + 1]) if k + 1 < len(vs) else vs[k] for k in range(0, len(vs), 2)]
    return vs[0]


def _left(a11, a12, a21, a22):
    return [a11 + a22, a21 + a22, a11, a22, a11 + a12, a21 - a11, a12 - a22]


def _right(b11, b12, b21, b22):
    return [b11 + b22, b11, b12 - b22, b21 - b11, b22, b11 + b12, b21 + b22]


_USES = (((0, 1), (3, 1)), ((2, 1), (3, -1)), ((1, 1), (3, 1)), ((0, 1), (2, 1)),
         ((0, -1), (1, 1)), ((3, 1),), ((0, 1),))


def _combine(mul, jobs, order=(0, 6, 5, 3, 4, 1, 2), early=None):
    c = [None] * 4
    for n, m in enumerate(order):
        if early and n == 6:
            early(c[0], c[2])
        t = mul(m)
        for k, sign in _USES[m]:
            if c[k] is None:
                c[k] = t if sign > 0 else -t
            else:
                c[k] = c[k] + t if sign > 0 else c[k] - t
        for at, fn in jobs:
            if at == n:
                fn()
    return (c[0], c[1]), (c[2], c[3])


def _red(v, op):
    r = _tree([v[k] for k in range(v.shape[0])], op)
    r = op(r, pltpu.roll(r, 4, 0))
    return op(r, pltpu.roll(r, 2, 0))


def _rcp(s):
    r = pl.reciprocal(s, approx=True)
    return r * (2.0 - s * r)


def _phi(p, tie):
    p = p.reshape(8, 8, 128)
    ep = jnp.exp2(p - tie(_red(p, jnp.maximum), 0))
    en = jnp.exp2(tie(_red(p, jnp.minimum), 1) - p)
    ep = ep * _rcp(_red(ep, jnp.add))
    en = en * _rcp(_red(en, jnp.add))
    return ep.reshape(64, 128), en.reshape(64, 128)


def _make_kernel(S, D, F, H, P):
    scope = jax.named_scope if P["PROF"] else (lambda n: contextlib.nullcontext())
    T = 256
    NTILE = S // T
    G = D // 128
    U = G // 2
    K2 = D // 2
    NF = F // 128
    F0 = P["F0"]
    NA = P["NA"]
    SUMS = (0, 2, 3, 5, 6)

    def kernel(ax_h, wqkv_h, wphi_h, wo_h, wr_h, wg_h, wu_h, wd_h, gw_h, out_h,
               x_v, xs_v, w_v, wa_v, wphi_v, wo_v, wr_v, gw_v, wg_v, wu_v, wd_v,
               pq_v, gate_v, kv_v, z_v, xb_v, out_v, sem):
        def cp_x(lo, hi, s, n=1):
            step = (hi - lo) * T // n
            return [pltpu.make_async_copy(ax_h.at[pl.ds(r, step)], x_v.at[pl.ds(r // 2, step // 2)].bitcast(BF16), sem.at[s])
                    for r in range(lo * T, hi * T, step)]

        def cp_q(u, s, n=1):
            cols = pl.ds(u * 256, 256)
            return [pltpu.make_async_copy(wqkv_h.at[pl.ds(r, D // n), cols],
                                          w_v.at[0, pl.ds(r // 2, D // n // 2), cols].bitcast(BF16), sem.at[s])
                    for r in range(0, D, D // n)]

        def cp_phi(u, s):
            heads = pl.ds(u * H // U, H // U)
            return pltpu.make_async_copy(wphi_h.at[heads], wphi_v.at[heads], sem.at[s])

        cp_small = [pltpu.make_async_copy(wr_h, wr_v, sem.at[0]), pltpu.make_async_copy(gw_h, gw_v, sem.at[0]),
                    cp_phi(0, 0)]
        def cp_rows(src, dst, n, s):
            return pltpu.make_async_copy(src.at[pl.ds(n * 256, 256)], dst.at[pl.ds(n * 128, 128)].bitcast(BF16), sem.at[s])

        def cp_slab(f, s):
            cols = pl.ds(f * 128, 128)
            return [pltpu.make_async_copy(wg_h.at[:, cols], wg_v.at[:, cols].bitcast(BF16), sem.at[s]),
                    pltpu.make_async_copy(wu_h.at[:, cols], wu_v.at[:, cols].bitcast(BF16), sem.at[s]),
                    pltpu.make_async_copy(wd_h.at[cols], wd_v.at[pl.ds(f * 64, 64)].bitcast(BF16), sem.at[s])]

        batch = {
            "q0": [cp_q(0, 8, P["NS"])],
            "x0": [cp_x(0, 1, 1, P["NS"])],
            "q1": [cp_q(1, 9, P["NS"]) + [cp_phi(1, 9)]],
            "x1": [cp_x(1, 2, 2, P["NS"])],
            "q2": [cp_q(2, 10, P["NS"]) + [cp_phi(2, 10)]],
            "q3": [cp_q(3, 10, P["NS"]) + [cp_phi(3, 10)]],
            "x": [cp_x(2, 5, 3, 3)],
            "kv": [cp_x(i, i + 1, 4) for i in (5, 6, 7)]
                  + [[cp_rows(wqkv_h.at[:, pl.ds(j * D, D)], w_v.at[j], n, 4)] for j in (2, 1) for n in range(U)],
            "f0": [cp_slab(f, 5) for f in range(NA)],
            "f1": [[cp_rows(wo_h, wo_v, n, 7)] + cp_slab(NA + n, 7) for n in range(U)]
                  + [cp_slab(f, 7) for f in range(NA + U, 2 * NA)],
            "f2": [cp_slab(f, 12) for f in range(2 * NA, NF)],
        }
        queue = [ds for name in batch for ds in batch[name]]

        def issue(n):
            for ds in queue[:n]:
                start(ds)
            del queue[:n]

        flying = []
        arrived = set()

        def start(ds):
            for d in ds:
                d.start()
                flying.append(d)

        def wait(ds, name):
            with scope(name):
                for d in ds:
                    assert any(d is e for e in flying)
                    flying[:] = [e for e in flying if e is not d]
                    d.wait()

        start(cp_small)
        issue(2)

        kv_v[...] = jnp.zeros_like(kv_v)
        z_v[...] = jnp.zeros_like(z_v)

        r128 = lax.broadcasted_iota(I32, (128, 128), 0)
        c128 = lax.broadcasted_iota(I32, (128, 128), 1)
        diag = (2 * ((r128 % 64) // 32) + r128 // 64) == (c128 // 32)
        er = lax.broadcasted_iota(I32, (128, 32), 0)
        ec = lax.broadcasted_iota(I32, (128, 32), 1)
        eye = jnp.where((er % 32) == ec, 1.0, 0.0).astype(BF16)
        wait(cp_small, "w_small")
        bd = {}

        def prep_phi(groups):
            for g in groups:
                wp = wphi_v[pl.ds(4 * g, 4)].reshape(128, 32)
                t = lax.dot_general(eye, wp, NT, preferred_element_type=F32)
                bd[g] = pltpu.bitcast(jnp.where(diag, t, 0.0).astype(BF16), I32)

        prep_phi(range(2))
        gw = gw_v[...].astype(F32).reshape(1, D)
        wr = wr_v[...].astype(F32).reshape(1, D)

        never = lax.broadcasted_iota(I32, (8, 128), 0) > (pltpu.bitcast(gw[:, 0:128], I32) & 0xFFFF) + 8
        clock = []

        def after(w, dep, every=False):
            if dep is None:
                return w
            dep = pltpu.bitcast(dep, w.dtype)
            if every:
                return jnp.concatenate([jnp.concatenate(
                    [jnp.where(never, dep, w[r:r + 8, c:c + 128]) for c in range(0, w.shape[1], 128)], axis=1)
                    for r in range(0, w.shape[0], 8)], axis=0)
            w0 = jnp.where(never, dep, w[0:8, 0:128])
            if w.shape[1] > 128:
                w0 = jnp.concatenate([w0, w[0:8, 128:]], axis=1)
            return jnp.concatenate([w0, w[8:]], axis=0) if w.shape[0] > 8 else w0

        def now(back=1, row=0):
            if not back or len(clock) < back:
                return None
            t = clock[-back]
            row = row * 8 % t.shape[0]
            return t[row:row + 8, 0:128]

        due = {}

        def before(v, ahead):
            if ahead is None:
                return
            v = pltpu.bitcast(v, I32)
            parts = [v[r:r + 8, c:c + 128] for r in range(0, v.shape[0], 8) for c in range(0, v.shape[1], 128)]
            due.setdefault(len(clock) + ahead, []).append(_tree(parts, jnp.bitwise_or))

        def mm(w, rhs, dims):
            deps = due.pop(len(clock), [])
            if deps:
                w = after(w, _tree(deps, jnp.bitwise_or))
            t = lax.dot_general(_ld(w), rhs, dims, preferred_element_type=F32)
            clock.append(t)
            return t

        def fold(j, s, n):
            def job(lo, hi):
                def run():
                    assert "q%d" % s in arrived if j == 0 else "kv" in arrived
                    blocks = [mm(bd[g], _ld(w_v[j, (k * K2 + lo) // 2:(k * K2 + hi) // 2, g * 128:(g + 1) * 128]), NT)
                              * LOG2E for g in (2 * s, 2 * s + 1) for k in range(2)]
                    for m, t in enumerate(_left(*blocks)):
                        w = _pack(t[0:64], t[64:128])
                        wa_v[j, s, m, :, lo:hi] = w
                        before(w, P["DK"] if j == 1 else None)
                return run
            return [job(c * K2 // n, (c + 1) * K2 // n) for c in range(n)]

        def run_all(jobs):
            for fn in jobs:
                fn()

        def prep_w(j, ref, s):
            def job(c):
                def run():
                    assert ("kv" if j == 2 else "f1") in arrived
                    blocks = [pltpu.bitcast(_ld(after(ref[(k * U + c) * 64:(k * U + c + 1) * 64, g * 128:(g + 1) * 128],
                                                      now(P["WL"]))).T, I32)
                              for g in (2 * s, 2 * s + 1) for k in range(2)]
                    lo, hi = [_left(*[_unpack(w, e) for w in blocks]) for e in range(2)]
                    for m in range(7):
                        w = blocks[0] if m == 2 else blocks[3] if m == 3 else _pack(lo[m], hi[m])
                        wa_v[j, s, m, :, c * 128:(c + 1) * 128] = w
                        before(w, None if m in (2, 3) else P["DW"])
                return run
            return [job(c) for c in range(U)]

        def xblk(i, t, k, c=None):
            cols = slice(k * K2, (k + 1) * K2) if c is None else slice(k * K2 + c * 128, k * K2 + (c + 1) * 128)
            return x_v[(2 * i + t) * 64:(2 * i + t + 1) * 64, cols]

        route = [jnp.full((8, 1), -jnp.inf, F32), jnp.zeros((8, 1), I32)]

        first_x = [[] for _ in range(7)]

        def prep_x(i):
            acc = {}

            def job(c):
                def run():
                    assert ("x%d" % i if i < 2 else "x" if i < 5 else "kv") in arrived
                    words = [after(xblk(i, 0, 0, c), now(P["XL"]), True), xblk(i, 1, 0, c),
                             xblk(i, 0, 1, c), after(xblk(i, 1, 1, c), now(P["XL"]), True)]
                    vals = [[_unpack(w, e) for w in words] for e in range(2)]
                    lo, hi = [_right(*v) for v in vals]
                    for m in range(7):
                        t = words[0] if m == 1 else words[3] if m == 4 else _pack(lo[m], hi[m])
                        if i == 0:
                            first_x[m].append(t)
                            continue
                        w = pltpu.bitcast(_ld(t).T, I32)
                        xs_v[i, m, c * 64:(c + 1) * 64, :] = w
                        before(w[0:8], P["DX"] if i > 0 else None)
                    w1, w2 = wr[:, c * 128:(c + 1) * 128], wr[:, K2 + c * 128:K2 + (c + 1) * 128]
                    for t in range(2):
                        for e in range(2):
                            part = vals[e][t] * w1 + vals[e][2 + t] * w2
                            acc[t, e] = part if c == 0 else acc[t, e] + part
                    if c < U - 1:
                        return
                    tok = i * T + 2 * lax.broadcasted_iota(I32, (8, 1), 0)
                    found = [tuple(route)]
                    for t in range(2):
                        rs = [jnp.sum(acc[t, e], axis=1, keepdims=True).astype(BF16).astype(F32) for e in range(2)]
                        rs = [jnp.where(r != r, -jnp.inf, r) for r in rs]
                        found += [(rs[e][8 * k:8 * k + 8], tok + (t * 128 + 16 * k + e))
                                  for k in range(8) for e in range(2)]
                    route[:] = _tree(found, lambda a, b: (jnp.maximum(a[0], b[0]), jnp.where(b[0] > a[0], b[1], a[1])))
                    before(jnp.broadcast_to(route[1], (8, 128)), P["DR"] if i > 0 else None)
                return run
            return [job(c) for c in range(U)]

        def gates(i):
            def job(t, r0):
                def run():
                    lo = (i * T + t * 128 + r0) // 2
                    xs = _ld(after(x_v[lo:lo + 32, :], now(P["GL"]))).astype(F32)
                    gs = jnp.sum(xs * gw, axis=1, keepdims=True)
                    gate = jnp.broadcast_to(jax.nn.sigmoid(gs), (64, 128))
                    gate_v[i, t, r0:r0 + 64, :] = gate
                    before(gate, P["DG"])
                return run
            return [job(t, r0) for t in range(2) for r0 in (0, 64)]

        def x_op(i, m):
            return xs_v[i, m]

        def proj(j, i, s, jobs):
            if i == 0:
                ops = [xblk(0, 0, 0) if m == 1 else xblk(0, 1, 1) if m == 4 else jnp.concatenate(first_x[m], axis=1)
                       for m in range(7)]
                order = (1, 4, 0, 6, 5, 3, 2) if (j, s) == (0, 0) else (0, 6, 5, 3, 4, 1, 2)
                return _combine(lambda m: mm(wa_v[j, s, m], _ld(ops[m]), NT), jobs, order)
            ops = [x_op(i, m) for m in range(7)]
            return _combine(lambda m: mm(wa_v[j, s, m], _ld(ops[m]), NN), jobs, P["OA"] if j == 0 else P["OB"])

        held = []

        def phi_q(i, s, ps):
            def job(e, q):
                def run():
                    for t in range(2):
                        held.append(((i, 2 * s + e, slice(q * 64, (q + 1) * 64), slice(t * 128, (t + 1) * 128)),
                                     _pack(*_phi(ps[e][t][q * 64:(q + 1) * 64],
                                                 lambda v, k: after(v, now(P["QL"], P["QR"][t][k]))))))
                        before(held[-1][1], P["DQ"])
                    if i < NTILE - 1:
                        store_held()
                return run
            return [job(e, q) for e in range(2) for q in range(2)]

        def store_held():
            while held:
                where, val = held.pop(0)
                pq_v[where] = val

        def at(slots, jobs):
            return list(zip(slots, jobs))

        def arrive(name):
            wait([d for ds in batch[name] for d in ds], "w_" + name)
            arrived.add(name)

        def sync(name, then=0):
            def run():
                arrive(name)
                issue(then)
            return [(P["HS"][name], run)]

        arrive("q0")
        issue(1)
        run_all(fold(0, 0, U))
        arrive("x0")
        issue(1)
        run_all(prep_x(0))
        pend = []
        pv = [fn for s in range(U) for fn in prep_w(2, w_v.at[2], s)]
        pk = [fn for s in range(U) for fn in fold(1, s, P["NK"])]
        px = [prep_x(i) for i in range(NTILE)]
        order = [(0, 0), (0, 1), (1, 0), (1, 1), (0, 2), (1, 2), (0, 3), (1, 3)]
        order += [(i, s) for i in range(2, NTILE - 1) for s in range(U)]
        for n, (i, s) in enumerate(order):
            jobs = []
            if n == 1:
                arrive("q1")
                issue(1)
                prep_phi(range(2, 4))
                run_all(fold(0, 1, U))
                jobs += sync("x1", 2) + at(P["HX1"], px[1])
            if n == 4:
                arrive("q2")
                arrive("q3")
                issue(1)
                prep_phi(range(4, G))
                run_all(fold(0, 2, U))
                jobs += at(P["HK0"], fold(0, 3, U))
            if n > 4:
                issue(P["IA"][n - 5])
            if n == 7:
                jobs += sync("x") + at(P["HX4"], px[2])
            if n >= 8:
                if (i, s) == (4, 2):
                    jobs += sync("kv")
                if i == 4:
                    jobs += at(P["HX2"], px[5][2 * (s - 2):2 * (s - 1)]) if s >= 2 else []
                else:
                    jobs += at(P["HX6" if i > 4 else "HX"], px[i + 1][s:s + 1])
                k = P["QW"].get(i, (0,) * U)[s]
                jobs += at(sorted(P["HW"][:k]), pv[:k])
                del pv[:k]
                k = P["QK"].get(i, (0,) * U)[s]
                jobs += at(sorted(P["HK"][:k]), pk[:k])
                del pk[:k]
            pend = phi_q(i, s, proj(0, i, s, jobs + at(P["HA6" if i > 4 else "HA"], pend)))

        assert not pv and not pk
        top = jnp.max(route[0], axis=0, keepdims=True)
        idx = jnp.clip(jnp.min(jnp.where(route[0] == top, route[1], S)), 0, S - 1)
        blk = _ld(x_v[pl.ds(pl.multiple_of((idx // 16) * 8, 8), 8), :]).astype(F32)
        sel = lax.broadcasted_iota(I32, (16, D), 0) == (idx % 16)
        xs = jnp.sum(jnp.where(sel, blk, 0.0), axis=0, keepdims=True)
        r_sel = jnp.sum(xs * wr, axis=1, keepdims=True)
        r_gate = jax.nn.sigmoid(r_sel.astype(BF16).astype(F32))

        def spread_token():
            for g in range(G):
                xb_v[g * 128:(g + 1) * 128, :] = after(
                    jnp.broadcast_to(xs[:, g * 128:(g + 1) * 128], (128, 128)), now()).T

        ffn = {"y": [jnp.zeros((8, K2), F32)] * 2}

        def ffn_jobs(f):
            def up(k):
                def run():
                    assert "f%d" % (f // NA) in arrived
                    xb = after(xb_v[k * 256:(k + 1) * 256, :], now(P["FL"]))
                    for name, w_ref in (("g", wg_v), ("u", wu_v)):
                        w = _ld(w_ref[k * 128:(k + 1) * 128, f * 128:(f + 1) * 128]).astype(F32)
                        t = jnp.sum((w * xb).reshape(32, 8, 128), axis=0)
                        ffn[name] = t if k == 0 else ffn[name] + t
                        before(ffn[name], P["DF"])
                    if k == 3:
                        g, u = [jnp.sum(ffn[name], axis=0, keepdims=True) for name in "gu"]
                        ffn["h", f] = jnp.broadcast_to(g * jax.nn.sigmoid(g) * u, (128, 128)).T
                return run

            def down(n):
                def run():
                    assert "f%d" % ((f - 1) // NA) in arrived
                    w = _ld(wd_v[(f - 1) * 64:f * 64, n * K2:(n + 1) * K2]).astype(F32)
                    hb = jnp.concatenate([after(ffn["h", f - 1], now(P["FL"]))] * U, axis=1)
                    ffn["y"][n] = ffn["y"][n] + jnp.sum((w * hb).reshape(16, 8, K2), axis=0)
                    before(ffn["y"][n], P["DF"])
                return run

            return ([down(n) for n in range(2)] if 0 < f else []) + ([up(k) for k in range(4)] if f < NF else [])

        kr = lax.broadcasted_iota(I32, (64, 128), 0)
        kc = lax.broadcasted_iota(I32, (64, 128), 1)
        kmask = (kr // 32) == ((kc // 2) % 2)
        kvb = [None] * (H // 2)

        def kv_step(i, s, ps, vs):
            def job(e, q):
                def run():
                    g = 2 * s + e
                    j = 2 * g + q
                    rows = slice(q * 64, (q + 1) * 64)
                    phis = [_phi(ps[e][t][rows], lambda v, k: after(v, now(P["KVL"], P["KR"][t][k]))) for t in range(2)]
                    zs = [z_v[g, sign, rows] + (phis[0][sign] + phis[1][sign]) for sign in range(2)]
                    phb = jnp.concatenate([_pack(*ph) for ph in phis], axis=1)
                    kv_v[j] += mm(vs[2 * e + q], _ld(phb), NT)
                    if i == NTILE - 1:
                        zs = [jnp.broadcast_to(jnp.sum(z, axis=1, keepdims=True), (64, 128)) for z in zs]
                        t = jnp.concatenate([kv_v[j, pl.ds(0, 32, stride=2), :], kv_v[j, pl.ds(1, 32, stride=2), :]],
                                            axis=0)
                        kvb[j] = pltpu.bitcast(jnp.where(kmask, t, 0.0).astype(BF16), I32)
                    for sign in range(2):
                        z_v[g, sign, rows] = zs[sign]
                return run
            return [job(e, q) for e in range(2) for q in range(2)]

        def tile(i):
            return idx // T if i == NTILE - 1 else i + (idx // T <= i).astype(I32)

        o_pairs, o_parts = {}, {}

        def attn(i, g):
            def pair(h, q):
                def run():
                    rows = slice(q * 64, (q + 1) * 64)
                    w = pq_v[tile(i), h, rows]
                    dn = (_unpack(w, 0) * jnp.concatenate([after(z_v[h, 0, rows], now(P["AL"], P["AR"][q]))] * 2, axis=1)
                          + _unpack(w, 1) * jnp.concatenate([z_v[h, 1, rows]] * 2, axis=1))
                    rden = 1.0 / (_red(dn.reshape(8, 8, T), jnp.add) + 1e-6)
                    num = mm(kvb[2 * h + q], _ld(w), NN)
                    o_pairs[i, h, q] = [num[0:32] * rden[0:1], num[32:64] * rden[1:2]]
                return run

            def join():
                a, b = [jnp.concatenate(o_pairs.pop((i, h, 0)) + o_pairs.pop((i, h, 1)), axis=0) for h in (g, g + U)]
                o_parts[i, g] = _right(a[:, :128], a[:, 128:], b[:, :128], b[:, 128:])
                for m in SUMS:
                    before(o_parts[i, g][m][0:8], P["DA"])

            return [pair(h, q) for h in (g, g + U) for q in range(2)] + [join]

        def o_ops(i):
            parts = [o_parts.pop((i, g)) for g in range(U)]
            return [jnp.concatenate([p[m] for p in parts], axis=0).astype(BF16) for m in range(7)]

        first = [attn(0, g) for g in range(U)]
        def finish_ffn():
            ffn["out"] = jnp.sum(jnp.concatenate(ffn["y"], axis=1), axis=0, keepdims=True) * r_gate

        rest = [(f, fn) for f in range(NF + 1) for fn in ffn_jobs(f)] + [(0, finish_ffn)]
        ready = [0]

        def take(n):
            got, rest[:] = rest[:n], rest[n:]
            assert all(min(f, NF - 1) < ready[0] for f, _ in got)
            return [fn for _, fn in got]

        HB = P["HB"]
        for i in range(NTILE):
            gj = gates(i)
            ready[0] = 2 * NA if i >= P["F1"] else NA if i >= F0 else 0
            for s in range(U):
                fj = take(P["QB"][i][s])
                if (i, s) == (0, 0):
                    fj = [spread_token]
                issue(P["IB"][i][s])
                vt = proj(2, i, s, (sync("f0") if (i, s) == (F0, 0) else sync("f1") if (i, s) == (P["F1"], 0) else [])
                          + at(HB[1], pend[:HB[0]]) + at(sorted(P["HF0"][len(fj) // 2 * -1:]), fj[:len(fj) // 2]) + at(P["HG"], gj[s:s + 1]))
                vts = [jnp.concatenate([_pack(b[q * 64:q * 64 + 32], b[q * 64 + 32:q * 64 + 64]) for b in vt[e]], axis=1)
                       for e in range(2) for q in range(2)]
                jobs = at(HB[2], pend[HB[0]:]) + at(sorted(P["HF1"][:(len(fj) + 1) // 2]), fj[len(fj) // 2:])
                if P["F1"] <= i < P["F1"] + 2:
                    jobs += at(P["HO"], prep_w(3, wo_v, (i - P["F1"]) * 2 + s // 2)[2 * (s % 2):2 * (s % 2) + 2])
                if i == NTILE - 1 and s >= 2:
                    jobs += at(P["H0"], [first[g][n] for g in (2 * s - 4, 2 * s - 3) for n in range(2)])
                pend = kv_step(i, s, proj(1, i, s, jobs), vts)

        late = [[], [(0, 2), (0, 3), (0, 4), (1, 2), (1, 3), (1, 4)], [(2, 2), (2, 3), (2, 4)], [(3, 2), (3, 3), (3, 4)]]
        for s in range(U):
            jobs = at(P["HA7"], pend) + at(P["H1"][s], [first[g][n] for g, n in late[s]])
            pend = phi_q(NTILE - 1, s, proj(0, NTILE - 1, s, jobs))

        def cp_o(i, r0, nr, c0, nc):
            rows = pl.ds(pl.multiple_of(tile(i) * T + r0, 128), nr)
            return pltpu.make_async_copy(out_v.at[pl.ds(i * T + r0, nr), pl.ds(c0, nc)],
                                         out_h.at[rows, pl.ds(c0, nc)], sem.at[6])

        outs = []

        def mix(i, c, blocks):
            def job(n, t):
                def run():
                    r0, c0 = i * T + t * 128, (2 * c + n) * 128
                    g = gate_v[tile(i), t]
                    xt = _ld(x_v[pl.ds(pl.multiple_of(tile(i) * 128 + t * 64, 64), 64), c0:c0 + 128]).astype(F32)
                    upd = xt * 0.0
                    if i == NTILE - 1:
                        tok = t * 128 + lax.broadcasted_iota(I32, (128, 128), 0)
                        upd = upd + jnp.where(tok == idx % T, ffn["out"][:, c0:c0 + 128], 0.0)
                    a = after(blocks[n][t], now(P["ML"], P["MR"][2 * t + n])).T
                    res = g * a + (1.0 - g) * (xt + upd)
                    out_v[r0:r0 + 128, c0:c0 + 128] = res.astype(BF16)
                    before(res, P["DM"])
                    if i == NTILE - 1:
                        new = [cp_o(i, t * 128, 128, c * 256, 256)] if n == 1 else []
                    else:
                        new = [cp_o(i, 0, T, 0, D)] if (c, n, t) == (U - 1, 1, 1) else []
                    start(new)
                    outs.extend(new)
                return run
            return [job(n, t) for t in range(2) for n in range(2)]

        for i in range(NTILE):
            ops = o_ops(i)
            assert i < NTILE - 1 or not rest
            aj = [fn for g in range(U) for fn in attn(i + 1, g)] if i + 1 < NTILE else []
            for c in range(U):
                jobs = at(P["HM"], pend) + [(n - 7 * c, fn) for n, fn in zip(P["HT"], aj) if n // 7 == c]
                if (i, c) == (1, 0):
                    store_held()
                if (i, c) == P["W7"]:
                    jobs = sync("f2") + jobs
                    ready[0] = NF
                fj = take(P["QC"][c])
                jobs += at(P["HC"][-len(fj):], fj)
                if (i, c) == (NTILE - 1, U - 1):
                    def early(c11, c21):
                        for fn in mix(i, c, ((c11, None), (c21, None)))[:2]:
                            fn()
                    pend = mix(i, c, _combine(lambda m: mm(wa_v[3, c, m], ops[m], NN), jobs, early=early))[2:]
                else:
                    pend = mix(i, c, _combine(lambda m: mm(wa_v[3, c, m], ops[m], NN), jobs, P["OC"]))
        for fn in pend:
            fn()
        wait(outs, "w_out")
        assert not flying

    return kernel


DEFAULTS = dict(
    F0=2,
    F1=5,
    NA=12,
    W7=(0, 0),
    HS={'x1': 2, 'x': 1, 'kv': 3, 'f0': 1, 'f1': 1, 'f2': 3},
    OA=(0, 6, 5, 3, 4, 1, 2),
    OB=(0, 3, 1, 2, 4, 6, 5),
    OC=(0, 6, 5, 3, 4, 1, 2),
    PROF=False,
    FLAGS=None,
    NS=1,
    HS1=2,
    HX1=(2, 3, 4, 5),
    HK0=(0, 2, 4, 6),
    IA=(0, 1, 1, 1, 1, 1, 1, 1, 1, 1, 1, 1, 0, 1, 0, 1, 0, 1, 0, 1, 0, 1, 0),
    IB=((1, 1, 2, 1), (1, 1, 1, 1), (1, 1, 1, 1), (1, 1, 1, 1), (1, 1, 1, 1), (1, 1, 1, 1), (1, 1, 1, 1), (1, 1, 1, 1)),
    QB=((0, 0, 0, 0), (0, 0, 0, 0), (4, 6, 6, 6), (6, 6, 6, 6), (6, 6, 6, 6), (6, 6, 6, 6), (6, 6, 6, 6), (6, 6, 6, 6)),
    QC=(1, 1, 1, 1),
    QW={5: (2, 2, 2, 2), 6: (2, 2, 2, 2)},
    NK=2,
    QK={5: (1, 1, 1, 1), 6: (1, 1, 1, 1)},
    HA=(0, 2, 4, 6),
    QL=2,
    DQ=None,
    XL=3,
    DX=4,
    DR=None,
    HX=(4,),
    HX4=(1, 2, 4, 5),
    QR=((0, 4), (8, 12)),
    HA6=(0, 2, 4, 6),
    HX6=(1,),
    HX2=(3, 6),
    HW=(1, 5, 3),
    DK=None,
    DW=5,
    WL=3,
    HB=(2, (3, 6), (2, 5)),
    KVL=4,
    KR=((0, 4), (8, 12)),
    HG=(6,),
    DG=5,
    GL=2,
    HF0=(0, 2, 5),
    HF1=(1, 4, 6),
    DF=8,
    FL=1,
    HO=(2, 6),
    H0=(0, 3, 6, 6),
    H1=((), (0, 1, 2, 3, 5, 6), (1, 1, 5), (1, 1, 3)),
    HA7=(0, 0, 4, 5),
    HM=(0, 1, 4, 6),
    HT=(0, 2, 3, 3, 5, 5, 6, 7, 8, 10, 11, 11, 12, 13, 15, 15, 16, 17, 18, 21),
    HC=(6,),
    DM=4,
    ML=3,
    AL=2,
    DA=None,
    MR=(8, 0, 0, 0),
    AR=(0, 0),
    HK=(0, 4),
)


def make(**kw):
    P = dict(DEFAULTS, **kw)

    @jax.jit
    def run(A_x, A_wqkv, A_w_phi, A_wo, B_x, B_w_r, B_w_gate, B_w_up, B_w_down, gate_w):
        B, S, D = A_x.shape
        F = B_w_gate.shape[1]
        H = A_w_phi.shape[0]
        NTILE = S // 256
        G = D // 128
        any_spec = pl.BlockSpec(memory_space=pl.ANY)
        V = pltpu.VMEM
        scratch = [
            V((S // 2, D), I32),
            V((NTILE, 7, D // 4, 128), I32),
            V((3, D // 2, D), I32),
            V((4, G // 2, 7, 64, D // 2), I32),
            V((H, 32, 32), BF16),
            V((D // 2, D), I32),
            V((D,), BF16),
            V((D,), BF16),
            V((D // 2, F), I32),
            V((D // 2, F), I32),
            V((F // 2, D), I32),
            V((NTILE, G, 128, 256), I32),
            V((NTILE, 2, 128, 128), F32),
            V((H // 2, 64, 128), F32),
            V((G, 2, 128, 128), F32),
            V((D, 128), F32),
            V((S, D), BF16),
            pltpu.SemaphoreType.DMA((13,)),
        ]
        out = pl.pallas_call(
            _make_kernel(S, D, F, H, P),
            out_shape=jax.ShapeDtypeStruct((S, D), A_x.dtype),
            in_specs=[any_spec] * 9,
            out_specs=any_spec,
            scratch_shapes=scratch,
            compiler_params=pltpu.CompilerParams(vmem_limit_bytes=110 * 2**20, flags=P["FLAGS"]),
        )(A_x.reshape(S, D), A_wqkv, A_w_phi, A_wo, B_w_r, B_w_gate, B_w_up, B_w_down, gate_w)
        return out.reshape(B, S, D)
    return run


_run = make()


@jax.jit
def pallas_gated_mix__linear_kernel_hedgehog__moe_arch_mod__prompt_kernel(
    A_x, A_wqkv, A_w_phi, A_wo, B_x, B_w_r, B_w_gate, B_w_up, B_w_down, gate_w
):
    return _run(A_x, A_wqkv, A_w_phi, A_wo, B_x, B_w_r, B_w_gate, B_w_up, B_w_down, gate_w)
```

```python
import jax
import jax.numpy as jnp
from jax import lax
import jax.experimental.pallas as pl
import jax.experimental.pallas.tpu as pltpu

F32 = jnp.float32
BF16 = jnp.bfloat16
I32 = jnp.int32
LOG2E = 1.4426950408889634
NT = (((1,), (1,)), ((), ()))
NN = (((1,), (0,)), ((), ()))
T = 256

_PLACE = dict(
    order_q=(0, 6, 5, 3, 4, 1, 2), order_kv=(0, 3, 1, 2, 4, 6, 5), order_o=(0, 6, 5, 3, 4, 1, 2),
    wait=dict(x1=2, x=1, kv=3, f0=1, f1=1, f2=3),
    issue_a=(0, 1, 1, 1, 1, 1, 1, 1, 1, 1, 1, 1, 0, 1, 0, 1, 0, 1, 0, 1, 0, 1, 0),
    issue_b=((1, 1, 2, 1),) + ((1, 1, 1, 1),) * 7,
    phi_q=(0, 2, 4, 6), phi_q_last=(0, 0, 4, 5), phi_q_lag=2, phi_rows=((0, 4), (8, 12)),
    x1=(2, 3, 4, 5), x2=(1, 2, 4, 5), x_early=(4,), x_half=(3, 6), x_late=(1,), x_lag=3, x_due=4,
    fold_q=(0, 2, 4, 6), fold_k=(0,), prep_v=(1, 5), prep_o=(2, 6), w_lag=3, w_due=5,
    kv_v=(3, 6), kv_k=(2, 5), kv_lag=4, gate=(6,), gate_lag=2, gate_due=5,
    ffn_jobs=((0,) * 4, (0,) * 4, (4, 6, 6, 6)) + ((6,) * 4,) * 5,
    ffn_v=(0, 2, 5), ffn_k=(1, 4, 6), ffn_c=(6,), ffn_lag=1, ffn_due=8,
    attn_b=(0, 2, 3, 5, 6), attn_a=((5, 7, 9, 11, 13), (15, 17, 19, 21, 23)),
    mix=(0, 1, 4, 6), mix_lag=3, mix_rows=(8, 0, 0, 0), mix_due=4, attn_lag=2,
    attn=(0, 2, 3, 3, 5, 5, 6, 7, 8, 10, 11, 11, 12, 13, 15, 15, 16, 17, 18, 21),
)


def _bf16(words):
    return pltpu.bitcast(words, BF16)


def _pack(a, b):
    return pltpu.bitcast(pltpu.pack_elementwise([a, b], packed_dtype=BF16), I32)


def _unpack(w, k):
    return pltpu.unpack_elementwise(w, index=k, packed_dtype=BF16, unpacked_dtype=F32)


def _tree(vs, op):
    while len(vs) > 1:
        vs = [op(vs[k], vs[k + 1]) if k + 1 < len(vs) else vs[k] for k in range(0, len(vs), 2)]
    return vs[0]


def _left(a11, a12, a21, a22):
    return [a11 + a22, a21 + a22, a11, a22, a11 + a12, a21 - a11, a12 - a22]


def _right(b11, b12, b21, b22):
    return [b11 + b22, b11, b12 - b22, b21 - b11, b22, b11 + b12, b21 + b22]


_USES = (((0, 1), (3, 1)), ((2, 1), (3, -1)), ((1, 1), (3, 1)), ((0, 1), (2, 1)),
         ((0, -1), (1, 1)), ((3, 1),), ((0, 1),))


def _combine(mul, jobs, order, early=None):
    c = [None] * 4
    for n, m in enumerate(order):
        if early and n == 6:
            assert m == 2
            early(c[0], c[2])
        t = mul(m)
        for k, sign in _USES[m]:
            if c[k] is None:
                c[k] = t if sign > 0 else -t
            else:
                c[k] = c[k] + t if sign > 0 else c[k] - t
        for slot, fn in jobs:
            if slot == n:
                fn()
    return (c[0], c[1]), (c[2], c[3])


def _at(slots, jobs):
    assert len(jobs) <= len(slots)
    return list(zip(slots, jobs))


def _run(jobs):
    for fn in jobs:
        fn()


def _per_head(v, op):
    r = _tree([v[k] for k in range(v.shape[0])], op)
    r = op(r, pltpu.roll(r, 4, 0))
    return op(r, pltpu.roll(r, 2, 0))


def _rcp(s):
    r = pltpu.reciprocal(s, approx=True)
    return r * (2.0 - s * r)


def _phi(p, tie):
    p = p.reshape(8, 8, 128)
    ep = jnp.exp2(p - tie(_per_head(p, jnp.maximum), 0))
    en = jnp.exp2(tie(_per_head(p, jnp.minimum), 1) - p)
    ep = ep * _rcp(_per_head(ep, jnp.add))
    en = en * _rcp(_per_head(en, jnp.add))
    return ep.reshape(64, 128), en.reshape(64, 128)


def _make_kernel(S, D, F, H, P):
    NTILE = S // T
    G = D // 128
    U = G // 2
    K2 = D // 2
    NF = F // 128
    NA = 12
    assert (NTILE, U, NF, H) == (8, 4, 28, 32)

    def kernel(ax_h, wqkv_h, wphi_h, wo_h, wr_h, wg_h, wu_h, wd_h, gw_h, out_h,
               x_v, xs_v, w_v, wa_v, wphi_v, wo_v, wr_v, gw_v, wg_v, wu_v, wd_v,
               pq_v, gate_v, kv_v, z_v, xb_v, out_v, sem):
        ax_h, wqkv_h, wo_h, wg_h, wu_h, wd_h = [r.bitcast(I32) for r in (ax_h, wqkv_h, wo_h, wg_h, wu_h, wd_h)]

        def cp(src, dst, s):
            return pltpu.make_async_copy(src, dst, sem.at[s])

        def cp_rows(src, dst, n, s):
            return cp(src.at[pl.ds(n * 128, 128)], dst.at[pl.ds(n * 128, 128)], s)

        def cp_q(u, s):
            return cp(wqkv_h.at[:, pl.ds(u * 256, 256)], w_v.at[0, :, pl.ds(u * 256, 256)], s)

        def cp_phi(u, s):
            return cp(wphi_h.at[pl.ds(u * 8, 8)], wphi_v.at[pl.ds(u * 8, 8)], s)

        def cp_slab(f, s):
            cols, rows = pl.ds(f * 128, 128), pl.ds(f * 64, 64)
            return [cp(wg_h.at[:, cols], wg_v.at[:, cols], s), cp(wu_h.at[:, cols], wu_v.at[:, cols], s),
                    cp(wd_h.at[rows], wd_v.at[rows], s)]

        batch = {
            "small": [[cp(wr_h, wr_v, 0), cp(gw_h, gw_v, 0), cp_phi(0, 0)]],
            "q0": [[cp_q(0, 1)]],
            "x0": [[cp_rows(ax_h, x_v, 0, 2)]],
            "q1": [[cp_q(1, 3), cp_phi(1, 3)]],
            "x1": [[cp_rows(ax_h, x_v, 1, 4)]],
            "q2": [[cp_q(u, 5), cp_phi(u, 5)] for u in (2, 3)],
            "x": [[cp_rows(ax_h, x_v, i, 6) for i in (2, 3, 4)]],
            "kv": [[cp_rows(ax_h, x_v, i, 7)] for i in (5, 6, 7)]
                  + [[cp_rows(wqkv_h.at[:, pl.ds(j * D, D)], w_v.at[j], n, 7)] for j in (2, 1) for n in range(U)],
            "f0": [cp_slab(f, 8) for f in range(NA)],
            "f1": [[cp_rows(wo_h, wo_v, n, 9)] + cp_slab(NA + n, 9) for n in range(U)]
                  + [cp_slab(f, 9) for f in range(NA + U, 2 * NA)],
            "f2": [cp_slab(f, 10) for f in range(2 * NA, NF)],
        }
        queue = [ds for name in batch for ds in batch[name]]
        flying = []
        arrived = []

        def start(ds):
            for d in ds:
                d.start()
                flying.append(d)

        def wait(ds):
            for d in ds:
                assert any(d is e for e in flying)
                flying[:] = [e for e in flying if e is not d]
                d.wait()

        def issue(n):
            for ds in queue[:n]:
                start(ds)
            del queue[:n]

        def arrive(name, then=0):
            wait([d for ds in batch[name] for d in ds])
            arrived.append(name)
            issue(then)

        def sync(name, then=0):
            return [(P["wait"][name], lambda: arrive(name, then))]

        issue(3)
        kv_v[...] = jnp.zeros_like(kv_v)
        z_v[...] = jnp.zeros_like(z_v)
        r128 = lax.broadcasted_iota(I32, (128, 128), 0)
        c128 = lax.broadcasted_iota(I32, (128, 128), 1)
        diag = (2 * ((r128 % 64) // 32) + r128 // 64) == (c128 // 32)
        eye = jnp.where(lax.broadcasted_iota(I32, (128, 32), 0) % 32 == lax.broadcasted_iota(I32, (128, 32), 1),
                        1.0, 0.0).astype(BF16)
        arrive("small")
        gw = gw_v[...].astype(F32).reshape(1, D)
        wr = wr_v[...].astype(F32).reshape(1, D)

        never = lax.broadcasted_iota(I32, (8, 128), 0) > (pltpu.bitcast(gw[:, 0:128], I32) & 0xFFFF) + 8
        clock = []
        due = {}

        def after(w, dep, every=False):
            if dep is None:
                return w
            dep = pltpu.bitcast(dep, w.dtype)
            if every:
                return jnp.concatenate([jnp.where(never, dep, w[r:r + 8]) for r in range(0, w.shape[0], 8)], axis=0)
            w0 = jnp.where(never, dep, w[0:8, 0:128])
            if w.shape[1] > 128:
                w0 = jnp.concatenate([w0, w[0:8, 128:]], axis=1)
            return jnp.concatenate([w0, w[8:]], axis=0) if w.shape[0] > 8 else w0

        def now(back, row=0):
            if len(clock) < back:
                return None
            t = clock[-back]
            row = row * 8 % t.shape[0]
            return t[row:row + 8, 0:128]

        def before(v, ahead):
            v = pltpu.bitcast(v, I32)
            parts = [v[r:r + 8, c:c + 128] for r in range(0, v.shape[0], 8) for c in range(0, v.shape[1], 128)]
            due.setdefault(len(clock) + ahead, []).append(_tree(parts, jnp.bitwise_or))

        def mm(w, rhs, dims):
            deps = due.pop(len(clock), [])
            if deps:
                w = after(w, _tree(deps, jnp.bitwise_or))
            t = lax.dot_general(_bf16(w), rhs, dims, preferred_element_type=F32)
            clock.append(t)
            return t

        bd = {}

        def prep_phi(groups):
            for g in groups:
                wp = wphi_v[pl.ds(4 * g, 4)].reshape(128, 32)
                t = lax.dot_general(eye, wp, NT, preferred_element_type=F32)
                bd[g] = pltpu.bitcast(jnp.where(diag, t, 0.0).astype(BF16), I32)

        def fold(j, s, n):
            def job(lo, hi):
                def run():
                    assert ("q%d" % min(s, 2) if j == 0 else "kv") in arrived
                    blocks = [mm(bd[g], _bf16(w_v[j, (k * K2 + lo) // 2:(k * K2 + hi) // 2, g * 128:(g + 1) * 128]), NT)
                              * LOG2E for g in (2 * s, 2 * s + 1) for k in range(2)]
                    for m, t in enumerate(_left(*blocks)):
                        wa_v[j, s, m, :, lo:hi] = _pack(t[0:64], t[64:128])
                return run
            return [job(c * K2 // n, (c + 1) * K2 // n) for c in range(n)]

        def prep_w(j, ref, s):
            def job(c):
                def run():
                    assert ("kv" if j == 2 else "f1") in arrived
                    rows = (c, U + c) if j == 2 else (2 * c, 2 * c + 1)
                    blocks = [pltpu.bitcast(_bf16(after(ref[r * 64:(r + 1) * 64, g * 128:(g + 1) * 128],
                                                        now(P["w_lag"]))).T, I32)
                              for g in (2 * s, 2 * s + 1) for r in rows]
                    lo, hi = [_left(*[_unpack(w, e) for w in blocks]) for e in range(2)]
                    for m in range(7):
                        w = blocks[0] if m == 2 else blocks[3] if m == 3 else _pack(lo[m], hi[m])
                        wa_v[j, s, m, :, c * 128:(c + 1) * 128] = w
                        if m not in (2, 3):
                            before(w, P["w_due"])
                return run
            return [job(c) for c in range(U)]

        def x_block(i, t, lo, n):
            return x_v[(2 * i + t) * 64:(2 * i + t + 1) * 64, lo:lo + n]

        route = [jnp.full((8, 1), -jnp.inf, F32), jnp.zeros((8, 1), I32)]
        first_x = [[] for _ in range(7)]

        def prep_x(i):
            acc = {}

            def job(c):
                def run():
                    assert ("x%d" % i if i < 2 else "x" if i < 5 else "kv") in arrived
                    c1, c2 = c * 128, K2 + c * 128
                    words = [after(x_block(i, 0, c1, 128), now(P["x_lag"]), True), x_block(i, 1, c1, 128),
                             x_block(i, 0, c2, 128), after(x_block(i, 1, c2, 128), now(P["x_lag"]), True)]
                    vals = [[_unpack(w, e) for w in words] for e in range(2)]
                    lo, hi = [_right(*v) for v in vals]
                    for m in range(7):
                        t = words[0] if m == 1 else words[3] if m == 4 else _pack(lo[m], hi[m])
                        if i == 0:
                            first_x[m].append(t)
                        else:
                            w = pltpu.bitcast(_bf16(t).T, I32)
                            xs_v[i, m, c * 64:(c + 1) * 64, :] = w
                            before(w[0:8], P["x_due"])
                    for t in range(2):
                        for e in range(2):
                            part = vals[e][t] * wr[:, c1:c1 + 128] + vals[e][2 + t] * wr[:, c2:c2 + 128]
                            acc[t, e] = part if c == 0 else acc[t, e] + part
                    if c < U - 1:
                        return
                    tok = i * T + 2 * lax.broadcasted_iota(I32, (8, 1), 0)
                    found = [tuple(route)]
                    for t in range(2):
                        rs = [jnp.sum(acc[t, e], axis=1, keepdims=True).astype(BF16).astype(F32) for e in range(2)]
                        rs = [jnp.where(r != r, -jnp.inf, r) for r in rs]
                        found += [(rs[e][8 * k:8 * k + 8], tok + (t * 128 + 16 * k + e))
                                  for k in range(8) for e in range(2)]
                    route[:] = _tree(found, lambda a, b: (jnp.maximum(a[0], b[0]), jnp.where(b[0] > a[0], b[1], a[1])))
                return run
            return [job(c) for c in range(U)]

        def proj(j, i, s, jobs):
            if i == 0:
                ops = [x_block(0, 0, 0, K2) if m == 1 else x_block(0, 1, K2, K2) if m == 4
                       else jnp.concatenate(first_x[m], axis=1) for m in range(7)]
                order = (1, 4, 0, 6, 5, 3, 2) if (j, s) == (0, 0) else P["order_q"]
                return _combine(lambda m: mm(wa_v[j, s, m], _bf16(ops[m]), NT), jobs, order)
            ops = [xs_v[i, m] for m in range(7)]
            return _combine(lambda m: mm(wa_v[j, s, m], _bf16(ops[m]), NN), jobs,
                            P["order_q"] if j == 0 else P["order_kv"])

        held = []

        def store_held():
            while held:
                where, val = held.pop(0)
                pq_v[where] = val

        def phi_q(i, s, ps):
            def job(e, q):
                def run():
                    rows = slice(q * 64, (q + 1) * 64)
                    for t in range(2):
                        phi = _phi(ps[e][t][rows], lambda v, k: after(v, now(P["phi_q_lag"], P["phi_rows"][t][k])))
                        held.append(((i, 2 * s + e, rows, slice(t * 128, (t + 1) * 128)), _pack(*phi)))
                    if i < NTILE - 1:
                        store_held()
                return run
            return [job(e, q) for e in range(2) for q in range(2)]

        prep_phi(range(2))
        arrive("q0", 1)
        _run(fold(0, 0, U))
        arrive("x0", 1)
        _run(prep_x(0))
        pv = [fn for s in range(U) for fn in prep_w(2, w_v.at[2], s)]
        pk = [fn for s in range(U) for fn in fold(1, s, 2)]
        px = [prep_x(i) for i in range(NTILE)]
        units = [(0, 0), (0, 1), (1, 0), (1, 1), (0, 2), (1, 2), (0, 3), (1, 3)]
        units += [(i, s) for i in range(2, NTILE - 1) for s in range(U)]
        pend = []
        for n, (i, s) in enumerate(units):
            jobs = []
            if n == 1:
                arrive("q1", 1)
                prep_phi(range(2, 4))
                _run(fold(0, 1, U))
                jobs += sync("x1", 2) + _at(P["x1"], px[1])
            elif n == 4:
                arrive("q2", 1)
                prep_phi(range(4, G))
                _run(fold(0, 2, U))
                jobs += _at(P["fold_q"], fold(0, 3, U))
            elif n > 4:
                issue(P["issue_a"][n - 5])
            if n == 7:
                jobs += sync("x") + _at(P["x2"], px[2])
            elif i in (2, 3):
                jobs += _at(P["x_early"], px[i + 1][s:s + 1])
            elif i == 4 and s >= 2:
                jobs += (sync("kv") if s == 2 else []) + _at(P["x_half"], px[5][2 * (s - 2):2 * (s - 1)])
            elif i > 4:
                k = (i - 5) * U + s
                jobs += (_at(P["x_late"], px[i + 1][s:s + 1]) + _at(P["prep_v"], pv[2 * k:2 * k + 2])
                         + _at(P["fold_k"], pk[k:k + 1]))
            pend = phi_q(i, s, proj(0, i, s, jobs + _at(P["phi_q"], pend)))

        top = jnp.max(route[0], axis=0, keepdims=True)
        idx = jnp.clip(jnp.min(jnp.where(route[0] == top, route[1], S)), 0, S - 1)
        blk = _bf16(x_v[pl.ds(pl.multiple_of((idx // 16) * 8, 8), 8), :]).astype(F32)
        sel = lax.broadcasted_iota(I32, (16, D), 0) == (idx % 16)
        xs = jnp.sum(jnp.where(sel, blk, 0.0), axis=0, keepdims=True)
        r_gate = jax.nn.sigmoid(jnp.sum(xs * wr, axis=1, keepdims=True).astype(BF16).astype(F32))

        def spread_token():
            for g in range(G):
                xb_v[g * 128:(g + 1) * 128, :] = after(
                    jnp.broadcast_to(xs[:, g * 128:(g + 1) * 128], (128, 128)), now(1)).T

        def tile(i):
            return idx // T if i == NTILE - 1 else i + (idx // T <= i).astype(I32)

        ffn = {"y": [jnp.zeros((8, K2), F32)] * 2}

        def ffn_up(f, k):
            def run():
                assert "f%d" % (f // NA) in arrived
                xb = after(xb_v[k * 256:(k + 1) * 256, :], now(P["ffn_lag"]))
                for name, w_ref in (("g", wg_v), ("u", wu_v)):
                    w = _bf16(w_ref[k * 128:(k + 1) * 128, f * 128:(f + 1) * 128]).astype(F32)
                    t = jnp.sum((w * xb).reshape(32, 8, 128), axis=0)
                    ffn[name, f, k] = t if k == 0 else ffn[name, f, k - 1] + t
                    before(ffn[name, f, k], P["ffn_due"])
                if k == 3:
                    g, u = [jnp.sum(ffn[name, f, k], axis=0, keepdims=True) for name in "gu"]
                    ffn["h", f] = jnp.broadcast_to(g * jax.nn.sigmoid(g) * u, (128, 128)).T
            return run

        def ffn_down(f, n):
            def run():
                w = _bf16(wd_v[f * 64:(f + 1) * 64, n * K2:(n + 1) * K2]).astype(F32)
                hb = jnp.concatenate([after(ffn["h", f], now(P["ffn_lag"]))] * U, axis=1)
                ffn["y"][n] = ffn["y"][n] + jnp.sum((w * hb).reshape(16, 8, K2), axis=0)
                ffn["done", f, n] = True
                before(ffn["y"][n], P["ffn_due"])
            return run

        def ffn_finish():
            assert all(("done", f, n) in ffn for f in range(NF) for n in range(2))
            ffn["out"] = jnp.sum(jnp.concatenate(ffn["y"], axis=1), axis=0, keepdims=True) * r_gate

        ffn_left = [fn for f in range(NF) for fn in [ffn_up(f, k) for k in range(4)] + [ffn_down(f, n) for n in range(2)]]
        ffn_left.append(ffn_finish)

        def take(n):
            got, ffn_left[:] = ffn_left[:n], ffn_left[n:]
            return got

        def gates(i):
            def job(t, r0):
                def run():
                    lo = (i * T + t * 128 + r0) // 2
                    xt = _bf16(after(x_v[lo:lo + 32, :], now(P["gate_lag"]))).astype(F32)
                    gate = jnp.broadcast_to(jax.nn.sigmoid(jnp.sum(xt * gw, axis=1, keepdims=True)), (64, 128))
                    gate_v[i, t, r0:r0 + 64, :] = gate
                    before(gate, P["gate_due"])
                return run
            return [job(t, r0) for t in range(2) for r0 in (0, 64)]

        kr = lax.broadcasted_iota(I32, (64, 128), 0)
        kc = lax.broadcasted_iota(I32, (64, 128), 1)
        same_head = (kr // 32) == ((kc // 2) % 2)
        kvb = {}

        def kv_step(i, s, ps, vs):
            def job(e, q):
                def run():
                    g = 2 * s + e
                    j = 2 * g + q
                    rows = slice(q * 64, (q + 1) * 64)
                    phis = [_phi(ps[e][t][rows], lambda v, k: after(v, now(P["kv_lag"], P["phi_rows"][t][k])))
                            for t in range(2)]
                    zs = [z_v[g, sign, rows] + (phis[0][sign] + phis[1][sign]) for sign in range(2)]
                    phi = jnp.concatenate([_pack(*ph) for ph in phis], axis=1)
                    kv_v[j] += mm(vs[2 * e + q], _bf16(phi), NT)
                    if i == NTILE - 1:
                        zs = [jnp.broadcast_to(jnp.sum(z, axis=1, keepdims=True), (64, 128)) for z in zs]
                        t = jnp.concatenate([kv_v[j, pl.ds(h, 32, stride=2), :] for h in range(2)], axis=0)
                        kvb[j] = pltpu.bitcast(jnp.where(same_head, t, 0.0).astype(BF16), I32)
                    for sign in range(2):
                        z_v[g, sign, rows] = zs[sign]
                return run
            return [job(e, q) for e in range(2) for q in range(2)]

        o_pairs, o_parts = {}, {}

        def attn(i, g):
            def pair(h, q):
                def run():
                    rows = slice(q * 64, (q + 1) * 64)
                    w = pq_v[tile(i), h, rows]
                    den = (_unpack(w, 0) * jnp.concatenate([after(z_v[h, 0, rows], now(P["attn_lag"]))] * 2, axis=1)
                           + _unpack(w, 1) * jnp.concatenate([z_v[h, 1, rows]] * 2, axis=1))
                    rden = 1.0 / (_per_head(den.reshape(8, 8, T), jnp.add) + 1e-6)
                    num = mm(kvb[2 * h + q], _bf16(w), NN)
                    o_pairs[i, h, q] = [num[0:32] * rden[0:1], num[32:64] * rden[1:2]]
                return run

            def join():
                a, b = [jnp.concatenate(o_pairs.pop((i, h, 0)) + o_pairs.pop((i, h, 1)), axis=0)
                        for h in (2 * g, 2 * g + 1)]
                o_parts[i, g] = _right(a[:, :128], a[:, 128:], b[:, :128], b[:, 128:])

            return [pair(h, q) for h in (2 * g, 2 * g + 1) for q in range(2)] + [join]

        first = [attn(0, g) for g in range(U)]
        po = [fn for s in range(U) for fn in prep_w(3, wo_v, s)]
        for i in range(NTILE):
            gj = gates(i)
            for s in range(U):
                fj = [spread_token] if (i, s) == (0, 0) else take(P["ffn_jobs"][i][s])
                issue(P["issue_b"][i][s])
                half = len(fj) // 2
                jobs = sync("f0") if (i, s) == (2, 0) else sync("f1") if (i, s) == (5, 0) else []
                jobs += (_at(P["kv_v"], pend[:2]) + _at(P["ffn_v"][3 - half:], fj[:half]) + _at(P["gate"], gj[s:s + 1]))
                vt = proj(2, i, s, jobs)
                vs = [jnp.concatenate([_pack(b[q * 64:q * 64 + 32], b[q * 64 + 32:q * 64 + 64]) for b in vt[e]], axis=1)
                      for e in range(2) for q in range(2)]
                jobs = _at(P["kv_k"], pend[2:]) + _at(P["ffn_k"], fj[half:])
                if i in (5, 6):
                    k = (i - 5) * U + s
                    jobs += _at(P["prep_o"], po[2 * k:2 * k + 2])
                if i == NTILE - 1 and s >= 2:
                    jobs += _at(P["attn_b"], first[s - 2])
                pend = kv_step(i, s, proj(1, i, s, jobs), vs)

        for s in range(U):
            jobs = _at(P["phi_q_last"], pend)
            for g in range(2, U):
                jobs += [(n - 7 * s, fn) for n, fn in _at(P["attn_a"][g - 2], first[g]) if n // 7 == s]
            pend = phi_q(NTILE - 1, s, proj(0, NTILE - 1, s, jobs))

        outs = []

        def store_out(i, r0, nr, c0, nc):
            rows = pl.ds(pl.multiple_of(tile(i) * T + r0, 128), nr)
            outs.append(cp(out_v.at[pl.ds(i * T + r0, nr), pl.ds(c0, nc)], out_h.at[rows, pl.ds(c0, nc)], 11))
            start(outs[-1:])

        def mix(i, c, blocks):
            def job(n, t):
                def run():
                    r0, c0 = i * T + t * 128, (2 * c + n) * 128
                    g = gate_v[tile(i), t]
                    xt = _bf16(x_v[pl.ds(pl.multiple_of(tile(i) * 128 + t * 64, 64), 64), c0:c0 + 128]).astype(F32)
                    upd = xt * 0.0
                    if i == NTILE - 1:
                        tok = t * 128 + lax.broadcasted_iota(I32, (128, 128), 0)
                        upd = upd + jnp.where(tok == idx % T, ffn["out"][:, c0:c0 + 128], 0.0)
                    a = after(blocks[n][t], now(P["mix_lag"], P["mix_rows"][2 * t + n])).T
                    res = g * a + (1.0 - g) * (xt + upd)
                    out_v[r0:r0 + 128, c0:c0 + 128] = res.astype(BF16)
                    before(res, P["mix_due"])
                    if i == NTILE - 1:
                        if n == 1:
                            store_out(i, t * 128, 128, c * 256, 256)
                    elif (c, n, t) == (U - 1, 1, 1):
                        store_out(i, 0, T, 0, D)
                return run
            return [job(n, t) for t in range(2) for n in range(2)]

        assert list(P["mix"]) == sorted(P["mix"])
        for i in range(NTILE):
            parts = [o_parts.pop((i, g)) for g in range(U)]
            ops = [jnp.concatenate([p[m] for p in parts], axis=0).astype(BF16) for m in range(7)]
            aj = [fn for g in range(U) for fn in attn(i + 1, g)] if i + 1 < NTILE else []
            for c in range(U):
                if (i, c) == (1, 0):
                    store_held()
                jobs = (sync("f2") if (i, c) == (0, 0) else []) + _at(P["mix"], pend)
                jobs += [(n - 7 * c, fn) for n, fn in _at(P["attn"], aj) if n // 7 == c] + _at(P["ffn_c"], take(1))
                last = (i, c) == (NTILE - 1, U - 1)
                early = (lambda c11, c21: _run(mix(i, c, ((c11, None), (c21, None)))[:2])) if last else None
                pend = mix(i, c, _combine(lambda m: mm(wa_v[3, c, m], ops[m], NN), jobs, P["order_o"], early))
        _run(pend[2:])
        wait(outs)
        assert not (flying or queue or held or ffn_left)

    return kernel


def _build(P):
    def run(A_x, A_wqkv, A_w_phi, A_wo, B_x, B_w_r, B_w_gate, B_w_up, B_w_down, gate_w):
        B, S, D = A_x.shape
        F = B_w_gate.shape[1]
        H = A_w_phi.shape[0]
        NTILE, G = S // T, D // 128
        hbm = pl.BlockSpec(memory_space=pl.ANY)
        V = pltpu.VMEM
        scratch = [
            V((S // 2, D), I32),
            V((NTILE, 7, D // 4, 128), I32),
            V((3, D // 2, D), I32),
            V((4, G // 2, 7, 64, D // 2), I32),
            V((H, 32, 32), BF16),
            V((D // 2, D), I32),
            V((D,), BF16),
            V((D,), BF16),
            V((D // 2, F), I32),
            V((D // 2, F), I32),
            V((F // 2, D), I32),
            V((NTILE, G, 128, T), I32),
            V((NTILE, 2, 128, 128), F32),
            V((H // 2, 64, 128), F32),
            V((G, 2, 128, 128), F32),
            V((D, 128), F32),
            V((S, D), BF16),
            pltpu.SemaphoreType.DMA((12,)),
        ]
        out = pl.pallas_call(
            _make_kernel(S, D, F, H, P),
            out_shape=jax.ShapeDtypeStruct((S, D), BF16),
            in_specs=[hbm] * 9,
            out_specs=hbm,
            scratch_shapes=scratch,
            compiler_params=pltpu.CompilerParams(vmem_limit_bytes=110 * 2**20),
        )(A_x.reshape(S, D), A_wqkv, A_w_phi, A_wo, B_w_r, B_w_gate, B_w_up, B_w_down, gate_w)
        return out.reshape(B, S, D)
    return run


@jax.jit
def pallas_gated_mix__linear_kernel_hedgehog__moe_arch_mod__prompt_kernel(
    A_x: jax.Array,
    A_wqkv: jax.Array,
    A_w_phi: jax.Array,
    A_wo: jax.Array,
    B_x: jax.Array,
    B_w_r: jax.Array,
    B_w_gate: jax.Array,
    B_w_up: jax.Array,
    B_w_down: jax.Array,
    gate_w: jax.Array,
):
    return _build(_PLACE)(A_x, A_wqkv, A_w_phi, A_wo, B_x, B_w_r, B_w_gate, B_w_up, B_w_down, gate_w)
```

```python
import jax
import jax.numpy as jnp
from jax import lax
import jax.experimental.pallas as pl
import jax.experimental.pallas.tpu as pltpu

F32 = jnp.float32
BF16 = jnp.bfloat16
I32 = jnp.int32
LOG2E = 1.4426950408889634
NT = (((1,), (1,)), ((), ()))
NN = (((1,), (0,)), ((), ()))
T = 256

_PLACE = dict(
    order_q=(0, 6, 5, 3, 4, 1, 2), order_kv=(0, 3, 1, 2, 4, 6, 5), order_o=(0, 6, 5, 3, 4, 1, 2),
    wait=dict(x1=2, x=1, kv=3, f0=1, f1=1, f2=3),
    issue_a=(0, 1, 1, 1, 1, 1, 1, 1, 1, 1, 1, 1, 0, 1, 0, 1, 0, 1, 0, 1, 0, 1, 0),
    issue_b=((1, 1, 2, 1),) + ((1, 1, 1, 1),) * 7,
    phi_q=(0, 2, 4, 6), phi_q_last=(0, 0, 4, 5), phi_q_lag=2, phi_rows=((0, 4), (8, 12)),
    x1=(2, 3, 4, 5), x2=(1, 3, 4, 5), x_early=(4,), x_half=(3, 5), x_late=(1,), x_lag=3, x_due=4,
    fold_q=(0, 2, 4, 6), fold_k=(0,), prep_v=(1, 5), prep_o=(2, 6), w_lag=2, w_due=5,
    kv_v=(3, 6), kv_k=(2, 5), kv_lag=4, gate=((5,), (6,)), gate_lag=(3, 2), gate_due=(9, 5),
    ffn_jobs=((0,) * 4, (0,) * 4, (4, 6, 6, 6)) + ((6,) * 4,) * 5,
    ffn_v=(0, 2, 5), ffn_k=(1, 4, 6), ffn_c=(6,), ffn_lag=1, ffn_due=8,
    attn_b=(0, 2, 3, 5, 6), attn_a=((5, 7, 9, 11, 13), (15, 17, 19, 21, 23)),
    mix=(0, 1, 4, 6), mix_lag=3, mix_rows=(8, 0, 12, 8), mix_due=4, attn_lag=2,
    attn=(0, 2, 2, 3, 5, 5, 6, 7, 8, 10, 11, 11, 12, 13, 15, 15, 16, 17, 18, 21),
)


def _bf16(words):
    return pltpu.bitcast(words, BF16)


def _pack(a, b):
    return pltpu.bitcast(pltpu.pack_elementwise([a, b], packed_dtype=BF16), I32)


def _unpack(w, k):
    return pltpu.unpack_elementwise(w, index=k, packed_dtype=BF16, unpacked_dtype=F32)


def _tree(vs, op):
    while len(vs) > 1:
        vs = [op(vs[k], vs[k + 1]) if k + 1 < len(vs) else vs[k] for k in range(0, len(vs), 2)]
    return vs[0]


def _left(a11, a12, a21, a22):
    return [a11 + a22, a21 + a22, a11, a22, a11 + a12, a21 - a11, a12 - a22]


def _right(b11, b12, b21, b22):
    return [b11 + b22, b11, b12 - b22, b21 - b11, b22, b11 + b12, b21 + b22]


_USES = (((0, 1), (3, 1)), ((2, 1), (3, -1)), ((1, 1), (3, 1)), ((0, 1), (2, 1)),
         ((0, -1), (1, 1)), ((3, 1),), ((0, 1),))


def _combine(mul, jobs, order, early=None):
    c = [None] * 4
    for n, m in enumerate(order):
        if early and n == 6:
            assert m == 2
            early(c[0], c[2])
        t = mul(m)
        for k, sign in _USES[m]:
            if c[k] is None:
                c[k] = t if sign > 0 else -t
            else:
                c[k] = c[k] + t if sign > 0 else c[k] - t
        for slot, fn in jobs:
            if slot == n:
                fn()
    return (c[0], c[1]), (c[2], c[3])


def _at(slots, jobs):
    assert len(jobs) <= len(slots)
    return list(zip(slots, jobs))


def _run(jobs):
    for fn in jobs:
        fn()


def _per_head(v, op):
    r = _tree([v[k] for k in range(v.shape[0])], op)
    r = op(r, pltpu.roll(r, 4, 0))
    return op(r, pltpu.roll(r, 2, 0))


def _rcp(s):
    r = pltpu.reciprocal(s, approx=True)
    return r * (2.0 - s * r)


def _phi(p, tie):
    p = p.reshape(8, 8, 128)
    ep = jnp.exp2(p - tie(_per_head(p, jnp.maximum), 0))
    en = jnp.exp2(tie(_per_head(p, jnp.minimum), 1) - p)
    ep = ep * _rcp(_per_head(ep, jnp.add))
    en = en * _rcp(_per_head(en, jnp.add))
    return ep.reshape(64, 128), en.reshape(64, 128)


def _make_kernel(S, D, F, H, P):
    NTILE = S // T
    G = D // 128
    U = G // 2
    K2 = D // 2
    NF = F // 128
    NA = 12
    assert (NTILE, U, NF, H) == (8, 4, 28, 32)

    def kernel(ax_h, wqkv_h, wphi_h, wo_h, wr_h, wg_h, wu_h, wd_h, gw_h, out_h,
               x_v, xs_v, w_v, wa_v, wphi_v, wo_v, wr_v, gw_v, wg_v, wu_v, wd_v,
               pq_v, gate_v, kv_v, z_v, xb_v, out_v, sem):
        ax_h, wqkv_h, wo_h, wg_h, wu_h, wd_h = [r.bitcast(I32) for r in (ax_h, wqkv_h, wo_h, wg_h, wu_h, wd_h)]

        def cp(src, dst, s):
            return pltpu.make_async_copy(src, dst, sem.at[s])

        def cp_rows(src, dst, n, s):
            return cp(src.at[pl.ds(n * 128, 128)], dst.at[pl.ds(n * 128, 128)], s)

        def cp_q(u, s):
            return cp(wqkv_h.at[:, pl.ds(u * 256, 256)], w_v.at[0, :, pl.ds(u * 256, 256)], s)

        def cp_phi(u, s):
            return cp(wphi_h.at[pl.ds(u * 8, 8)], wphi_v.at[pl.ds(u * 8, 8)], s)

        def cp_slab(f, s):
            cols, rows = pl.ds(f * 128, 128), pl.ds(f * 64, 64)
            return [cp(wg_h.at[:, cols], wg_v.at[:, cols], s), cp(wu_h.at[:, cols], wu_v.at[:, cols], s),
                    cp(wd_h.at[rows], wd_v.at[rows], s)]

        batch = {
            "small": [[cp(wr_h, wr_v, 0), cp(gw_h, gw_v, 0), cp_phi(0, 0)]],
            "q0": [[cp_q(0, 1)]],
            "x0": [[cp_rows(ax_h, x_v, 0, 2)]],
            "q1": [[cp_q(1, 3), cp_phi(1, 3)]],
            "x1": [[cp_rows(ax_h, x_v, 1, 4)]],
            "q2": [[cp_q(u, 5), cp_phi(u, 5)] for u in (2, 3)],
            "x": [[cp_rows(ax_h, x_v, i, 6) for i in (2, 3, 4)]],
            "kv": [[cp_rows(ax_h, x_v, i, 7)] for i in (5, 6, 7)]
                  + [[cp_rows(wqkv_h.at[:, pl.ds(j * D, D)], w_v.at[j], n, 7)] for j in (2, 1) for n in range(U)],
            "f0": [cp_slab(f, 8) for f in range(NA)],
            "f1": [[cp_rows(wo_h, wo_v, n, 9)] + cp_slab(NA + n, 9) for n in range(U)]
                  + [cp_slab(f, 9) for f in range(NA + U, 2 * NA)],
            "f2": [cp_slab(f, 10) for f in range(2 * NA, NF)],
        }
        queue = [ds for name in batch for ds in batch[name]]
        flying = []
        arrived = []

        def start(ds):
            for d in ds:
                d.start()
                flying.append(d)

        def wait(ds):
            for d in ds:
                assert any(d is e for e in flying)
                flying[:] = [e for e in flying if e is not d]
                d.wait()

        def issue(n):
            for ds in queue[:n]:
                start(ds)
            del queue[:n]

        def arrive(name, then=0):
            wait([d for ds in batch[name] for d in ds])
            arrived.append(name)
            issue(then)

        def sync(name, then=0):
            return [(P["wait"][name], lambda: arrive(name, then))]

        issue(3)
        kv_v[...] = jnp.zeros_like(kv_v)
        z_v[...] = jnp.zeros_like(z_v)
        r128 = lax.broadcasted_iota(I32, (128, 128), 0)
        c128 = lax.broadcasted_iota(I32, (128, 128), 1)
        diag = (2 * ((r128 % 64) // 32) + r128 // 64) == (c128 // 32)
        eye = jnp.where(lax.broadcasted_iota(I32, (128, 32), 0) % 32 == lax.broadcasted_iota(I32, (128, 32), 1),
                        1.0, 0.0).astype(BF16)
        arrive("small")
        gw = gw_v[...].astype(F32).reshape(1, D)
        wr = wr_v[...].astype(F32).reshape(1, D)

        never = lax.broadcasted_iota(I32, (8, 128), 0) > (pltpu.bitcast(gw[:, 0:128], I32) & 0xFFFF) + 8
        clock = []
        due = {}

        def after(w, dep, every=False):
            if dep is None:
                return w
            dep = pltpu.bitcast(dep, w.dtype)
            if every:
                return jnp.concatenate([jnp.where(never, dep, w[r:r + 8]) for r in range(0, w.shape[0], 8)], axis=0)
            w0 = jnp.where(never, dep, w[0:8, 0:128])
            if w.shape[1] > 128:
                w0 = jnp.concatenate([w0, w[0:8, 128:]], axis=1)
            return jnp.concatenate([w0, w[8:]], axis=0) if w.shape[0] > 8 else w0

        def now(back, row=0):
            if len(clock) < back:
                return None
            t = clock[-back]
            row = row * 8 % t.shape[0]
            return t[row:row + 8, 0:128]

        def before(v, ahead):
            v = pltpu.bitcast(v, I32)
            parts = [v[r:r + 8, c:c + 128] for r in range(0, v.shape[0], 8) for c in range(0, v.shape[1], 128)]
            due.setdefault(len(clock) + ahead, []).append(_tree(parts, jnp.bitwise_or))

        def mm(w, rhs, dims):
            deps = due.pop(len(clock), [])
            if deps:
                w = after(w, _tree(deps, jnp.bitwise_or))
            t = lax.dot_general(_bf16(w), rhs, dims, preferred_element_type=F32)
            clock.append(t)
            return t

        bd = {}

        def prep_phi(groups):
            for g in groups:
                wp = wphi_v[pl.ds(4 * g, 4)].reshape(128, 32)
                t = lax.dot_general(eye, wp, NT, preferred_element_type=F32)
                bd[g] = pltpu.bitcast(jnp.where(diag, t, 0.0).astype(BF16), I32)

        def fold(j, s, n):
            def job(lo, hi):
                def run():
                    assert ("q%d" % min(s, 2) if j == 0 else "kv") in arrived
                    blocks = [mm(bd[g], _bf16(w_v[j, (k * K2 + lo) // 2:(k * K2 + hi) // 2, g * 128:(g + 1) * 128]), NT)
                              * LOG2E for g in (2 * s, 2 * s + 1) for k in range(2)]
                    for m, t in enumerate(_left(*blocks)):
                        wa_v[j, s, m, :, lo:hi] = _pack(t[0:64], t[64:128])
                return run
            return [job(c * K2 // n, (c + 1) * K2 // n) for c in range(n)]

        def prep_w(j, ref, s):
            def job(c):
                def run():
                    assert ("kv" if j == 2 else "f1") in arrived
                    rows = (c, U + c) if j == 2 else (2 * c, 2 * c + 1)
                    blocks = [pltpu.bitcast(_bf16(after(ref[r * 64:(r + 1) * 64, g * 128:(g + 1) * 128],
                                                        now(P["w_lag"]))).T, I32)
                              for g in (2 * s, 2 * s + 1) for r in rows]
                    lo, hi = [_left(*[_unpack(w, e) for w in blocks]) for e in range(2)]
                    for m in range(7):
                        w = blocks[0] if m == 2 else blocks[3] if m == 3 else _pack(lo[m], hi[m])
                        wa_v[j, s, m, :, c * 128:(c + 1) * 128] = w
                        if m not in (2, 3):
                            before(w, P["w_due"])
                return run
            return [job(c) for c in range(U)]

        def x_block(i, t, lo, n):
            return x_v[(2 * i + t) * 64:(2 * i + t + 1) * 64, lo:lo + n]

        route = [jnp.full((8, 1), -jnp.inf, F32), jnp.zeros((8, 1), I32)]
        first_x = [[] for _ in range(7)]

        def prep_x(i):
            acc = {}

            def job(c):
                def run():
                    assert ("x%d" % i if i < 2 else "x" if i < 5 else "kv") in arrived
                    c1, c2 = c * 128, K2 + c * 128
                    words = [after(x_block(i, 0, c1, 128), now(P["x_lag"]), True), x_block(i, 1, c1, 128),
                             x_block(i, 0, c2, 128), after(x_block(i, 1, c2, 128), now(P["x_lag"]), True)]
                    vals = [[_unpack(w, e) for w in words] for e in range(2)]
                    lo, hi = [_right(*v) for v in vals]
                    for m in range(7):
                        t = words[0] if m == 1 else words[3] if m == 4 else _pack(lo[m], hi[m])
                        if i == 0:
                            first_x[m].append(t)
                        else:
                            w = pltpu.bitcast(_bf16(t).T, I32)
                            xs_v[i, m, c * 64:(c + 1) * 64, :] = w
                            before(w[0:8], P["x_due"])
                    for t in range(2):
                        for e in range(2):
                            part = vals[e][t] * wr[:, c1:c1 + 128] + vals[e][2 + t] * wr[:, c2:c2 + 128]
                            acc[t, e] = part if c == 0 else acc[t, e] + part
                    if c < U - 1:
                        return
                    tok = i * T + 2 * lax.broadcasted_iota(I32, (8, 1), 0)
                    found = [tuple(route)]
                    for t in range(2):
                        rs = [jnp.sum(acc[t, e], axis=1, keepdims=True).astype(BF16).astype(F32) for e in range(2)]
                        rs = [jnp.where(r != r, -jnp.inf, r) for r in rs]
                        found += [(rs[e][8 * k:8 * k + 8], tok + (t * 128 + 16 * k + e))
                                  for k in range(8) for e in range(2)]
                    route[:] = _tree(found, lambda a, b: (jnp.maximum(a[0], b[0]), jnp.where(b[0] > a[0], b[1], a[1])))
                return run
            return [job(c) for c in range(U)]

        def proj(j, i, s, jobs):
            if i == 0:
                ops = [x_block(0, 0, 0, K2) if m == 1 else x_block(0, 1, K2, K2) if m == 4
                       else jnp.concatenate(first_x[m], axis=1) for m in range(7)]
                order = (1, 4, 0, 6, 5, 3, 2) if (j, s) == (0, 0) else P["order_q"]
                return _combine(lambda m: mm(wa_v[j, s, m], _bf16(ops[m]), NT), jobs, order)
            ops = [xs_v[i, m] for m in range(7)]
            return _combine(lambda m: mm(wa_v[j, s, m], _bf16(ops[m]), NN), jobs,
                            P["order_q"] if j == 0 else P["order_kv"])

        held = []

        def store_held():
            while held:
                where, val = held.pop(0)
                pq_v[where] = val

        def phi_q(i, s, ps):
            def job(e, q):
                def run():
                    rows = slice(q * 64, (q + 1) * 64)
                    for t in range(2):
                        phi = _phi(ps[e][t][rows], lambda v, k: after(v, now(P["phi_q_lag"], P["phi_rows"][t][k])))
                        held.append(((i, 2 * s + e, rows, slice(t * 128, (t + 1) * 128)), _pack(*phi)))
                    if i < NTILE - 1:
                        store_held()
                return run
            return [job(e, q) for e in range(2) for q in range(2)]

        prep_phi(range(2))
        arrive("q0", 1)
        _run(fold(0, 0, U))
        arrive("x0", 1)
        _run(prep_x(0))
        pv = [fn for s in range(U) for fn in prep_w(2, w_v.at[2], s)]
        pk = [fn for s in range(U) for fn in fold(1, s, 2)]
        px = [prep_x(i) for i in range(NTILE)]
        units = [(0, 0), (0, 1), (1, 0), (1, 1), (0, 2), (1, 2), (0, 3), (1, 3)]
        units += [(i, s) for i in range(2, NTILE - 1) for s in range(U)]
        pend = []
        for n, (i, s) in enumerate(units):
            jobs = []
            if n == 1:
                arrive("q1", 1)
                prep_phi(range(2, 4))
                _run(fold(0, 1, U))
                jobs += sync("x1", 2) + _at(P["x1"], px[1])
            elif n == 4:
                arrive("q2", 1)
                prep_phi(range(4, G))
                _run(fold(0, 2, U))
                jobs += _at(P["fold_q"], fold(0, 3, U))
            elif n > 4:
                issue(P["issue_a"][n - 5])
            if n == 7:
                jobs += sync("x") + _at(P["x2"], px[2])
            elif i in (2, 3):
                jobs += _at(P["x_early"], px[i + 1][s:s + 1])
            elif i == 4 and s >= 2:
                jobs += (sync("kv") if s == 2 else []) + _at(P["x_half"], px[5][2 * (s - 2):2 * (s - 1)])
            elif i > 4:
                k = (i - 5) * U + s
                jobs += (_at(P["x_late"], px[i + 1][s:s + 1]) + _at(P["prep_v"], pv[2 * k:2 * k + 2])
                         + _at(P["fold_k"], pk[k:k + 1]))
            pend = phi_q(i, s, proj(0, i, s, jobs + _at(P["phi_q"], pend)))

        top = jnp.max(route[0], axis=0, keepdims=True)
        idx = jnp.clip(jnp.min(jnp.where(route[0] == top, route[1], S)), 0, S - 1)
        blk = _bf16(x_v[pl.ds(pl.multiple_of((idx // 16) * 8, 8), 8), :]).astype(F32)
        sel = lax.broadcasted_iota(I32, (16, D), 0) == (idx % 16)
        xs = jnp.sum(jnp.where(sel, blk, 0.0), axis=0, keepdims=True)
        r_gate = jax.nn.sigmoid(jnp.sum(xs * wr, axis=1, keepdims=True).astype(BF16).astype(F32))

        def spread_token():
            for g in range(G):
                xb_v[g * 128:(g + 1) * 128, :] = after(
                    jnp.broadcast_to(xs[:, g * 128:(g + 1) * 128], (128, 128)), now(1)).T

        def tile(i):
            return idx // T if i == NTILE - 1 else i + (idx // T <= i).astype(I32)

        ffn = {"y": [jnp.zeros((8, K2), F32)] * 2}

        def ffn_up(f, k):
            def run():
                assert "f%d" % (f // NA) in arrived
                xb = after(xb_v[k * 256:(k + 1) * 256, :], now(P["ffn_lag"]))
                for name, w_ref in (("g", wg_v), ("u", wu_v)):
                    w = _bf16(w_ref[k * 128:(k + 1) * 128, f * 128:(f + 1) * 128]).astype(F32)
                    t = jnp.sum((w * xb).reshape(32, 8, 128), axis=0)
                    ffn[name, f, k] = t if k == 0 else ffn[name, f, k - 1] + t
                    before(ffn[name, f, k], P["ffn_due"])
                if k == 3:
                    g, u = [jnp.sum(ffn[name, f, k], axis=0, keepdims=True) for name in "gu"]
                    ffn["h", f] = jnp.broadcast_to(g * jax.nn.sigmoid(g) * u, (128, 128)).T
            return run

        def ffn_down(f, n):
            def run():
                w = _bf16(wd_v[f * 64:(f + 1) * 64, n * K2:(n + 1) * K2]).astype(F32)
                hb = jnp.concatenate([after(ffn["h", f], now(P["ffn_lag"]))] * U, axis=1)
                ffn["y"][n] = ffn["y"][n] + jnp.sum((w * hb).reshape(16, 8, K2), axis=0)
                ffn["done", f, n] = True
                before(ffn["y"][n], P["ffn_due"])
            return run

        def ffn_finish():
            assert all(("done", f, n) in ffn for f in range(NF) for n in range(2))
            ffn["out"] = jnp.sum(jnp.concatenate(ffn["y"], axis=1), axis=0, keepdims=True) * r_gate

        ffn_left = [fn for f in range(NF) for fn in [ffn_up(f, k) for k in range(4)] + [ffn_down(f, n) for n in range(2)]]
        ffn_left.append(ffn_finish)

        def take(n):
            got, ffn_left[:] = ffn_left[:n], ffn_left[n:]
            return got

        def gates(i):
            def job(t, r0):
                def run():
                    lo = (i * T + t * 128 + r0) // 2
                    xt = _bf16(after(x_v[lo:lo + 32, :], now(P["gate_lag"][i > 1]))).astype(F32)
                    gate = jnp.broadcast_to(jax.nn.sigmoid(jnp.sum(xt * gw, axis=1, keepdims=True)), (64, 128))
                    gate_v[i, t, r0:r0 + 64, :] = gate
                    before(gate, P["gate_due"][i > 1])
                return run
            return [job(t, r0) for t in range(2) for r0 in (0, 64)]

        kr = lax.broadcasted_iota(I32, (64, 128), 0)
        kc = lax.broadcasted_iota(I32, (64, 128), 1)
        same_head = (kr // 32) == ((kc // 2) % 2)
        kvb = {}

        def kv_step(i, s, ps, vs):
            def job(e, q):
                def run():
                    g = 2 * s + e
                    j = 2 * g + q
                    rows = slice(q * 64, (q + 1) * 64)
                    phis = [_phi(ps[e][t][rows], lambda v, k: after(v, now(P["kv_lag"], P["phi_rows"][t][k])))
                            for t in range(2)]
                    zs = [z_v[g, sign, rows] + (phis[0][sign] + phis[1][sign]) for sign in range(2)]
                    phi = jnp.concatenate([_pack(*ph) for ph in phis], axis=1)
                    kv_v[j] += mm(vs[2 * e + q], _bf16(phi), NT)
                    if i == NTILE - 1:
                        zs = [jnp.broadcast_to(jnp.sum(z, axis=1, keepdims=True), (64, 128)) for z in zs]
                        t = jnp.concatenate([kv_v[j, pl.ds(h, 32, stride=2), :] for h in range(2)], axis=0)
                        kvb[j] = pltpu.bitcast(jnp.where(same_head, t, 0.0).astype(BF16), I32)
                    for sign in range(2):
                        z_v[g, sign, rows] = zs[sign]
                return run
            return [job(e, q) for e in range(2) for q in range(2)]

        o_pairs, o_parts = {}, {}

        def attn(i, g):
            def pair(h, q):
                def run():
                    rows = slice(q * 64, (q + 1) * 64)
                    w = pq_v[tile(i), h, rows]
                    den = (_unpack(w, 0) * jnp.concatenate([after(z_v[h, 0, rows], now(P["attn_lag"]))] * 2, axis=1)
                           + _unpack(w, 1) * jnp.concatenate([z_v[h, 1, rows]] * 2, axis=1))
                    rden = 1.0 / (_per_head(den.reshape(8, 8, T), jnp.add) + 1e-6)
                    num = mm(kvb[2 * h + q], _bf16(w), NN)
                    o_pairs[i, h, q] = [num[0:32] * rden[0:1], num[32:64] * rden[1:2]]
                return run

            def join():
                a, b = [jnp.concatenate(o_pairs.pop((i, h, 0)) + o_pairs.pop((i, h, 1)), axis=0)
                        for h in (2 * g, 2 * g + 1)]
                o_parts[i, g] = _right(a[:, :128], a[:, 128:], b[:, :128], b[:, 128:])

            return [pair(h, q) for h in (2 * g, 2 * g + 1) for q in range(2)] + [join]

        first = [attn(0, g) for g in range(U)]
        po = [fn for s in range(U) for fn in prep_w(3, wo_v, s)]
        for i in range(NTILE):
            gj = gates(i)
            for s in range(U):
                fj = [spread_token] if (i, s) == (0, 0) else take(P["ffn_jobs"][i][s])
                issue(P["issue_b"][i][s])
                half = len(fj) // 2
                jobs = sync("f0") if (i, s) == (2, 0) else sync("f1") if (i, s) == (5, 0) else []
                jobs += (_at(P["kv_v"], pend[:2]) + _at(P["ffn_v"][3 - half:], fj[:half]) + _at(P["gate"][i > 1], gj[s:s + 1]))
                vt = proj(2, i, s, jobs)
                vs = [jnp.concatenate([_pack(b[q * 64:q * 64 + 32], b[q * 64 + 32:q * 64 + 64]) for b in vt[e]], axis=1)
                      for e in range(2) for q in range(2)]
                jobs = _at(P["kv_k"], pend[2:]) + _at(P["ffn_k"], fj[half:])
                if i in (5, 6):
                    k = (i - 5) * U + s
                    jobs += _at(P["prep_o"], po[2 * k:2 * k + 2])
                if i == NTILE - 1 and s >= 2:
                    jobs += _at(P["attn_b"], first[s - 2])
                pend = kv_step(i, s, proj(1, i, s, jobs), vs)

        for s in range(U):
            jobs = _at(P["phi_q_last"], pend)
            for g in range(2, U):
                jobs += [(n - 7 * s, fn) for n, fn in _at(P["attn_a"][g - 2], first[g]) if n // 7 == s]
            pend = phi_q(NTILE - 1, s, proj(0, NTILE - 1, s, jobs))

        outs = []

        def store_out(i, r0, nr, c0, nc):
            rows = pl.ds(pl.multiple_of(tile(i) * T + r0, 128), nr)
            outs.append(cp(out_v.at[pl.ds(i * T + r0, nr), pl.ds(c0, nc)], out_h.at[rows, pl.ds(c0, nc)], 11))
            start(outs[-1:])

        def mix(i, c, blocks):
            def job(n, t):
                def run():
                    r0, c0 = i * T + t * 128, (2 * c + n) * 128
                    g = gate_v[tile(i), t]
                    xt = _bf16(x_v[pl.ds(pl.multiple_of(tile(i) * 128 + t * 64, 64), 64), c0:c0 + 128]).astype(F32)
                    upd = xt * 0.0
                    if i == NTILE - 1:
                        tok = t * 128 + lax.broadcasted_iota(I32, (128, 128), 0)
                        upd = upd + jnp.where(tok == idx % T, ffn["out"][:, c0:c0 + 128], 0.0)
                    a = after(blocks[n][t], now(P["mix_lag"], P["mix_rows"][2 * t + n])).T
                    res = g * a + (1.0 - g) * (xt + upd)
                    out_v[r0:r0 + 128, c0:c0 + 128] = res.astype(BF16)
                    before(res, P["mix_due"])
                    if i == NTILE - 1:
                        if n == 1:
                            store_out(i, t * 128, 128, c * 256, 256)
                    elif (c, n, t) == (U - 1, 1, 1):
                        store_out(i, 0, T, 0, D)
                return run
            return [job(n, t) for t in range(2) for n in range(2)]

        assert list(P["mix"]) == sorted(P["mix"])
        for i in range(NTILE):
            parts = [o_parts.pop((i, g)) for g in range(U)]
            ops = [jnp.concatenate([p[m] for p in parts], axis=0).astype(BF16) for m in range(7)]
            aj = [fn for g in range(U) for fn in attn(i + 1, g)] if i + 1 < NTILE else []
            for c in range(U):
                if (i, c) == (1, 0):
                    store_held()
                jobs = (sync("f2") if (i, c) == (0, 0) else []) + _at(P["mix"], pend)
                jobs += [(n - 7 * c, fn) for n, fn in _at(P["attn"], aj) if n // 7 == c] + _at(P["ffn_c"], take(1))
                last = (i, c) == (NTILE - 1, U - 1)
                early = (lambda c11, c21: _run(mix(i, c, ((c11, None), (c21, None)))[:2])) if last else None
                pend = mix(i, c, _combine(lambda m: mm(wa_v[3, c, m], ops[m], NN), jobs, P["order_o"], early))
        _run(pend[2:])
        wait(outs)
        assert not (flying or queue or held or ffn_left)

    return kernel


def _build(P):
    def run(A_x, A_wqkv, A_w_phi, A_wo, B_x, B_w_r, B_w_gate, B_w_up, B_w_down, gate_w):
        B, S, D = A_x.shape
        F = B_w_gate.shape[1]
        H = A_w_phi.shape[0]
        NTILE, G = S // T, D // 128
        hbm = pl.BlockSpec(memory_space=pl.ANY)
        V = pltpu.VMEM
        scratch = [
            V((S // 2, D), I32),
            V((NTILE, 7, D // 4, 128), I32),
            V((3, D // 2, D), I32),
            V((4, G // 2, 7, 64, D // 2), I32),
            V((H, 32, 32), BF16),
            V((D // 2, D), I32),
            V((D,), BF16),
            V((D,), BF16),
            V((D // 2, F), I32),
            V((D // 2, F), I32),
            V((F // 2, D), I32),
            V((NTILE, G, 128, T), I32),
            V((NTILE, 2, 128, 128), F32),
            V((H // 2, 64, 128), F32),
            V((G, 2, 128, 128), F32),
            V((D, 128), F32),
            V((S, D), BF16),
            pltpu.SemaphoreType.DMA((12,)),
        ]
        out = pl.pallas_call(
            _make_kernel(S, D, F, H, P),
            out_shape=jax.ShapeDtypeStruct((S, D), BF16),
            in_specs=[hbm] * 9,
            out_specs=hbm,
            scratch_shapes=scratch,
            compiler_params=pltpu.CompilerParams(vmem_limit_bytes=110 * 2**20),
        )(A_x.reshape(S, D), A_wqkv, A_w_phi, A_wo, B_w_r, B_w_gate, B_w_up, B_w_down, gate_w)
        return out.reshape(B, S, D)
    return run


@jax.jit
def pallas_gated_mix__linear_kernel_hedgehog__moe_arch_mod__prompt_kernel(
    A_x: jax.Array,
    A_wqkv: jax.Array,
    A_w_phi: jax.Array,
    A_wo: jax.Array,
    B_x: jax.Array,
    B_w_r: jax.Array,
    B_w_gate: jax.Array,
    B_w_up: jax.Array,
    B_w_down: jax.Array,
    gate_w: jax.Array,
):
    return _build(_PLACE)(A_x, A_wqkv, A_w_phi, A_wo, B_x, B_w_r, B_w_gate, B_w_up, B_w_down, gate_w)
```
